```python
import jax
import jax.numpy as jnp

def _softmax(x, axis=-1):
    return jax.nn.softmax(x, axis=axis)
def _gelu(x):
    return jax.nn.gelu(x, approximate=True)
def _silu(x):
    return jax.nn.silu(x)
def _sigmoid(x):
    return jax.nn.sigmoid(x)
def _layernorm(x, axis=-1, eps=1e-5):
    m = jnp.mean(x, axis=axis, keepdims=True)
    v = jnp.var(x, axis=axis, keepdims=True)
    return (x - m) / jnp.sqrt(v + eps)
def _scatter_add(tgt, idx, src, axis=0):
    return tgt.at[idx].add(src)
def _segment_sum(src, seg, n):
    return jax.ops.segment_sum(src, seg, n)
class _Rng:
    def __init__(self, key):
        self._k = key
    def _next(self):
        self._k, sub = jax.random.split(self._k)
        return sub
    def normal(self, shape):
        return jax.random.normal(self._next(), shape, dtype=jnp.bfloat16)
    def randint(self, lo, hi, shape):
        return jax.random.randint(self._next(), shape, lo, hi, dtype=jnp.int32)
    def uniform(self, shape, lo=0.0, hi=1.0):
        return jax.random.uniform(self._next(), shape, jnp.bfloat16, lo, hi)
    def permutation(self, n):
        return jax.random.permutation(self._next(), n)


kernel_name = 'interleave_layers__sliding_local_dilated__dense_activation_squared_relu__prompt'

def setup_inputs():
    _rng = _Rng(jax.random.key(int.from_bytes(__import__("os").urandom(4), "little")))
    _w = (lambda a: (lambda t: t.astype(jnp.bfloat16) if jnp.issubdtype(t.dtype, jnp.floating) else t)(jnp.asarray(a)))
    def _A_setup():
        B, S, D = 1, 2048, 1024
        return {
            "x": _w((lambda *s: _rng.normal(s) * 0.05)(B, S, D)),
            "wqkv": _w((lambda *s: _rng.normal(s) * 0.05)(D, 3 * D)),
            "wo": _w((lambda *s: _rng.normal(s) * 0.05)(D, D)),
        }
    _A_in = _A_setup()

    def _B_setup():
        B, S, D, F = 1, 2048, 1024, 3584
        return {
            "x": _w((lambda *s: _rng.normal(s) * 0.05)(B, S, D)),
            "w1": _w((lambda *s: _rng.normal(s) * 0.05)(D, F)),
            "b1": _w((lambda *s: _rng.normal(s) * 0.05)(F)),
            "w2": _w((lambda *s: _rng.normal(s) * 0.05)(F, D)),
            "b2": _w((lambda *s: _rng.normal(s) * 0.05)(D)),
        }
    _B_in = _B_setup()

    return {
        "A_x": _A_in["x"],
        "A_wqkv": _A_in["wqkv"],
        "A_wo": _A_in["wo"],
        "B_x": _B_in["x"],
        "B_w1": _B_in["w1"],
        "B_b1": _B_in["b1"],
        "B_w2": _B_in["w2"],
        "B_b2": _B_in["b2"],
    }

def reference(A_x, A_wqkv, A_wo, B_x, B_w1, B_b1, B_w2, B_b2):
    def _A_ref(x, wqkv, wo):
        B, S, D = x.shape
        H = 32; Dh = D // H
        W, dil = 8, 2
        qkv = (lambda x, *d: x.transpose(*d))((x @ wqkv).reshape(B, S, 3, H, Dh), 2, 0, 3, 1, 4)
        q, k, v = qkv[0], qkv[1], qkv[2]
        scale = Dh ** -0.5
        pos = jnp.arange(S)
        off = jnp.arange(W) * dil
        idx = pos[:, None] - off[None, :]
        mask = idx >= 0
        idx_c = jnp.where(mask, idx, 0).reshape(-1)
        kg = k[:, :, idx_c, :].reshape(B, H, S, W, Dh)
        vg = v[:, :, idx_c, :].reshape(B, H, S, W, Dh)
        logits = jnp.einsum("bhsd,bhswd->bhsw", q, kg) * scale
        logits = jnp.where(mask[None, None, :, :], logits, -1e9)
        attn = _softmax(logits, axis=-1)
        o = jnp.einsum("bhsw,bhswd->bhsd", attn, vg)
        return (lambda x, *d: x.transpose(*d))(o, 0, 2, 1, 3).reshape(B, S, D) @ wo

    def _B_ref(x, w1, b1, w2, b2):
        h = jnp.einsum("bsd,df->bsf", x, w1) + b1
        zero = jnp.zeros_like(h)
        r = jnp.where(h > zero, h, zero)
        h = r * r
        out = jnp.einsum("bsf,fd->bsd", h, w2) + b2
        return out

    x = A_x
    x = x + _A_ref(_layernorm(x, axis=-1), A_wqkv, A_wo)
    x = x + _B_ref(_layernorm(x, axis=-1), B_w1, B_b1, B_w2, B_b2)
    x = x + _A_ref(_layernorm(x, axis=-1), A_wqkv, A_wo)
    x = x + _B_ref(_layernorm(x, axis=-1), B_w1, B_b1, B_w2, B_b2)
    return x
```

```python
import contextlib
import functools
import numpy as np
import jax
import jax.numpy as jnp
from jax import lax
import jax.experimental.pallas as pl
import jax.experimental.pallas.tpu as pltpu

S, D, F = 2048, 1024, 3584
H, DH, W, DIL = 32, 32, 8, 2
TM = 512
HM = TM // 2
HF = F // 2
NT = S // TM
HALO = 16
EPS = 1e-5
TINY = 1e-30
QSCALE = float(DH ** -0.5 * np.log2(np.e))
NEG = float(-1e9 * np.log2(np.e))
f32, bf16, u32 = jnp.float32, jnp.bfloat16, jnp.uint32
SCOPES = False
MODE = "all"
NPRE = 4
QK = (10900, 21500)
PV = (21000, 32200)
L2B = (36600, 39900)
THREE = 1
TQK = 1
TPV = 0
TL2 = 0
OPQ = 1
LN3 = 0
G1 = 0
L1 = (42000, 60000)
L2A = (0, 0)
DS = 1
D1POS = 2
RC0 = 128
RCQ = 256
RCL = 128
CB = 5
QKF = (14000, 21400)
L1F = (34500, 45500)
RC1 = 32


def _tree(op, xs):
    xs = list(xs)
    while len(xs) > 1:
        xs = [op(xs[i], xs[i + 1]) if i + 1 < len(xs) else xs[i] for i in range(0, len(xs), 2)]
    return xs[0]


def _a_sums(a11, a12, a21, a22):
    return (a11 + a22, a21 + a22, a11, a22, a11 + a12, a21 - a11, a12 - a22)


def _b_sums(c11, c12, c21, c22):
    return (c11 + c22, c11, c12 - c22, c21 - c11, c22, c11 + c12, c21 + c22)


def _pow2(s):
    bits = pltpu.bitcast(s, jnp.int32)
    return pltpu.bitcast((bits + 0x007FFFFF) & 0x7F800000, f32)


def _tile(j, n=1):
    return slice(j * 128, (j + n) * 128)


def _skew_select(ts, index, unit):
    ts = [ts[-i % 8] for i in range(8)]
    for b in (1, 2, 4):
        take = (index & (unit * b)) != 0
        ts = [jnp.where(take, ts[(i - b) % 8], ts[i]) for i in range(8)]
    return ts


def _kernel(zero_ref, x_hbm, wqkv_hbm, wo_hbm, w1_hbm, b1_ref, w2_hbm, b2_ref, out_hbm,
            ostage, xin, x, wqkv_raw, wo_raw, w1_raw, w2_raw,
            wq, wo, w1, w2, xs1, xs2, os_, hs, qa, qb, k, v, wv, pra, prb, ua, xt, part, pre, carry,
            mu0, mu1, gg0, gg1, s1, sq, s2, so, sg, gh, sh, b1, b2, stat, isem, osem):
    sub = lax.broadcasted_iota(jnp.int32, (8, 128), 0)
    P = functools.partial

    zero = zero_ref[0]
    never = jnp.full((16, 128), zero, jnp.int32).astype(bf16) != 0
    clock = [0]
    queue = []

    def plan(window, items):
        lo, hi = window
        queue.extend((lo + (hi - lo) * (n + 1) / len(items), f) for n, f in enumerate(items))
        queue.sort(key=lambda e: e[0])

    later = []

    def now(window, items):
        later.append(items)

    def release():
        if later:
            for f in later.pop(0):
                f()

    def flush(until):
        vals = []
        while queue and queue[0][0] <= until:
            vals.append(queue.pop(0)[1]())
        return vals

    def tie(panel, r, vals):
        d = _tree(jnp.add, vals)
        d = jnp.concatenate([d, d], axis=0).astype(bf16)
        parts = [panel[:r], jnp.where(never, d, panel[r:r + 16]), panel[r + 16:]]
        return jnp.concatenate([p for p in parts if p.shape[0]], axis=0)

    def mm(a_ref, w_ref, i, c):
        kt = a_ref.shape[1]
        ls = [a_ref[i, t] for t in range(kt)]
        t0 = clock[0]
        if kt == 4:
            out = []
            for n in range(2):
                l0 = ls[0]
                for r in range(0, HM, 64):
                    vals = flush(t0 + n * 256 + r + 63)
                    if vals:
                        l0 = tie(l0, r, vals)
                out.append(jnp.dot(jnp.concatenate([l0] + ls[1:], axis=1), w_ref[i, 2 * c + n],
                                   preferred_element_type=f32))
            clock[0] = t0 + 512
            return jnp.concatenate(out, axis=1)
        rs = [w_ref[i, 2 * c + n] for n in range(2)]
        for g in range(3):
            for r in range(0, HM, 64):
                vals = flush(t0 + g * 256 + r + 63)
                if vals:
                    ls[4 * g] = tie(ls[4 * g], r, vals)
        for g in range(4):
            for u in range(2):
                vals = flush(t0 + 768 + g * 256 + u * 128 + 127)
                if vals:
                    rs[1] = tie(rs[1], (4 * g + u) * 128, vals)
        clock[0] = t0 + 128 * kt
        return jnp.dot(jnp.concatenate(ls, axis=1), jnp.concatenate(rs, axis=1), preferred_element_type=f32)

    def put(dst, i, t0, rows, val):
        for t in range(val.shape[1] // 128):
            dst[i, t0 + t, rows, :] = val[:, _tile(t)].astype(bf16)

    def put_a(dst, r, ua_):
        ua[r:r + 16, :] = ua_
        put(dst, 2, 0, slice(r, r + 16), ua_[:, :512])
        put(dst, 4, 0, slice(r, r + 16), ua_[:, :512] + ua_[:, 512:])

    def put_b(dst, r, ub):
        ss = _a_sums(ua[r:r + 16, :512], ua[r:r + 16, 512:], ub[:, :512], ub[:, 512:])
        for i in (0, 1, 3, 5, 6):
            put(dst, i, 0, slice(r, r + 16), ss[i])

    gate = []

    def ln(xv, g_=None):
        if g_ is not None:
            nv = jnp.full((16, 128), zero, jnp.int32) != 0
            xv = jnp.concatenate([jnp.where(nv, g_, xv[:, :128]), xv[:, 128:]], axis=1)
        z = xv - jnp.sum(xv, axis=1, keepdims=True) * (1.0 / D)
        var = jnp.sum(z * z, axis=1, keepdims=True) * (1.0 / D)
        vt = jnp.maximum(var, TINY)
        g = lax.rsqrt(vt)
        s = lax.rsqrt(var + EPS) * (vt * g)
        return z * g, jnp.broadcast_to(s, (xv.shape[0], 128))

    def ln1(base, n, r):
        if True:
            g_ = gate[-1][r:r + n, 0:128] if gate else None
            ua_, sa = ln(x[pl.ds(pl.multiple_of(base + r, n), n), :], g_)
            ub, sb = ln(x[pl.ds(pl.multiple_of(base + HM + r, n), n), :], g_)
            ss = _a_sums(ua_[:, :512], ua_[:, 512:], ub[:, :512], ub[:, 512:])
            for i in range(7):
                put(xs1, i, 0, slice(r, r + n), ss[i])
            s1[r:r + n, :] = sa
            s1[HM + r:HM + r + n, :] = sb
            sq[r:r + n, :] = sa * QSCALE
            sq[HM + r:HM + r + n, :] = sb * QSCALE
            wv[HALO + r:HALO + r + n, :] = _pow2(sa)
            wv[HALO + HM + r:HALO + HM + r + n, :] = _pow2(sb)
            return (sa + sb)[0:8]

    def ln2_3(half, n, rr):
        mu, gg = (mu0, gg0) if half == 0 else (mu1, gg1)
        at = lambda z, r: pl.ds(pl.multiple_of(zero_ref[z] + r, n), n)
        if rr is None:
            for r in range(0, HM, n):
                xv = xt[at(0, half * HM + r), :]
                mu[r:r + n, :] = jnp.broadcast_to(jnp.sum(xv, axis=1, keepdims=True) * (1.0 / D), (n, 128))
            for r in range(0, HM, n):
                m = mu[at(1, r), :]
                z = _tree(jnp.add, [jnp.square(xt[at(1, half * HM + r), _tile(j)] - m) for j in range(8)])
                var = jnp.broadcast_to(jnp.sum(z, axis=1, keepdims=True) * (1.0 / D), (n, 128))
                vt = jnp.maximum(var, TINY)
                g = lax.rsqrt(vt)
                s = lax.rsqrt(var + EPS) * (vt * g)
                gg[r:r + n, :] = g
                rows = slice(half * HM + r, half * HM + r + n)
                p = s * s * stat[0:1, :] + stat[1:2, :]
                g = lax.rsqrt(p)
                gh[rows, :] = g
                sg[rows, :] = s * g
                sh[rows, :] = p
            return
        r = rr
        m, g = mu[at(2, r), :], gg[at(2, r), :]
        u = jnp.concatenate([(xt[at(2, half * HM + r), _tile(j)] - m) * g for j in range(8)], axis=1)
        (put_b if half else put_a)(xs2, r, u)
        return u[0:8, 0:128]

    def ln2(half, r):
        if LN3:
            if r == 0:
                ln2_3(half, 16, None)
            return ln2_3(half, 16, r)
        if True:
            rows = slice(half * HM + r, half * HM + r + 16)
            u, s = ln(xt[rows, :])
            (put_b if half else put_a)(xs2, r, u)
            p = s * s * stat[0:1, :] + stat[1:2, :]
            g = lax.rsqrt(p)
            gh[rows, :] = g
            sg[rows, :] = s * g
            sh[rows, :] = p
            return p[0:8]

    def qkv_dst(g, j, half):
        if g == 0:
            return (qa, qb)[half].at[j]
        return (k, v)[g - 1].at[j, pl.ds(HALO + half * HM, HM), :]

    def qkv_p1(g, c):
        sc = (sq if g == 0 else s1)[0:HM, :]
        sc = jnp.concatenate([sc, sc], axis=1)
        md = P(mm, xs1, wq, c=g * 2 + c)

        def out(j, half, val):
            for t in range(2):
                qkv_dst(g, c * 2 + j + t, half)[...] = val[:, _tile(t)]
        m3 = md(2)
        m5 = md(4)
        out(4, 0, (m3 + m5) * sc)
        m1 = md(0)
        out(4, 1, m1 + m3)
        acc = m1 - m5
        m4 = md(3)
        out(0, 1, m4)
        out(0, 0, (acc + m4 + md(6)) * sc)

    def qkv_p2(g, c):
        sc = (sq if g == 0 else s1)[HM:TM, :]
        m2 = mm(xs1, wq, 1, g * 2 + c)
        acc = []
        for t in range(2):
            l, r = qkv_dst(g, c * 2 + t, 1), qkv_dst(g, c * 2 + t + 4, 1)
            l[...] = (l[...] + m2[:, _tile(t)]) * sc
            acc.append(r[...] - m2[:, _tile(t)])
        m6 = mm(xs1, wq, 5, g * 2 + c)
        for t in range(2):
            qkv_dst(g, c * 2 + t + 4, 1)[...] = (acc[t] + m6[:, _tile(t)]) * sc

    def qk8(r, first):
        rq = pl.ds(pl.multiple_of(zero + r % HM, 8), 8) if OPQ else pl.ds(r % HM, 8)
        qs = [(qa, qb)[r // HM][j, rq, :] for j in range(8)]
        ls = []
        for w in range(W):
            s0 = HALO + r - DIL * w
            p = _tree(jnp.add, [qs[j] * k[j, s0:s0 + 8, :] for j in range(8)])
            if THREE:
                p = (p + pltpu.roll(p, 64, 1)) + (pltpu.roll(p, 32, 1) + pltpu.roll(p, 96, 1))
            else:
                p = p + pltpu.roll(p, 64, 1)
                p = p + pltpu.roll(p, 32, 1)
            if r - DIL * w < 0:
                p = jnp.where(jnp.logical_and(first, sub + (r - DIL * w) < 0), NEG, p)
            ls.append(p)
        m = _tree(jnp.maximum, ls)
        es = [jnp.exp2(l - m) for l in ls]
        sc = _tree(jnp.maximum, [wv[HALO + r - DIL * w:HALO + r - DIL * w + 8, :] for w in range(W)])
        so[r:r + 8, :] = sc
        inv = pltpu.bitcast(0x7F000000 - pltpu.bitcast(sc, jnp.int32), f32) / _tree(jnp.add, es)
        for w in range(W):
            (pra, prb)[r // HM][w, r % HM:r % HM + 8, :] = es[w] * inv
        return inv

    def pv8(r):
        rp = pl.ds(pl.multiple_of(zero + r % HM, 8), 8) if OPQ else pl.ds(r % HM, 8)
        ps = [(pra, prb)[r // HM][w, rp, :] for w in range(W)]
        return jnp.concatenate(
            [_tree(jnp.add, [ps[w] * v[j, HALO + r - DIL * w:HALO + r - DIL * w + 8, :] for w in range(W)])
             for j in range(8)], axis=1)

    def pv16(half, r):
        r0 = half * HM + r
        u = jnp.concatenate([pv8(r0), pv8(r0 + 8)], axis=0)
        (put_b if half else put_a)(os_, r, u)
        return _tree(jnp.add, [u[0:8, _tile(j)] + u[8:16, _tile(j)] for j in range(8)])

    def v_first(first):
        for j in range(8):
            v0 = jnp.broadcast_to(v[j, HALO:HALO + 1, :], (HALO, 128))
            v[j, 0:HALO, :] = jnp.where(first, v0, v[j, 0:HALO, :])

    def halo_save():
        wv[0:HALO, :] = wv[TM:TM + HALO, :]
        for j in range(8):
            k[j, 0:HALO, :] = k[j, TM:TM + HALO, :]
            v[j, 0:HALO, :] = v[j, TM:TM + HALO, :]

    def acc_x(base, half, j, val):
        rows = pl.ds(pl.multiple_of(base + half * HM, HM), HM)
        sc = so[half * HM:(half + 1) * HM, :]
        for t in range(2):
            r = x[rows, _tile(j + t)] + val[:, _tile(t)] * sc
            xt[half * HM:(half + 1) * HM, _tile(j + t)] = r
            if half:
                x[rows, _tile(j + t)] = r

    def wo_p1(base, c):
        m3 = mm(os_, wo, 2, c)
        part[2, :, _tile(c * 2, 2)] = m3
        m5 = mm(os_, wo, 4, c)
        part[0, :, _tile(c * 2, 2)] = m5
        acc_x(base, 0, 4 + c * 2, m3 + m5)

    def wo_p2(base, c):
        cols = _tile(c * 2, 2)
        m1 = mm(os_, wo, 0, c)
        part[2, :, cols] = part[2, :, cols] + m1
        acc = m1 - part[0, :, cols]
        m4 = mm(os_, wo, 3, c)
        part[1, :, cols] = m4
        acc_x(base, 0, c * 2, acc + m4 + mm(os_, wo, 6, c))

    def wo_p3(base, c):
        cols = _tile(c * 2, 2)
        m2 = mm(os_, wo, 1, c)
        acc_x(base, 1, c * 2, part[1, :, cols] + m2)
        acc = part[2, :, cols] - m2
        acc_x(base, 1, 4 + c * 2, acc + mm(os_, wo, 5, c))

    def w1_pre(c):
        pre[0, :, _tile(c * 2, 2)] = mm(xs2, w1, 2, c)
        pre[1, :, _tile(c * 2, 2)] = mm(xs2, w1, 4, c)

    def w1_chunk(c):
        md = P(mm, xs2, w1, c=c)

        def act(z, half, side):
            rows = slice(half * HM, (half + 1) * HM)
            out = []
            for t in range(2):
                b = b1[0:1, _tile(side * 14 + c * 2 + t)]
                y = jnp.maximum(z[:, _tile(t)] * sg[rows, :] + gh[rows, :] * b, 0.0)
                out.append(y * y)
            return jnp.concatenate(out, axis=1)

        def out(i, val):
            put(hs, i, c * 2, slice(0, HM), val)
        if c < NPRE:
            m3, m5 = pre[0, :, _tile(c * 2, 2)], pre[1, :, _tile(c * 2, 2)]
        else:
            m3, m5 = md(2), md(4)
        h12 = act(m3 + m5, 0, 1)
        m4 = md(3)
        acc1 = m4 - m5
        m2 = md(1)
        h21 = act(m4 + m2, 1, 0)
        acc2 = m3 - m2
        m1 = md(0)
        acc1, acc2 = acc1 + m1, acc2 + m1
        h22 = act(acc2 + md(5), 1, 1)
        out(1, h21 + h22)
        out(3, h22)
        out(6, h12 - h22)
        h11 = act(acc1 + md(6), 0, 0)
        if G1 and c == 6:
            gate.append(h11)
        out(0, h11 + h22)
        out(2, h11)
        out(4, h11 + h12)
        out(5, h21 - h11)

    def fin(res, base, slot, half, c, side, val, sc):
        rows = pl.ds(pl.multiple_of(base + half * HM, HM), HM)
        for t in range(2):
            cols = _tile(side * 4 + c * 2 + t)
            r = res(rows, cols) + val[:, _tile(t)] * sc + b2[0:1, cols]
            x[rows, cols] = r
            ostage[slot, half, :, cols] = r.astype(bf16)

    def w2_p1(base, slot, c):
        done = P(fin, lambda rows, cols: xt[0:HM, cols], base, slot, 0, c, sc=sh[0:HM, :])
        m3 = mm(hs, w2, 2, c)
        m5 = mm(hs, w2, 4, c)
        done(1, m3 + m5)
        m1 = mm(hs, w2, 0, c)
        carry[1, :, _tile(2 * c, 2)] = m1 + m3
        acc = m1 - m5
        m4 = mm(hs, w2, 3, c)
        carry[0, :, _tile(2 * c, 2)] = m4
        done(0, acc + m4 + mm(hs, w2, 6, c))
        if c == 1:
            carry[2, :, 0:128] = sh[HM:TM, :]

    def w2_p2(base, slot, c):
        done = P(fin, lambda rows, cols: x[rows, cols], base, slot, 1, c, sc=carry[2, :, 0:128])
        m2 = mm(hs, w2, 1, c)
        done(0, carry[0, :, _tile(2 * c, 2)] + m2)
        acc = carry[1, :, _tile(2 * c, 2)] - m2
        done(1, acc + mm(hs, w2, 5, c))

    def out_copy(slot, half, t):
        row = pl.multiple_of((t % NT) * TM + half * HM, HM)
        return pltpu.make_async_copy(ostage.at[slot, half], out_hbm.at[pl.ds(row, HM), :], osem.at[half])

    def put_sums(dst, rows, t, blocks):
        for i, s in enumerate(_b_sums(*blocks)):
            put(dst, i, t, rows, s)

    def permuted(r, n, g):
        lane = lax.broadcasted_iota(jnp.int32, (n // 2, 128), 1)
        src = ((lane & 31) << 2) | (lane >> 5)
        ts = [pltpu.bitcast(wqkv_raw[r:r + n, _tile(g * 8 + j)], u32) for j in range(8)]
        ts = [pltpu.roll(t, 4 * j, 1) if j else t for j, t in enumerate(ts)]
        ts = _skew_select(ts, lane, 4)
        return [pltpu.bitcast(jnp.take_along_axis(t, (src + 4 * j) & 127, axis=1), bf16).astype(f32)
                for j, t in enumerate(ts)]

    def prep_qkv(g, n, lo, hi):
        for r in range(lo, hi, n):
            p = permuted(r, n, g)
            wq_rows = slice(r, r + n)
            p2 = permuted(512 + r, n, g)
            for t in range(4):
                put_sums(wq, wq_rows, g * 4 + t, (p[t], p[t + 4], p2[t], p2[t + 4]))

    def prep_wo():
        for hl in range(4):
            for d3 in range(2):
                blk = {}
                for d4 in range(2):
                    src = []
                    for hh in range(8):
                        r = hh * 128 + hl * 32 + d4 * 16
                        t = wo_raw[r:r + 16, :].astype(f32)[8 * d3:8 * d3 + 8]
                        src.append(pltpu.roll(t, hh, 0) if hh else t)
                    for dl, t in enumerate(_skew_select(src, sub[:, :1], 1)):
                        blk[d4, dl] = pltpu.roll(t, 8 - dl, 0) if dl else t
                for dl in range(8):
                    r = d3 * 256 + dl * 32 + (hl // 2) * 16
                    blk[dl, hl] = (blk[0, dl], blk[1, dl])
                wo_tmp[hl, d3] = blk

    wo_tmp = {}

    def prep_wo():
        for d3 in range(2):
            for h1 in range(2):
                blk = {}
                for d4 in range(2):
                    for h0 in range(2):
                        src = []
                        for hh in range(8):
                            r = hh * 128 + h1 * 64 + h0 * 32 + d4 * 16
                            t = wo_raw[r:r + 16, :].astype(f32)[8 * d3:8 * d3 + 8]
                            src.append(pltpu.roll(t, hh, 0) if hh else t)
                        index = lax.broadcasted_iota(jnp.int32, (8, D), 0)
                        for dl, t in enumerate(_skew_select(src, index, 1)):
                            blk[d4, h0, dl] = pltpu.roll(t, 8 - dl, 0) if dl else t
                for dl in range(8):
                    r = d3 * 256 + dl * 32 + h1 * 16
                    top, bot = (jnp.concatenate([blk[d4, 0, dl], blk[d4, 1, dl]], axis=0) for d4 in range(2))
                    put_sums(wo, slice(r, r + 16), 0, (top[:, :512], top[:, 512:], bot[:, :512], bot[:, 512:]))

    def prep_w1(c):
        es = []
        for t in (2 * c, 2 * c + 1):
            for r in range(0, 512, 64):
                blocks = [w1_raw[rr:rr + 64, _tile(j)].astype(f32) for rr in (r, 512 + r) for j in (t, t + 14)]
                put_sums(w1, slice(r, r + 64), t, blocks)
                if c == 0:
                    e = _tree(jnp.add, [y * y for y in blocks])
                    es.append(_tree(jnp.add, [e[a:a + 8] for a in range(0, 64, 8)]))
        if c == 0:
            tot = jnp.sum(jnp.sum(_tree(jnp.add, es), axis=1, keepdims=True), axis=0, keepdims=True)
            stat[0:1, :] = jnp.broadcast_to(tot * (1.0 / 512), (1, 128))
            bb = b1[0:1, :]
            stat[1:2, :] = jnp.broadcast_to(jnp.sum(bb * bb, axis=1, keepdims=True) * (1.0 / F) + TINY, (1, 128))

    def prep_w2():
        for t in range(4):
            for r in range(0, HF, 64):
                put_sums(w2, slice(r, r + 64), t,
                         [w2_raw[rr:rr + 64, _tile(j)].astype(f32) for rr in (r, HF + r) for j in (t, t + 4)])

    def cvt_x(lo, hi):
        for r in range(lo, hi, 64):
            val = xin[r:r + 64, :].astype(f32)
            x[r:r + 64, :] = val
        return _tree(jnp.add, [val[a:a + 8, 0:128] for a in range(0, 64, 8)])

    def dma(src, dst, i):
        if MODE == "body":
            return None
        return pltpu.make_async_copy(src, dst, isem.at[i])

    def cols2(src, dst, lo, hi, i):
        return [dma(src.at[:, pl.ds(s * HF + lo, hi - lo)], dst.at[:, pl.ds(s * HF + lo, hi - lo)], i + s)
                for s in range(2)]

    NQ = 512 // RC0
    cp_x = [dma(x_hbm.at[pl.ds(lo, n), :], xin.at[pl.ds(lo, n), :], i)
            for i, (lo, n) in enumerate(((0, TM), (TM, TM), (2 * TM, 2 * TM)))]
    cp_kv = [dma(wqkv_hbm.at[:, pl.ds(g * D, D)], wqkv_raw.at[:, pl.ds(g * D, D)], 2 + g) for g in (1, 2)]
    cp_wo = dma(wo_hbm, wo_raw, 5)
    cp_w2 = dma(w2_hbm, w2_raw, 6)
    cp_w1a = cols2(w1_hbm, w1_raw, 0, 256 * NPRE, 7)
    cp_w1b = cols2(w1_hbm, w1_raw, 256 * NPRE, HF, 9)
    cp_q = [[dma(wqkv_hbm.at[pl.ds(r, RCQ), pl.ds(0, D)], wqkv_raw.at[pl.ds(r, RCQ), pl.ds(0, D)], 11 + 2 * n + s)
             for s, r in enumerate((n * RCQ, 512 + n * RCQ))] for n in range(512 // RCQ)]

    def step(t, peeled):
        base = (t % NT) * TM
        pbase = ((t + NT - 1) % NT) * TM
        nbase = ((t + 1) % NT) * TM
        slot = t % 2
        first = t % NT == 0
        clock[0] = 0
        two = lambda f, *a: [f(*a, c) for c in range(2)]
        qk_items = [P(qk8, r, first) for r in range(0, TM, 8)]
        ln1_items = [P(ln1, nbase, 16, r) for r in range(0, HM, 16)]
        if peeled:
            for cp in [cp_x[0], *sum(cp_q, []), *cp_kv, cp_wo, cp_x[1], *cp_w1a, *cp_w1b, cp_w2, cp_x[2]]:
                cp.start()
            wv[0:HALO, :] = jnp.zeros((HALO, 128), f32)
            k[:, 0:HALO, :] = jnp.zeros((8, HALO, 128), f32)
            b1[0:1, :] = b1_ref[...].astype(f32)
            b2[0:1, :] = b2_ref[...].astype(f32)
            ostage[slot, 1] = jnp.zeros((HM, D), bf16)
            cp_x[0].wait()
            cvt_x(0, TM)
            for r in range(0, HM, RCL):
                ln1(base, RCL, r)
            for n, cps in enumerate(cp_q):
                for cp in cps:
                    cp.wait()
                prep_qkv(0, RC0, n * RCQ, (n + 1) * RCQ)
            plan(QKF, qk_items)
            plan(L1F, ln1_items)
            two(qkv_p1, 0)
            cp_kv[0].wait()
            prep_qkv(1, RC1, 0, 512)
            two(qkv_p2, 0)
            two(qkv_p1, 1)
            cp_kv[1].wait()
            cp_wo.wait()
            prep_qkv(2, RC1, 0, 512)
            prep_wo()
        else:
            plan(QK, qk_items)
            plan(L1, ln1_items)
            two(qkv_p1, 0)
            two(qkv_p1, 1)
            two(qkv_p2, 0)
        two(qkv_p2, 1)
        two(qkv_p1, 2)
        v_first(first)
        two(qkv_p2, 2)
        flush(L1[0] - 8000)
        for half in range(2):
            for r in range(0, HM, 16):
                pv16(half, r)
        if not peeled:
            w2_p2(pbase, slot, 0)
        two(wo_p1, base)
        halo_save()
        if peeled:
            for cp in [cp_x[1], *cp_w1a]:
                cp.wait()
            cvt_x(TM, 2 * TM)
            for c in range(NPRE):
                prep_w1(c)
        two(wo_p2, base)
        two(wo_p3, base)
        if not peeled:
            w2_p2(pbase, slot, 1)
        for r in range(0, HM, 16):
            ln2(0, r)
        if peeled:
            for cp in cp_w1b:
                cp.wait()
            for c in range(NPRE, 7):
                prep_w1(c)
        for r in range(0, HM, 16):
            ln2(1, r)
        for c in range(NPRE):
            w1_pre(c)
        for c in range(7):
            if peeled and c == CB:
                flush(1e9)
                cp_w2.wait()
                cp_x[2].wait()
                prep_w2()
                plan((clock[0] + 9000, clock[0] + 22000), [P(cvt_x, r, r + 64) for r in range(2 * TM, S, 64)])
            w1_chunk(c)
        two(w2_p1, base, slot)
        flush(1e9)

    scope = jax.named_scope if SCOPES else (lambda n: contextlib.nullcontext())
    if MODE != "body":
        with scope("first"):
            step(0, True)

    def copies(t):
        return out_copy(t % 2, 0, t), out_copy(t % 2, 1, t + NT - 1)

    def body(t, c):
        for cp in copies(t - 1):
            cp.start()
        with scope("body"):
            step(t, False)
        for cp in copies(t - 1):
            cp.wait()
        return c

    last = 2 * NT - 1
    if MODE != "first":
        lax.fori_loop(1, 2 * NT, body, 0)
    for cp in copies(last):
        cp.start()
    for c in range(2):
        w2_p2(S - TM, 0, c)
    for cp in copies(last):
        cp.wait()
    out_copy(0, 1, last).start()
    out_copy(0, 1, last).wait()


@jax.jit
def pallas_interleave_layers__sliding_local_dilated__dense_activation_squared_relu__prompt_kernel(A_x, A_wqkv, A_wo, B_x, B_w1, B_b1, B_w2, B_b2):
    del B_x
    any_spec = pl.BlockSpec(memory_space=pl.ANY)
    vmem_spec = pl.BlockSpec(memory_space=pltpu.VMEM)
    V = pltpu.VMEM
    out = pl.pallas_call(
        _kernel,
        in_specs=[pl.BlockSpec(memory_space=pltpu.SMEM), any_spec, any_spec, any_spec, any_spec, vmem_spec, any_spec, vmem_spec],
        out_specs=any_spec,
        out_shape=jax.ShapeDtypeStruct((S, D), bf16),
        scratch_shapes=[
            V((2, 2, HM, D), bf16), V((S, D), bf16), V((S, D), f32),
            V((D, 3 * D), bf16), V((D, D), bf16), V((D, F), bf16), V((F, D), bf16),
            V((7, 12, 512, 128), bf16), V((7, 4, 512, 128), bf16), V((7, 14, 512, 128), bf16), V((7, 4, HF, 128), bf16),
            V((7, 4, HM, 128), bf16), V((7, 4, HM, 128), bf16), V((7, 4, HM, 128), bf16), V((7, 14, HM, 128), bf16),
            V((8, HM, 128), f32), V((8, HM, 128), f32), V((8, TM + HALO, 128), f32), V((8, TM + HALO, 128), f32),
            V((TM + HALO, 128), f32), V((8, HM, 128), f32), V((8, HM, 128), f32),
            V((HM, D), f32), V((TM, D), f32), V((3, HM, 512), f32), V((2, HM, 256 * max(NPRE, 1)), f32), V((3, HM, 512), f32),
            V((HM, 128), f32), V((HM, 128), f32), V((HM, 128), f32), V((HM, 128), f32),
            V((TM, 128), f32), V((TM, 128), f32), V((TM, 128), f32), V((TM, 128), f32),
            V((TM, 128), f32), V((TM, 128), f32), V((TM, 128), f32),
            V((8, F), f32), V((8, D), f32), V((8, 128), f32),
            pltpu.SemaphoreType.DMA((19,)), pltpu.SemaphoreType.DMA((2,)),
        ],
        compiler_params=pltpu.CompilerParams(vmem_limit_bytes=127 * 1024 * 1024),
    )(np.zeros((3,), np.int32), A_x.reshape(S, D), A_wqkv, A_wo, B_w1, B_b1.reshape(1, F), B_w2, B_b2.reshape(1, D))
    return out.reshape(1, S, D)
```

```python
import functools

import jax
import jax.numpy as jnp
import numpy as np
from jax import lax
import jax.experimental.pallas as pl
import jax.experimental.pallas.tpu as pltpu

S, D, F = 2048, 1024, 3584
DH, W, DIL = 32, 8, 2
TM = 512
HM = TM // 2
HF = F // 2
NT = S // TM
HALO = 16
EPS = 1e-5
TINY = 1e-30
QSCALE = float(DH ** -0.5 * np.log2(np.e))
NEG = float(-1e9 * np.log2(np.e))
NPRE = 4
RQ = 256
QK = (10900, 21500)
QKF = (14000, 21400)
L1 = (42000, 60000)
MODE = "all"
f32, bf16, u32, i32 = jnp.float32, jnp.bfloat16, jnp.uint32, jnp.int32
P = functools.partial


def _tree(op, xs):
    xs = list(xs)
    while len(xs) > 1:
        xs = [op(xs[i], xs[i + 1]) if i + 1 < len(xs) else xs[i] for i in range(0, len(xs), 2)]
    return xs[0]


def _a_sums(a11, a12, a21, a22):
    return (a11 + a22, a21 + a22, a11, a22, a11 + a12, a21 - a11, a12 - a22)


def _b_sums(b11, b12, b21, b22):
    return (b11 + b22, b11, b12 - b22, b21 - b11, b22, b11 + b12, b21 + b22)


M1, M2, M3, M4, M5, M6, M7 = range(7)


def _tile(j, n=1):
    return slice(j * 128, (j + n) * 128)


def _pow2(s):
    return pltpu.bitcast((pltpu.bitcast(s, i32) + 0x007FFFFF) & 0x7F800000, f32)


def _pow2_inv(s):
    return pltpu.bitcast(0x7F000000 - pltpu.bitcast(s, i32), f32)


def _skew_select(ts, index, unit):
    ts = [ts[-i % 8] for i in range(8)]
    for b in (1, 2, 4):
        take = (index & (unit * b)) != 0
        ts = [jnp.where(take, ts[(i - b) % 8], ts[i]) for i in range(8)]
    return ts


def _kernel(x_hbm, wqkv_hbm, wo_hbm, w1_hbm, b1_ref, w2_hbm, b2_ref, out_hbm,
            ostage, xin, x, wqkv_raw, wo_raw, w1_raw, w2_raw,
            wq, wo, w1, w2, xs1, xs2, os_, hs, q, k, v, pr, ua, xt, part, pre, carry,
            s1, sq, sv, so, sg, gh, sh, b1, b2, stat, isem, osem):
    sub = lax.broadcasted_iota(i32, (8, 128), 0)

    clock = [0]
    queue = []

    def plan(window, items):
        lo, hi = window
        queue.extend((lo + (hi - lo) * (n + 1) / len(items), f) for n, f in enumerate(items))
        queue.sort(key=lambda e: e[0])

    def flush(until):
        vals = []
        while queue and queue[0][0] <= until:
            vals.append(queue.pop(0)[1]())
        return vals

    def tie(operand, r, until):
        vals = flush(until)
        if not vals:
            return operand
        d = _tree(jnp.add, vals)
        d = jnp.concatenate([d, d], axis=0).astype(bf16)
        never = jnp.broadcast_to(jnp.abs(b2[0:1, 0:128]), (16, 128)).astype(bf16) < 0
        parts = [operand[:r], jnp.where(never, d, operand[r:r + 16]), operand[r + 16:]]
        return jnp.concatenate([p for p in parts if p.shape[0]], axis=0)

    def mm(a_ref, w_ref, i, c):
        kt = a_ref.shape[1]
        ls = [a_ref[i, t] for t in range(kt)]
        rs = [w_ref[i, 2 * c + n] for n in range(2)]
        t0 = clock[0]
        clock[0] = t0 + 128 * kt
        if kt == 4:
            out = []
            for n in range(2):
                l0 = ls[0]
                for r in range(0, HM, 64):
                    l0 = tie(l0, r, t0 + n * 256 + r + 63)
                out.append(jnp.dot(jnp.concatenate([l0] + ls[1:], axis=1), rs[n], preferred_element_type=f32))
            return jnp.concatenate(out, axis=1)
        for g in range(kt // 4 + 1):
            for r in range(0, HM, 64):
                ls[4 * g] = tie(ls[4 * g], r, t0 + g * 448 + r + 63)
        return jnp.dot(jnp.concatenate(ls, axis=1), jnp.concatenate(rs, axis=1), preferred_element_type=f32)

    def put(dst, i, t0, rows, val):
        for t in range(val.shape[1] // 128):
            dst[i, t0 + t, rows, :] = val[:, _tile(t)].astype(bf16)

    def put_a(dst, r, ua_):
        ua[r:r + 16, :] = ua_
        put(dst, M3, 0, slice(r, r + 16), ua_[:, :512])
        put(dst, M5, 0, slice(r, r + 16), ua_[:, :512] + ua_[:, 512:])

    def put_b(dst, r, ub):
        ss = _a_sums(ua[r:r + 16, :512], ua[r:r + 16, 512:], ub[:, :512], ub[:, 512:])
        for i in (M1, M2, M4, M6, M7):
            put(dst, i, 0, slice(r, r + 16), ss[i])

    def ln(xv):
        z = xv - jnp.sum(xv, axis=1, keepdims=True) * (1.0 / D)
        var = jnp.sum(z * z, axis=1, keepdims=True) * (1.0 / D)
        vt = jnp.maximum(var, TINY)
        g = lax.rsqrt(vt)
        s = lax.rsqrt(var + EPS) * (vt * g)
        return z * g, jnp.broadcast_to(s, (xv.shape[0], 128))

    def ln1(base, n, r):
        ua_, sa = ln(x[pl.ds(pl.multiple_of(base + r, n), n), :])
        ub, sb = ln(x[pl.ds(pl.multiple_of(base + HM + r, n), n), :])
        for i, val in enumerate(_a_sums(ua_[:, :512], ua_[:, 512:], ub[:, :512], ub[:, 512:])):
            put(xs1, i, 0, slice(r, r + n), val)
        for r0, s in ((r, sa), (HM + r, sb)):
            s1[r0:r0 + n, :] = s
            sq[r0:r0 + n, :] = s * QSCALE
            sv[HALO + r0:HALO + r0 + n, :] = _pow2(s)
        return (sa + sb)[0:8]

    def ln2(half, r):
        rows = slice(half * HM + r, half * HM + r + 16)
        u, s = ln(xt[rows, :])
        (put_b if half else put_a)(xs2, r, u)
        p = s * s * stat[0:1, :] + stat[1:2, :]
        g = lax.rsqrt(p)
        gh[rows, :] = g
        sg[rows, :] = s * g
        sh[rows, :] = p

    def qkv_dst(g, j, half):
        if g == 0:
            return q.at[j, pl.ds(half * HM, HM), :]
        return (k, v)[g - 1].at[j, pl.ds(HALO + half * HM, HM), :]

    def qkv_p1(g, c):
        sc = (sq if g == 0 else s1)[0:HM, :]
        sc = jnp.concatenate([sc, sc], axis=1)
        md = P(mm, xs1, wq, c=g * 2 + c)

        def out(j, half, val):
            for t in range(2):
                qkv_dst(g, c * 2 + j + t, half)[...] = val[:, _tile(t)]
        m3 = md(M3)
        m5 = md(M5)
        out(4, 0, (m3 + m5) * sc)
        m1 = md(M1)
        out(4, 1, m1 + m3)
        acc = m1 - m5
        m4 = md(M4)
        out(0, 1, m4)
        out(0, 0, (acc + m4 + md(M7)) * sc)

    def qkv_p2(g, c):
        sc = (sq if g == 0 else s1)[HM:TM, :]
        m2 = mm(xs1, wq, M2, g * 2 + c)
        acc = []
        for t in range(2):
            l, r = qkv_dst(g, c * 2 + t, 1), qkv_dst(g, c * 2 + t + 4, 1)
            l[...] = (l[...] + m2[:, _tile(t)]) * sc
            acc.append(r[...] - m2[:, _tile(t)])
        m6 = mm(xs1, wq, M6, g * 2 + c)
        for t in range(2):
            qkv_dst(g, c * 2 + t + 4, 1)[...] = (acc[t] + m6[:, _tile(t)]) * sc

    def window(ref, lead, r):
        return [ref[lead + (pl.ds(HALO + r - DIL * w, 8), slice(None))] for w in range(W)]

    def qk8(r, first):
        qs = [q[j, r:r + 8, :] for j in range(8)]
        ks = [window(k, (j,), r) for j in range(8)]
        ls = []
        for w in range(W):
            p = _tree(jnp.add, [qs[j] * ks[j][w] for j in range(8)])
            p = (p + pltpu.roll(p, 64, 1)) + (pltpu.roll(p, 32, 1) + pltpu.roll(p, 96, 1))
            if r - DIL * w < 0:
                p = jnp.where(jnp.logical_and(first, sub + (r - DIL * w) < 0), NEG, p)
            ls.append(p)
        m = _tree(jnp.maximum, ls)
        es = [jnp.exp2(l - m) for l in ls]
        sc = _tree(jnp.maximum, window(sv, (), r))
        so[r:r + 8, :] = sc
        inv = _pow2_inv(sc) / _tree(jnp.add, es)
        for w in range(W):
            pr[w, r:r + 8, :] = es[w] * inv
        return inv

    def pv8(r):
        ps = [pr[w, r:r + 8, :] for w in range(W)]
        return jnp.concatenate(
            [_tree(jnp.add, [a * b for a, b in zip(ps, window(v, (j,), r))]) for j in range(8)], axis=1)

    def pv16(half, r):
        r0 = half * HM + r
        (put_b if half else put_a)(os_, r, jnp.concatenate([pv8(r0), pv8(r0 + 8)], axis=0))

    def v_first(first):
        for j in range(8):
            v0 = jnp.broadcast_to(v[j, HALO:HALO + 1, :], (HALO, 128))
            v[j, 0:HALO, :] = jnp.where(first, v0, v[j, 0:HALO, :])

    def halo_save():
        sv[0:HALO, :] = sv[TM:TM + HALO, :]
        for j in range(8):
            k[j, 0:HALO, :] = k[j, TM:TM + HALO, :]
            v[j, 0:HALO, :] = v[j, TM:TM + HALO, :]

    def acc_x(base, half, j, val):
        rows = pl.ds(pl.multiple_of(base + half * HM, HM), HM)
        sc = so[half * HM:(half + 1) * HM, :]
        for t in range(2):
            r = x[rows, _tile(j + t)] + val[:, _tile(t)] * sc
            xt[half * HM:(half + 1) * HM, _tile(j + t)] = r
            if half:
                x[rows, _tile(j + t)] = r

    def wo_p1(base, c):
        cols = _tile(c * 2, 2)
        m3 = mm(os_, wo, M3, c)
        part[2, :, cols] = m3
        m5 = mm(os_, wo, M5, c)
        part[0, :, cols] = m5
        acc_x(base, 0, 4 + c * 2, m3 + m5)

    def wo_p2(base, c):
        cols = _tile(c * 2, 2)
        m1 = mm(os_, wo, M1, c)
        part[2, :, cols] = part[2, :, cols] + m1
        acc = m1 - part[0, :, cols]
        m4 = mm(os_, wo, M4, c)
        part[1, :, cols] = m4
        acc_x(base, 0, c * 2, acc + m4 + mm(os_, wo, M7, c))

    def wo_p3(base, c):
        cols = _tile(c * 2, 2)
        m2 = mm(os_, wo, M2, c)
        acc_x(base, 1, c * 2, part[1, :, cols] + m2)
        acc = part[2, :, cols] - m2
        acc_x(base, 1, 4 + c * 2, acc + mm(os_, wo, M6, c))

    def w1_pre(c):
        pre[0, :, _tile(c * 2, 2)] = mm(xs2, w1, M3, c)
        pre[1, :, _tile(c * 2, 2)] = mm(xs2, w1, M5, c)

    def w1_chunk(c):
        md = P(mm, xs2, w1, c=c)

        def act(z, half, side):
            rows = slice(half * HM, (half + 1) * HM)
            out = []
            for t in range(2):
                b = b1[0:1, _tile(side * 14 + c * 2 + t)]
                y = jnp.maximum(z[:, _tile(t)] * sg[rows, :] + gh[rows, :] * b, 0.0)
                out.append(y * y)
            return jnp.concatenate(out, axis=1)

        def out(i, val):
            put(hs, i, c * 2, slice(0, HM), val)
        if c < NPRE:
            m3, m5 = pre[0, :, _tile(c * 2, 2)], pre[1, :, _tile(c * 2, 2)]
        else:
            m3, m5 = md(M3), md(M5)
        h12 = act(m3 + m5, 0, 1)
        m4 = md(M4)
        acc1 = m4 - m5
        m2 = md(M2)
        h21 = act(m4 + m2, 1, 0)
        acc2 = m3 - m2
        m1 = md(M1)
        acc1, acc2 = acc1 + m1, acc2 + m1
        h22 = act(acc2 + md(M6), 1, 1)
        out(M2, h21 + h22)
        out(M4, h22)
        out(M7, h12 - h22)
        h11 = act(acc1 + md(M7), 0, 0)
        out(M1, h11 + h22)
        out(M3, h11)
        out(M5, h11 + h12)
        out(M6, h21 - h11)

    def fin(res, base, slot, half, c, side, val, sc):
        rows = pl.ds(pl.multiple_of(base + half * HM, HM), HM)
        for t in range(2):
            cols = _tile(side * 4 + c * 2 + t)
            r = res(rows, cols) + val[:, _tile(t)] * sc + b2[0:1, cols]
            x[rows, cols] = r
            ostage[slot, half, :, cols] = r.astype(bf16)

    def w2_p1(base, slot, c):
        done = P(fin, lambda rows, cols: xt[0:HM, cols], base, slot, 0, c, sc=sh[0:HM, :])
        m3 = mm(hs, w2, M3, c)
        m5 = mm(hs, w2, M5, c)
        done(1, m3 + m5)
        m1 = mm(hs, w2, M1, c)
        carry[1, :, _tile(2 * c, 2)] = m1 + m3
        acc = m1 - m5
        m4 = mm(hs, w2, M4, c)
        carry[0, :, _tile(2 * c, 2)] = m4
        done(0, acc + m4 + mm(hs, w2, M7, c))
        if c == 1:
            carry[2, :, 0:128] = sh[HM:TM, :]

    def w2_p2(base, slot, c):
        done = P(fin, lambda rows, cols: x[rows, cols], base, slot, 1, c, sc=carry[2, :, 0:128])
        m2 = mm(hs, w2, M2, c)
        done(0, carry[0, :, _tile(2 * c, 2)] + m2)
        acc = carry[1, :, _tile(2 * c, 2)] - m2
        done(1, acc + mm(hs, w2, M6, c))

    def put_sums(dst, rows, t, blocks):
        for i, s in enumerate(_b_sums(*blocks)):
            put(dst, i, t, rows, s)

    def permuted(r, n, g):
        lane = lax.broadcasted_iota(i32, (n // 2, 128), 1)
        src = ((lane & 31) << 2) | (lane >> 5)
        ts = [pltpu.bitcast(wqkv_raw[r:r + n, _tile(g * 8 + j)], u32) for j in range(8)]
        ts = [pltpu.roll(t, 4 * j, 1) if j else t for j, t in enumerate(ts)]
        ts = _skew_select(ts, lane, 4)
        return [pltpu.bitcast(jnp.take_along_axis(t, (src + 4 * j) & 127, axis=1), bf16).astype(f32)
                for j, t in enumerate(ts)]

    def prep_qkv(g, n, lo, hi):
        for r in range(lo, hi, n):
            top, bot = permuted(r, n, g), permuted(512 + r, n, g)
            for t in range(4):
                put_sums(wq, slice(r, r + n), g * 4 + t, (top[t], top[t + 4], bot[t], bot[t + 4]))

    def prep_wo():
        index = lax.broadcasted_iota(i32, (8, D), 0)
        for d3 in range(2):
            for h1 in range(2):
                blk = {}
                for d4 in range(2):
                    for h0 in range(2):
                        src = []
                        for hh in range(8):
                            r = hh * 128 + h1 * 64 + h0 * 32 + d4 * 16
                            t = wo_raw[r:r + 16, :].astype(f32)[8 * d3:8 * d3 + 8]
                            src.append(pltpu.roll(t, hh, 0) if hh else t)
                        for dl, t in enumerate(_skew_select(src, index, 1)):
                            blk[d4, h0, dl] = pltpu.roll(t, 8 - dl, 0) if dl else t
                for dl in range(8):
                    r = d3 * 256 + dl * 32 + h1 * 16
                    top, bot = (jnp.concatenate([blk[d4, 0, dl], blk[d4, 1, dl]], axis=0) for d4 in range(2))
                    put_sums(wo, slice(r, r + 16), 0, (top[:, :512], top[:, 512:], bot[:, :512], bot[:, 512:]))

    def prep_w1(c):
        es = []
        for t in (2 * c, 2 * c + 1):
            for r in range(0, 512, 64):
                blocks = [w1_raw[rr:rr + 64, _tile(j)].astype(f32) for rr in (r, 512 + r) for j in (t, t + 14)]
                put_sums(w1, slice(r, r + 64), t, blocks)
                if c == 0:
                    e = _tree(jnp.add, [y * y for y in blocks])
                    es.append(_tree(jnp.add, [e[a:a + 8] for a in range(0, 64, 8)]))
        if c == 0:
            tot = jnp.sum(jnp.sum(_tree(jnp.add, es), axis=1, keepdims=True), axis=0, keepdims=True)
            stat[0:1, :] = jnp.broadcast_to(tot * (1.0 / 512), (1, 128))
            bb = b1[0:1, :]
            stat[1:2, :] = jnp.broadcast_to(jnp.sum(bb * bb, axis=1, keepdims=True) * (1.0 / F) + TINY, (1, 128))

    def prep_w2():
        for t in range(4):
            for r in range(0, HF, 64):
                put_sums(w2, slice(r, r + 64), t,
                         [w2_raw[rr:rr + 64, _tile(j)].astype(f32) for rr in (r, HF + r) for j in (t, t + 4)])

    def cvt_x(r):
        val = xin[r:r + 64, :].astype(f32)
        x[r:r + 64, :] = val
        return _tree(jnp.add, [val[a:a + 8, 0:128] for a in range(0, 64, 8)])

    def dma(src, dst, block, i):
        return pltpu.make_async_copy(src.at[block], dst.at[block], isem.at[i])

    full = slice(None)
    cp_x0 = dma(x_hbm, xin, (pl.ds(0, TM), full), 0)
    cp_x1 = dma(x_hbm, xin, (pl.ds(TM, S - TM), full), 1)
    cp_k, cp_v = (dma(wqkv_hbm, wqkv_raw, (full, pl.ds(g * D, D)), 1 + g) for g in (1, 2))
    cp_wo = dma(wo_hbm, wo_raw, (full, full), 4)
    cp_w2 = dma(w2_hbm, w2_raw, (full, full), 5)
    cp_w1a = [dma(w1_hbm, w1_raw, (full, pl.ds(s * HF, 256 * NPRE)), 6 + s) for s in range(2)]
    cp_w1b = [dma(w1_hbm, w1_raw, (full, pl.ds(s * HF + 256 * NPRE, HF - 256 * NPRE)), 8 + s) for s in range(2)]
    cp_q = [[dma(wqkv_hbm, wqkv_raw, (pl.ds(s * 512 + n * RQ, RQ), pl.ds(0, D)), 10 + 2 * n + s) for s in range(2)]
            for n in range(512 // RQ)]

    def step(t, peeled):
        base = (t % NT) * TM
        pbase = ((t + NT - 1) % NT) * TM
        nbase = ((t + 1) % NT) * TM
        slot = t % 2
        first = t % NT == 0
        clock[0] = 0
        qk_items = [P(qk8, r, first) for r in range(0, TM, 8)]
        ln1_items = [P(ln1, nbase, 16, r) for r in range(0, HM, 16)]

        def two(f, *a):
            for c in range(2):
                f(*a, c)
        if peeled:
            for cp in [cp_x0, *sum(cp_q, []), cp_k, cp_v, cp_wo, *cp_w1a, *cp_w1b, cp_w2, cp_x1]:
                cp.start()
            sv[0:HALO, :] = jnp.zeros((HALO, 128), f32)
            k[:, 0:HALO, :] = jnp.zeros((8, HALO, 128), f32)
            b1[0:1, :] = b1_ref[...].astype(f32).reshape(1, F)
            b2[0:1, :] = b2_ref[...].astype(f32).reshape(1, D)
            ostage[slot, 1] = jnp.zeros((HM, D), bf16)
            cp_x0.wait()
            for r in range(0, TM, 64):
                cvt_x(r)
            for r in range(0, HM, 128):
                ln1(base, 128, r)
            for n, cps in enumerate(cp_q):
                for cp in cps:
                    cp.wait()
                prep_qkv(0, 128, n * RQ, (n + 1) * RQ)
            plan(QKF, qk_items)
            qkv_p1(0, 0)
            cp_k.wait()
            prep_qkv(1, 128, 0, 512)
            qkv_p1(0, 1)
            two(qkv_p2, 0)
            cp_v.wait()
            cp_wo.wait()
            prep_qkv(2, 128, 0, 512)
            prep_wo()
            two(qkv_p1, 1)
        else:
            plan(QK, qk_items)
            plan(L1, ln1_items)
            two(qkv_p1, 0)
            two(qkv_p1, 1)
            two(qkv_p2, 0)
        two(qkv_p2, 1)
        two(qkv_p1, 2)
        v_first(first)
        two(qkv_p2, 2)
        flush(QK[1])
        for half in range(2):
            for r in range(0, HM, 16):
                pv16(half, r)
        if not peeled:
            w2_p2(pbase, slot, 0)
        two(wo_p1, base)
        halo_save()
        if peeled:
            for cp in cp_w1a:
                cp.wait()
            for c in range(NPRE):
                prep_w1(c)
        two(wo_p2, base)
        two(wo_p3, base)
        if not peeled:
            w2_p2(pbase, slot, 1)
        for half in range(2):
            for r in range(0, HM, 16):
                ln2(half, r)
        for c in range(NPRE):
            w1_pre(c)
        for c in range(7):
            if peeled and c == NPRE:
                for cp in [*cp_w1b, cp_w2, cp_x1]:
                    cp.wait()
                for cc in range(NPRE, 7):
                    prep_w1(cc)
                for r in range(TM, 2 * TM, 64):
                    cvt_x(r)
                plan((clock[0] + 2000, clock[0] + 12000), ln1_items)
                plan((clock[0] + 14000, clock[0] + 27000), [P(cvt_x, r) for r in range(2 * TM, S, 64)])
                prep_w2()
            w1_chunk(c)
        two(w2_p1, base, slot)
        flush(float("inf"))

    def out_copies(t):
        return [pltpu.make_async_copy(
            ostage.at[t % 2, half],
            out_hbm.at[pl.ds(pl.multiple_of(((t + (NT - 1) * half) % NT) * TM + half * HM, HM), HM), :],
            osem.at[half]) for half in range(2)]

    if MODE != "body":
        step(0, True)

    def body(t, c):
        cps = out_copies(t - 1)
        for cp in cps:
            cp.start()
        step(t, False)
        for cp in cps:
            cp.wait()
        return c

    if MODE != "first":
        lax.fori_loop(1, 2 * NT, body, 0)
    cps = out_copies(2 * NT - 1)
    for cp in cps:
        cp.start()
    for c in range(2):
        w2_p2(S - TM, 0, c)
    for cp in cps:
        cp.wait()
    last = out_copies(2 * NT)[1]
    last.start()
    last.wait()


@jax.jit
def pallas_interleave_layers__sliding_local_dilated__dense_activation_squared_relu__prompt_kernel(A_x, A_wqkv, A_wo, B_x, B_w1, B_b1, B_w2, B_b2):
    del B_x
    hbm = pl.BlockSpec(memory_space=pl.ANY)
    vmem = pl.BlockSpec(memory_space=pltpu.VMEM)
    V = pltpu.VMEM
    out = pl.pallas_call(
        _kernel,
        in_specs=[hbm, hbm, hbm, hbm, vmem, hbm, vmem],
        out_specs=hbm,
        out_shape=jax.ShapeDtypeStruct((S, D), bf16),
        scratch_shapes=[
            V((2, 2, HM, D), bf16), V((S, D), bf16), V((S, D), f32),
            V((D, 3 * D), bf16), V((D, D), bf16), V((D, F), bf16), V((F, D), bf16),
            V((7, 12, 512, 128), bf16), V((7, 4, 512, 128), bf16),
            V((7, 14, 512, 128), bf16), V((7, 4, HF, 128), bf16),
            V((7, 4, HM, 128), bf16), V((7, 4, HM, 128), bf16), V((7, 4, HM, 128), bf16), V((7, 14, HM, 128), bf16),
            V((8, TM, 128), f32), V((8, TM + HALO, 128), f32), V((8, TM + HALO, 128), f32), V((W, TM, 128), f32),
            V((HM, D), f32), V((TM, D), f32),
            V((3, HM, 512), f32), V((2, HM, 256 * NPRE), f32), V((3, HM, 512), f32),
            V((TM, 128), f32), V((TM, 128), f32), V((TM + HALO, 128), f32), V((TM, 128), f32),
            V((TM, 128), f32), V((TM, 128), f32), V((TM, 128), f32),
            V((8, F), f32), V((8, D), f32), V((8, 128), f32),
            pltpu.SemaphoreType.DMA((10 + 1024 // RQ,)), pltpu.SemaphoreType.DMA((2,)),
        ],
        compiler_params=pltpu.CompilerParams(vmem_limit_bytes=127 * 1024 * 1024),
    )(A_x.reshape(S, D), A_wqkv, A_wo, B_w1, B_b1, B_w2, B_b2)
    return out.reshape(1, S, D)
```

```python
import functools

import jax
import jax.numpy as jnp
import numpy as np
from jax import lax
import jax.experimental.pallas as pl
import jax.experimental.pallas.tpu as pltpu

S, D, F = 2048, 1024, 3584
DH, W, DIL = 32, 8, 2
TM = 512
HM = TM // 2
HF = F // 2
NT = S // TM
HALO = 16
EPS = 1e-5
TINY = 1e-30
QSCALE = float(DH ** -0.5 * np.log2(np.e))
NEG = float(-1e9 * np.log2(np.e))
NPRE = 4
RQ = 256
QK = (10900, 21500)
QKF = (14000, 21400)
L1 = (42000, 60000)
MODE = "all"
CH = 2
LAG = 0
CHF = 0
CQF = 0
CP = 0
THREE = 1
CQ = 2
TQ = 1
C1 = 0
f32, bf16, u32, i32 = jnp.float32, jnp.bfloat16, jnp.uint32, jnp.int32
P = functools.partial


def _tree(op, xs):
    xs = list(xs)
    while len(xs) > 1:
        xs = [op(xs[i], xs[i + 1]) if i + 1 < len(xs) else xs[i] for i in range(0, len(xs), 2)]
    return xs[0]


def _a_sums(a11, a12, a21, a22):
    return (a11 + a22, a21 + a22, a11, a22, a11 + a12, a21 - a11, a12 - a22)


def _b_sums(b11, b12, b21, b22):
    return (b11 + b22, b11, b12 - b22, b21 - b11, b22, b11 + b12, b21 + b22)


M1, M2, M3, M4, M5, M6, M7 = range(7)


def _tile(j, n=1):
    return slice(j * 128, (j + n) * 128)


def _pow2(s):
    return pltpu.bitcast((pltpu.bitcast(s, i32) + 0x007FFFFF) & 0x7F800000, f32)


def _pow2_inv(s):
    return pltpu.bitcast(0x7F000000 - pltpu.bitcast(s, i32), f32)


def _pow2_sqrt(s):
    half = lax.shift_right_logical(pltpu.bitcast(s, i32), 1)
    return pltpu.bitcast((half + 0x1FC00000) & 0x7F800000, f32)


def _skew_select(ts, index, unit):
    ts = [ts[-i % 8] for i in range(8)]
    for b in (1, 2, 4):
        take = (index & (unit * b)) != 0
        ts = [jnp.where(take, ts[(i - b) % 8], ts[i]) for i in range(8)]
    return ts


def _kernel(x_hbm, wqkv_hbm, wo_hbm, w1_hbm, b1_ref, w2_hbm, b2_ref, out_hbm,
            ostage, xin, x, wqkv_raw, wo_raw, w1_raw, w2_raw,
            wq, wo, w1, w2, xs1, xs2, os_, hs, q, k, v, pr, ua, xt, part, pre, carry,
            s1, sq, sv, so, sg, gh, sh, b1, b2, stat, isem, osem):
    sub = lax.broadcasted_iota(i32, (8, 128), 0)

    clock = [0]
    queue = []

    def plan(window, items):
        lo, hi = window
        queue.extend((lo + (hi - lo) * (n + 1) / len(items), f) for n, f in enumerate(items))
        queue.sort(key=lambda e: e[0])

    def flush(until):
        vals = []
        while queue and queue[0][0] <= until:
            vals.append(queue.pop(0)[1]())
        return vals

    def tie(operand, r, until):
        vals = flush(until)
        if not vals:
            return operand
        d = _tree(jnp.add, vals)
        d = jnp.concatenate([d, d], axis=0).astype(bf16)
        never = jnp.broadcast_to(jnp.abs(b2[0:1, 0:128]), (16, 128)).astype(bf16) < 0
        parts = [operand[:r], jnp.where(never, d, operand[r:r + 16]), operand[r + 16:]]
        return jnp.concatenate([p for p in parts if p.shape[0]], axis=0)

    last = {}
    opt = {}

    def after(key, val):
        if key not in last:
            return val
        never = jnp.broadcast_to(jnp.abs(b2[0:1, 0:128]), val.shape) < 0
        return jnp.where(never, last[key], val)

    def mm(a_ref, w_ref, i, c):
        kt = a_ref.shape[1]
        ls = [a_ref[i, t] for t in range(kt)]
        rs = [w_ref[i, 2 * c + n] for n in range(2)]
        t0 = clock[0]
        clock[0] = t0 + 128 * kt
        if kt == 4:
            out = []
            for n in range(2):
                l0 = ls[0]
                for r in range(0, HM, 64):
                    l0 = tie(l0, r, t0 + n * 256 + r + 63)
                out.append(jnp.dot(jnp.concatenate([l0] + ls[1:], axis=1), rs[n], preferred_element_type=f32))
            return jnp.concatenate(out, axis=1)
        for g in range(kt // 4 + 1):
            for r in range(0, HM, 64):
                ls[4 * g] = tie(ls[4 * g], r, t0 + g * 448 + r + 63)
        return jnp.dot(jnp.concatenate(ls, axis=1), jnp.concatenate(rs, axis=1), preferred_element_type=f32)

    def put(dst, i, t0, rows, val):
        for t in range(val.shape[1] // 128):
            dst[i, t0 + t, rows, :] = val[:, _tile(t)].astype(bf16)

    def put_a(dst, r, ua_):
        ua[r:r + 16, :] = ua_
        put(dst, M3, 0, slice(r, r + 16), ua_[:, :512])
        s5 = ua_[:, :512] + ua_[:, 512:]
        put(dst, M5, 0, slice(r, r + 16), s5)
        return [s5]

    def put_b(dst, r, ub):
        ss = _a_sums(ua[r:r + 16, :512], ua[r:r + 16, 512:], ub[:, :512], ub[:, 512:])
        for i in (M1, M2, M4, M6, M7):
            put(dst, i, 0, slice(r, r + 16), ss[i])
        return [ss[i] for i in (M1, M2, M6, M7)]

    def ln(xv, key=None):
        if key:
            xv = jnp.concatenate([after(key, xv[:, :128]), xv[:, 128:]], axis=1)
        mean = jnp.sum(xv, axis=1, keepdims=True) * (1.0 / D)
        z = xv - mean
        var = jnp.sum(z * z, axis=1, keepdims=True) * (1.0 / D)
        if key:
            last[key] = jnp.broadcast_to(mean if abs(CH) == 1 else var, (xv.shape[0], 128))
        var = jnp.broadcast_to(var, (xv.shape[0], 128))
        size = _pow2_sqrt(jnp.maximum(var, TINY))
        g = _pow2_inv(size)
        u = jnp.concatenate([z[:, _tile(j)] * g for j in range(8)], axis=1)
        return u, lax.rsqrt(var + EPS) * size

    def ln1(base, n, r):
        ua_, sa = ln(x[pl.ds(pl.multiple_of(base + r, n), n), :])
        ub, sb = ln(x[pl.ds(pl.multiple_of(base + HM + r, n), n), :])
        for i, val in enumerate(_a_sums(ua_[:, :512], ua_[:, 512:], ub[:, :512], ub[:, 512:])):
            put(xs1, i, 0, slice(r, r + n), val)
        for r0, s in ((r, sa), (HM + r, sb)):
            s1[r0:r0 + n, :] = s
            sq[r0:r0 + n, :] = s * QSCALE
            sv[HALO + r0:HALO + r0 + n, :] = _pow2(s)
        return (sa + sb)[0:8]

    def ln2(half, r):
        rows = slice(half * HM + r, half * HM + r + 16)
        xv = xt[rows, :]
        xv = jnp.concatenate([xv[:, :128], after(('full', half * HM // 16 + r // 16), xv[:, 128:256]), xv[:, 256:]], axis=1)
        u, s = ln(xv, ('ln2' + ('' if CH > 0 else str(half))) if opt['ch'] else None)
        outs = (put_b if half else put_a)(xs2, r, u)
        if LAG:
            bits = [pltpu.bitcast(o[:, _tile(t)], i32) for o in outs for t in range(4)]
            last['full', half * HM // 16 + r // 16 + LAG] = pltpu.bitcast(_tree(jnp.bitwise_or, bits), f32)
        p = s * s * stat[0:1, :] + stat[1:2, :]
        size = _pow2_sqrt(p)
        g = _pow2_inv(size)
        gh[rows, :] = g
        sg[rows, :] = s * g
        sh[rows, :] = size * size

    def qkv_dst(g, j, half):
        if g == 0:
            return q.at[j, pl.ds(half * HM, HM), :]
        return (k, v)[g - 1].at[j, pl.ds(HALO + half * HM, HM), :]

    def qkv_p1(g, c):
        sc = (sq if g == 0 else s1)[0:HM, :]
        sc = jnp.concatenate([sc, sc], axis=1)
        md = P(mm, xs1, wq, c=g * 2 + c)

        def out(j, half, val):
            for t in range(2):
                qkv_dst(g, c * 2 + j + t, half)[...] = val[:, _tile(t)]
        m3 = md(M3)
        m5 = md(M5)
        out(4, 0, (m3 + m5) * sc)
        m1 = md(M1)
        out(4, 1, m1 + m3)
        acc = m1 - m5
        m4 = md(M4)
        out(0, 1, m4)
        out(0, 0, (acc + m4 + md(M7)) * sc)

    def qkv_p2(g, c):
        sc = (sq if g == 0 else s1)[HM:TM, :]
        m2 = mm(xs1, wq, M2, g * 2 + c)
        acc = []
        for t in range(2):
            l, r = qkv_dst(g, c * 2 + t, 1), qkv_dst(g, c * 2 + t + 4, 1)
            l[...] = (l[...] + m2[:, _tile(t)]) * sc
            acc.append(r[...] - m2[:, _tile(t)])
        m6 = mm(xs1, wq, M6, g * 2 + c)
        for t in range(2):
            qkv_dst(g, c * 2 + t + 4, 1)[...] = (acc[t] + m6[:, _tile(t)]) * sc

    def window(ref, lead, r):
        return [ref[lead + (pl.ds(HALO + r - DIL * w, 8), slice(None))] for w in range(W)]

    def qk8(r, first):
        qs = [q[j, r:r + 8, :] for j in range(8)]
        CQ = opt['cq']
        if CQ == 3:
            qs = [after('qk2', t) for t in qs]
        elif CQ:
            qs = [after('qk', t) for t in qs] if CQ == 2 else [after('qk', qs[0])] + qs[1:]
        ks = [window(k, (j,), r) for j in range(8)]
        ls = []
        for w in range(W):
            p = _tree(jnp.add, [qs[j] * ks[j][w] for j in range(8)])
            if w == 0 and CQ == 3:
                last['qk2'] = pltpu.roll(p, 64, 1)
            if THREE:
                p = (p + pltpu.roll(p, 64, 1)) + (pltpu.roll(p, 32, 1) + pltpu.roll(p, 96, 1))
            else:
                p = p + pltpu.roll(p, 64, 1)
                p = p + pltpu.roll(p, 32, 1)
            if r - DIL * w < 0:
                p = jnp.where(jnp.logical_and(first, sub + (r - DIL * w) < 0), NEG, p)
            ls.append(p)
            if w == 0:
                last['qk'] = p
        m = _tree(jnp.maximum, ls)
        es = [jnp.exp2(l - m) for l in ls]
        sc = _tree(jnp.maximum, window(sv, (), r))
        so[r:r + 8, :] = sc
        den = _tree(jnp.add, es)
        inv = pltpu.reciprocal(den, approx=True)
        inv = inv * (2.0 - den * inv) * _pow2_inv(sc)
        for w in range(W):
            pr[w, r:r + 8, :] = es[w] * inv
        return inv

    def pv8(r):
        ps = [pr[w, r:r + 8, :] for w in range(W)]
        if CP:
            ps = [after('pv', t) for t in ps]
        outs = [_tree(jnp.add, [a * b for a, b in zip(ps, window(v, (j,), r))]) for j in range(8)]
        if CP and r % CP == 0:
            last['pv'] = outs[7]
        return jnp.concatenate(outs, axis=1)

    def pv16(half, r):
        r0 = half * HM + r
        (put_b if half else put_a)(os_, r, jnp.concatenate([pv8(r0), pv8(r0 + 8)], axis=0))

    def v_first(first):
        for j in range(8):
            v0 = jnp.broadcast_to(v[j, HALO:HALO + 1, :], (HALO, 128))
            v[j, 0:HALO, :] = jnp.where(first, v0, v[j, 0:HALO, :])

    def halo_save():
        sv[0:HALO, :] = sv[TM:TM + HALO, :]
        for j in range(8):
            k[j, 0:HALO, :] = k[j, TM:TM + HALO, :]
            v[j, 0:HALO, :] = v[j, TM:TM + HALO, :]

    def acc_x(base, half, j, val):
        rows = pl.ds(pl.multiple_of(base + half * HM, HM), HM)
        sc = so[half * HM:(half + 1) * HM, :]
        for t in range(2):
            r = x[rows, _tile(j + t)] + val[:, _tile(t)] * sc
            xt[half * HM:(half + 1) * HM, _tile(j + t)] = r
            if half:
                x[rows, _tile(j + t)] = r

    def wo_p1(base, c):
        cols = _tile(c * 2, 2)
        m3 = mm(os_, wo, M3, c)
        part[2, :, cols] = m3
        m5 = mm(os_, wo, M5, c)
        part[0, :, cols] = m5
        acc_x(base, 0, 4 + c * 2, m3 + m5)

    def wo_p2(base, c):
        cols = _tile(c * 2, 2)
        m1 = mm(os_, wo, M1, c)
        part[2, :, cols] = part[2, :, cols] + m1
        acc = m1 - part[0, :, cols]
        m4 = mm(os_, wo, M4, c)
        part[1, :, cols] = m4
        acc_x(base, 0, c * 2, acc + m4 + mm(os_, wo, M7, c))

    def wo_p3(base, c):
        cols = _tile(c * 2, 2)
        m2 = mm(os_, wo, M2, c)
        acc_x(base, 1, c * 2, part[1, :, cols] + m2)
        acc = part[2, :, cols] - m2
        acc_x(base, 1, 4 + c * 2, acc + mm(os_, wo, M6, c))

    def w1_pre(c):
        pre[0, :, _tile(c * 2, 2)] = mm(xs2, w1, M3, c)
        pre[1, :, _tile(c * 2, 2)] = mm(xs2, w1, M5, c)

    def w1_chunk(c):
        md = P(mm, xs2, w1, c=c)

        def act(z, half, side):
            rows = slice(half * HM, (half + 1) * HM)
            out = []
            for t in range(2):
                b = b1[0:1, _tile(side * 14 + c * 2 + t)]
                y = jnp.maximum(z[:, _tile(t)] * sg[rows, :] + gh[rows, :] * b, 0.0)
                out.append(y * y)
            return jnp.concatenate(out, axis=1)

        def out(i, val):
            put(hs, i, c * 2, slice(0, HM), val)
        if c < NPRE:
            m3, m5 = pre[0, :, _tile(c * 2, 2)], pre[1, :, _tile(c * 2, 2)]
        else:
            m3, m5 = md(M3), md(M5)
        h12 = act(m3 + m5, 0, 1)
        m4 = md(M4)
        acc1 = m4 - m5
        m2 = md(M2)
        h21 = act(m4 + m2, 1, 0)
        acc2 = m3 - m2
        m1 = md(M1)
        acc1, acc2 = acc1 + m1, acc2 + m1
        h22 = act(acc2 + md(M6), 1, 1)
        out(M2, h21 + h22)
        out(M4, h22)
        out(M7, h12 - h22)
        h11 = act(acc1 + md(M7), 0, 0)
        out(M1, h11 + h22)
        out(M3, h11)
        out(M5, h11 + h12)
        out(M6, h21 - h11)

    def fin(res, base, slot, half, c, side, val, sc):
        rows = pl.ds(pl.multiple_of(base + half * HM, HM), HM)
        for t in range(2):
            cols = _tile(side * 4 + c * 2 + t)
            r = res(rows, cols) + val[:, _tile(t)] * sc + b2[0:1, cols]
            x[rows, cols] = r
            ostage[slot, half, :, cols] = r.astype(bf16)

    def w2_p1(base, slot, c):
        done = P(fin, lambda rows, cols: xt[0:HM, cols], base, slot, 0, c, sc=sh[0:HM, :])
        m3 = mm(hs, w2, M3, c)
        m5 = mm(hs, w2, M5, c)
        done(1, m3 + m5)
        m1 = mm(hs, w2, M1, c)
        carry[1, :, _tile(2 * c, 2)] = m1 + m3
        acc = m1 - m5
        m4 = mm(hs, w2, M4, c)
        carry[0, :, _tile(2 * c, 2)] = m4
        done(0, acc + m4 + mm(hs, w2, M7, c))
        if c == 1:
            carry[2, :, 0:128] = sh[HM:TM, :]

    def w2_p2(base, slot, c):
        done = P(fin, lambda rows, cols: x[rows, cols], base, slot, 1, c, sc=carry[2, :, 0:128])
        m2 = mm(hs, w2, M2, c)
        done(0, carry[0, :, _tile(2 * c, 2)] + m2)
        acc = carry[1, :, _tile(2 * c, 2)] - m2
        done(1, acc + mm(hs, w2, M6, c))

    def put_sums(dst, rows, t, blocks):
        for i, s in enumerate(_b_sums(*blocks)):
            put(dst, i, t, rows, s)

    def permuted(r, n, g):
        lane = lax.broadcasted_iota(i32, (n // 2, 128), 1)
        src = ((lane & 31) << 2) | (lane >> 5)
        ts = [pltpu.bitcast(wqkv_raw[r:r + n, _tile(g * 8 + j)], u32) for j in range(8)]
        ts = [pltpu.roll(t, 4 * j, 1) if j else t for j, t in enumerate(ts)]
        ts = _skew_select(ts, lane, 4)
        return [pltpu.bitcast(jnp.take_along_axis(t, (src + 4 * j) & 127, axis=1), bf16).astype(f32)
                for j, t in enumerate(ts)]

    def prep_qkv(g, n, lo, hi):
        for r in range(lo, hi, n):
            top, bot = permuted(r, n, g), permuted(512 + r, n, g)
            for t in range(4):
                put_sums(wq, slice(r, r + n), g * 4 + t, (top[t], top[t + 4], bot[t], bot[t + 4]))

    def prep_wo():
        index = lax.broadcasted_iota(i32, (8, D), 0)
        for d3 in range(2):
            for h1 in range(2):
                blk = {}
                for d4 in range(2):
                    for h0 in range(2):
                        src = []
                        for hh in range(8):
                            r = hh * 128 + h1 * 64 + h0 * 32 + d4 * 16
                            t = wo_raw[r:r + 16, :].astype(f32)[8 * d3:8 * d3 + 8]
                            src.append(pltpu.roll(t, hh, 0) if hh else t)
                        for dl, t in enumerate(_skew_select(src, index, 1)):
                            blk[d4, h0, dl] = pltpu.roll(t, 8 - dl, 0) if dl else t
                for dl in range(8):
                    r = d3 * 256 + dl * 32 + h1 * 16
                    top, bot = (jnp.concatenate([blk[d4, 0, dl], blk[d4, 1, dl]], axis=0) for d4 in range(2))
                    put_sums(wo, slice(r, r + 16), 0, (top[:, :512], top[:, 512:], bot[:, :512], bot[:, 512:]))

    def prep_w1(c):
        es = []
        for t in (2 * c, 2 * c + 1):
            for r in range(0, 512, 64):
                blocks = [w1_raw[rr:rr + 64, _tile(j)].astype(f32) for rr in (r, 512 + r) for j in (t, t + 14)]
                put_sums(w1, slice(r, r + 64), t, blocks)
                if c == 0:
                    e = _tree(jnp.add, [y * y for y in blocks])
                    es.append(_tree(jnp.add, [e[a:a + 8] for a in range(0, 64, 8)]))
        if c == 0:
            tot = jnp.sum(jnp.sum(_tree(jnp.add, es), axis=1, keepdims=True), axis=0, keepdims=True)
            stat[0:1, :] = jnp.broadcast_to(tot * (1.0 / 512), (1, 128))
            bb = b1[0:1, :]
            stat[1:2, :] = jnp.broadcast_to(jnp.sum(bb * bb, axis=1, keepdims=True) * (1.0 / F) + TINY, (1, 128))

    def prep_w2():
        for t in range(4):
            for r in range(0, HF, 64):
                put_sums(w2, slice(r, r + 64), t,
                         [w2_raw[rr:rr + 64, _tile(j)].astype(f32) for rr in (r, HF + r) for j in (t, t + 4)])

    def cvt_x(r):
        val = xin[r:r + 64, :].astype(f32)
        x[r:r + 64, :] = val
        return _tree(jnp.add, [val[a:a + 8, 0:128] for a in range(0, 64, 8)])

    def dma(src, dst, block, i):
        return pltpu.make_async_copy(src.at[block], dst.at[block], isem.at[i])

    full = slice(None)
    cp_x0 = dma(x_hbm, xin, (pl.ds(0, TM), full), 0)
    cp_x1 = dma(x_hbm, xin, (pl.ds(TM, S - TM), full), 1)
    cp_k, cp_v = (dma(wqkv_hbm, wqkv_raw, (full, pl.ds(g * D, D)), 1 + g) for g in (1, 2))
    cp_wo = dma(wo_hbm, wo_raw, (full, full), 4)
    cp_w2 = dma(w2_hbm, w2_raw, (full, full), 5)
    cp_w1a = [dma(w1_hbm, w1_raw, (full, pl.ds(s * HF, 256 * NPRE)), 6 + s) for s in range(2)]
    cp_w1b = [dma(w1_hbm, w1_raw, (full, pl.ds(s * HF + 256 * NPRE, HF - 256 * NPRE)), 8 + s) for s in range(2)]
    cp_q = [[dma(wqkv_hbm, wqkv_raw, (pl.ds(s * 512 + n * RQ, RQ), pl.ds(0, D)), 10 + 2 * n + s) for s in range(2)]
            for n in range(512 // RQ)]

    def step(t, peeled):
        base = (t % NT) * TM
        pbase = ((t + NT - 1) % NT) * TM
        nbase = ((t + 1) % NT) * TM
        slot = t % 2
        first = t % NT == 0
        clock[0] = 0
        last.clear()
        opt.update(ch=CHF if peeled else CH, cq=CQF if peeled else CQ)
        qk_items = [P(qk8, r, first) for r in range(0, TM, 8)]
        ln1_items = [P(ln1, nbase, 16, r) for r in range(0, HM, 16)]

        def two(f, *a):
            for c in range(2):
                f(*a, c)
        if peeled:
            for cp in [cp_x0, *sum(cp_q, []), cp_k, cp_v, cp_wo, *cp_w1a, *cp_w1b, cp_w2, cp_x1]:
                cp.start()
            sv[0:HALO, :] = jnp.zeros((HALO, 128), f32)
            k[:, 0:HALO, :] = jnp.zeros((8, HALO, 128), f32)
            b1[0:1, :] = b1_ref[...].astype(f32).reshape(1, F)
            b2[0:1, :] = b2_ref[...].astype(f32).reshape(1, D)
            ostage[slot, 1] = jnp.zeros((HM, D), bf16)
            cp_x0.wait()
            for r in range(0, TM, 64):
                cvt_x(r)
            for r in range(0, HM, 128):
                ln1(base, 128, r)
            for n, cps in enumerate(cp_q):
                for cp in cps:
                    cp.wait()
                prep_qkv(0, 128, n * RQ, (n + 1) * RQ)
            plan(QKF, qk_items)
            qkv_p1(0, 0)
            cp_k.wait()
            prep_qkv(1, 128, 0, 512)
            qkv_p1(0, 1)
            two(qkv_p2, 0)
            cp_v.wait()
            cp_wo.wait()
            prep_qkv(2, 128, 0, 512)
            prep_wo()
            two(qkv_p1, 1)
        else:
            plan(QK if TQ else (QK[1], QK[1]), qk_items)
            plan(L1, ln1_items)
            two(qkv_p1, 0)
            two(qkv_p1, 1)
            two(qkv_p2, 0)
        two(qkv_p2, 1)
        two(qkv_p1, 2)
        v_first(first)
        two(qkv_p2, 2)
        flush(QK[1])
        for half in range(2):
            for r in range(0, HM, 16):
                pv16(half, r)
        if not peeled:
            w2_p2(pbase, slot, 0)
        two(wo_p1, base)
        halo_save()
        if peeled:
            for cp in cp_w1a:
                cp.wait()
            for c in range(NPRE):
                prep_w1(c)
        two(wo_p2, base)
        two(wo_p3, base)
        if not peeled:
            w2_p2(pbase, slot, 1)
        for half in range(2):
            for r in range(0, HM, 16):
                ln2(half, r)
        for c in range(NPRE):
            w1_pre(c)
        for c in range(7):
            if peeled and c == NPRE:
                for cp in [*cp_w1b, cp_w2, cp_x1]:
                    cp.wait()
                for cc in range(NPRE, 7):
                    prep_w1(cc)
                for r in range(TM, 2 * TM, 64):
                    cvt_x(r)
                plan((clock[0] + 2000, clock[0] + 12000), ln1_items)
                plan((clock[0] + 14000, clock[0] + 27000), [P(cvt_x, r) for r in range(2 * TM, S, 64)])
                prep_w2()
            w1_chunk(c)
        two(w2_p1, base, slot)
        flush(float("inf"))

    def out_copies(t):
        return [pltpu.make_async_copy(
            ostage.at[t % 2, half],
            out_hbm.at[pl.ds(pl.multiple_of(((t + (NT - 1) * half) % NT) * TM + half * HM, HM), HM), :],
            osem.at[half]) for half in range(2)]

    if MODE != "body":
        step(0, True)

    def body(t, c):
        cps = out_copies(t - 1)
        for cp in cps:
            cp.start()
        step(t, False)
        for cp in cps:
            cp.wait()
        return c

    if MODE != "first":
        lax.fori_loop(1, 2 * NT, body, 0)
    cps = out_copies(2 * NT - 1)
    for cp in cps:
        cp.start()
    for c in range(2):
        w2_p2(S - TM, 0, c)
    for cp in cps:
        cp.wait()
    last = out_copies(2 * NT)[1]
    last.start()
    last.wait()


@jax.jit
def pallas_interleave_layers__sliding_local_dilated__dense_activation_squared_relu__prompt_kernel(A_x, A_wqkv, A_wo, B_x, B_w1, B_b1, B_w2, B_b2):
    del B_x
    hbm = pl.BlockSpec(memory_space=pl.ANY)
    vmem = pl.BlockSpec(memory_space=pltpu.VMEM)
    V = pltpu.VMEM
    out = pl.pallas_call(
        _kernel,
        in_specs=[hbm, hbm, hbm, hbm, vmem, hbm, vmem],
        out_specs=hbm,
        out_shape=jax.ShapeDtypeStruct((S, D), bf16),
        scratch_shapes=[
            V((2, 2, HM, D), bf16), V((S, D), bf16), V((S, D), f32),
            V((D, 3 * D), bf16), V((D, D), bf16), V((D, F), bf16), V((F, D), bf16),
            V((7, 12, 512, 128), bf16), V((7, 4, 512, 128), bf16),
            V((7, 14, 512, 128), bf16), V((7, 4, HF, 128), bf16),
            V((7, 4, HM, 128), bf16), V((7, 4, HM, 128), bf16), V((7, 4, HM, 128), bf16), V((7, 14, HM, 128), bf16),
            V((8, TM, 128), f32), V((8, TM + HALO, 128), f32), V((8, TM + HALO, 128), f32), V((W, TM, 128), f32),
            V((HM, D), f32), V((TM, D), f32),
            V((3, HM, 512), f32), V((2, HM, 256 * NPRE), f32), V((3, HM, 512), f32),
            V((TM, 128), f32), V((TM, 128), f32), V((TM + HALO, 128), f32), V((TM, 128), f32),
            V((TM, 128), f32), V((TM, 128), f32), V((TM, 128), f32),
            V((8, F), f32), V((8, D), f32), V((8, 128), f32),
            pltpu.SemaphoreType.DMA((10 + 1024 // RQ,)), pltpu.SemaphoreType.DMA((2,)),
        ],
        compiler_params=pltpu.CompilerParams(vmem_limit_bytes=127 * 1024 * 1024),
    )(A_x.reshape(S, D), A_wqkv, A_wo, B_w1, B_b1, B_w2, B_b2)
    return out.reshape(1, S, D)
```

```python
import functools

import jax
import jax.numpy as jnp
import numpy as np
from jax import lax
import jax.experimental.pallas as pl
import jax.experimental.pallas.tpu as pltpu

S, D, F = 2048, 1024, 3584
DH, W, DIL = 32, 8, 2
TM = 512
HM = TM // 2
HF = F // 2
NT = S // TM
HALO = 16
EPS = 1e-5
TINY = 1e-30
QSCALE = float(DH ** -0.5 * np.log2(np.e))
NEG = float(-1e9 * np.log2(np.e))
NPRE = 4
RQ = 256
QK = (10900, 21500)
QKF = (14000, 21400)
L1 = (42000, 58000)
MODE = "all"
CH = 2
LAG = 0
CHF = 0
CQF = 0
CP = 0
THREE = 1
VB = 1
XF = 1
CQ = 2
TQ = 1
C1 = 0
f32, bf16, u32, i32 = jnp.float32, jnp.bfloat16, jnp.uint32, jnp.int32
P = functools.partial


def _tree(op, xs):
    xs = list(xs)
    while len(xs) > 1:
        xs = [op(xs[i], xs[i + 1]) if i + 1 < len(xs) else xs[i] for i in range(0, len(xs), 2)]
    return xs[0]


def _a_sums(a11, a12, a21, a22):
    return (a11 + a22, a21 + a22, a11, a22, a11 + a12, a21 - a11, a12 - a22)


def _b_sums(b11, b12, b21, b22):
    return (b11 + b22, b11, b12 - b22, b21 - b11, b22, b11 + b12, b21 + b22)


M1, M2, M3, M4, M5, M6, M7 = range(7)


def _tile(j, n=1):
    return slice(j * 128, (j + n) * 128)


def _pow2(s):
    return pltpu.bitcast((pltpu.bitcast(s, i32) + 0x007FFFFF) & 0x7F800000, f32)


def _pow2_inv(s):
    return pltpu.bitcast(0x7F000000 - pltpu.bitcast(s, i32), f32)


def _pow2_sqrt(s):
    half = lax.shift_right_logical(pltpu.bitcast(s, i32), 1)
    return pltpu.bitcast((half + 0x1FC00000) & 0x7F800000, f32)


def _skew_select(ts, index, unit):
    ts = [ts[-i % 8] for i in range(8)]
    for b in (1, 2, 4):
        take = (index & (unit * b)) != 0
        ts = [jnp.where(take, ts[(i - b) % 8], ts[i]) for i in range(8)]
    return ts


def _kernel(x_hbm, wqkv_hbm, wo_hbm, w1_hbm, b1_ref, w2_hbm, b2_ref, out_hbm,
            ostage, xin, x, wqkv_raw, wo_raw, w1_raw, w2_raw,
            wq, wo, w1, w2, xs1, xs2, os_, hs, q, k, v, pr, ua, xt, part, pre, carry,
            s1, sq, sv, so, sg, gh, sh, b1, b2, stat, isem, osem):
    sub = lax.broadcasted_iota(i32, (8, 128), 0)

    clock = [0]
    queue = []

    def plan(window, items):
        lo, hi = window
        queue.extend((lo + (hi - lo) * (n + 1) / len(items), f) for n, f in enumerate(items))
        queue.sort(key=lambda e: e[0])

    def flush(until):
        vals = []
        while queue and queue[0][0] <= until:
            vals.append(queue.pop(0)[1]())
        return vals

    def tie(operand, r, until):
        vals = flush(until)
        if not vals:
            return operand
        d = _tree(jnp.add, vals)
        d = jnp.concatenate([d, d], axis=0).astype(bf16)
        never = jnp.broadcast_to(jnp.abs(b2[0:1, 0:128]), (16, 128)).astype(bf16) < 0
        parts = [operand[:r], jnp.where(never, d, operand[r:r + 16]), operand[r + 16:]]
        return jnp.concatenate([p for p in parts if p.shape[0]], axis=0)

    last = {}
    opt = {}

    def after(key, val):
        if key not in last:
            return val
        never = jnp.broadcast_to(jnp.abs(b2[0:1, 0:128]), val.shape) < 0
        return jnp.where(never, last[key], val)

    def mm(a_ref, w_ref, i, c):
        kt = a_ref.shape[1]
        ls = [a_ref[i, t] for t in range(kt)]
        rs = [w_ref[i, 2 * c + n] for n in range(2)]
        t0 = clock[0]
        clock[0] = t0 + 128 * kt
        if kt == 4:
            out = []
            for n in range(2):
                l0 = ls[0]
                for r in range(0, HM, 64):
                    l0 = tie(l0, r, t0 + n * 256 + r + 63)
                out.append(jnp.dot(jnp.concatenate([l0] + ls[1:], axis=1), rs[n], preferred_element_type=f32))
            return jnp.concatenate(out, axis=1)
        for g in range(kt // 4 + 1):
            for r in range(0, HM, 64):
                ls[4 * g] = tie(ls[4 * g], r, t0 + g * 448 + r + 63)
        return jnp.dot(jnp.concatenate(ls, axis=1), jnp.concatenate(rs, axis=1), preferred_element_type=f32)

    def put(dst, i, t0, rows, val):
        for t in range(val.shape[1] // 128):
            dst[i, t0 + t, rows, :] = val[:, _tile(t)].astype(bf16)

    def put_a(dst, r, ua_):
        ua[r:r + 16, :] = ua_
        put(dst, M3, 0, slice(r, r + 16), ua_[:, :512])
        s5 = ua_[:, :512] + ua_[:, 512:]
        put(dst, M5, 0, slice(r, r + 16), s5)
        return [s5]

    def put_b(dst, r, ub):
        ss = _a_sums(ua[r:r + 16, :512], ua[r:r + 16, 512:], ub[:, :512], ub[:, 512:])
        for i in (M1, M2, M4, M6, M7):
            put(dst, i, 0, slice(r, r + 16), ss[i])
        return [ss[i] for i in (M1, M2, M6, M7)]

    def ln(xv, key=None):
        if key:
            xv = jnp.concatenate([after(key, xv[:, :128]), xv[:, 128:]], axis=1)
        mean = jnp.sum(xv, axis=1, keepdims=True) * (1.0 / D)
        z = xv - mean
        var = jnp.sum(z * z, axis=1, keepdims=True) * (1.0 / D)
        if key:
            last[key] = jnp.broadcast_to(mean if abs(CH) == 1 else var, (xv.shape[0], 128))
        var = jnp.broadcast_to(var, (xv.shape[0], 128))
        size = _pow2_sqrt(jnp.maximum(var, TINY))
        g = _pow2_inv(size)
        u = jnp.concatenate([z[:, _tile(j)] * g for j in range(8)], axis=1)
        return u, lax.rsqrt(var + EPS) * size

    def ln1(base, n, r):
        ua_, sa = ln(x[pl.ds(pl.multiple_of(base + r, n), n), :])
        ub, sb = ln(x[pl.ds(pl.multiple_of(base + HM + r, n), n), :])
        for i, val in enumerate(_a_sums(ua_[:, :512], ua_[:, 512:], ub[:, :512], ub[:, 512:])):
            put(xs1, i, 0, slice(r, r + n), val)
        for r0, s in ((r, sa), (HM + r, sb)):
            s1[r0:r0 + n, :] = s
            sq[r0:r0 + n, :] = s * QSCALE
            sv[HALO + r0:HALO + r0 + n, :] = _pow2(s)
        return (sa + sb)[0:8]

    def ln2(half, r):
        rows = slice(half * HM + r, half * HM + r + 16)
        xv = xt[rows, :]
        xv = jnp.concatenate([xv[:, :128], after(('full', half * HM // 16 + r // 16), xv[:, 128:256]), xv[:, 256:]], axis=1)
        u, s = ln(xv, ('ln2' + ('' if CH > 0 else str(half))) if opt['ch'] else None)
        outs = (put_b if half else put_a)(xs2, r, u)
        if LAG:
            bits = [pltpu.bitcast(o[:, _tile(t)], i32) for o in outs for t in range(4)]
            last['full', half * HM // 16 + r // 16 + LAG] = pltpu.bitcast(_tree(jnp.bitwise_or, bits), f32)
        p = s * s * stat[0:1, :] + stat[1:2, :]
        size = _pow2_sqrt(p)
        g = _pow2_inv(size)
        gh[rows, :] = g
        sg[rows, :] = s * g
        sh[rows, :] = size * size

    def qkv_dst(g, j, half):
        if g == 0:
            return q.at[j, pl.ds(half * HM, HM), :]
        return (k, v)[g - 1].at[j, pl.ds(HALO + half * HM, HM), :]

    def qkv_p1(g, c):
        sc = (sq if g == 0 else s1)[0:HM, :]
        sc = jnp.concatenate([sc, sc], axis=1)
        md = P(mm, xs1, wq, c=g * 2 + c)

        def out(j, half, val):
            for t in range(2):
                qkv_dst(g, c * 2 + j + t, half)[...] = val[:, _tile(t)]
        m3 = md(M3)
        m5 = md(M5)
        out(4, 0, (m3 + m5) * sc)
        m1 = md(M1)
        out(4, 1, m1 + m3)
        acc = m1 - m5
        m4 = md(M4)
        out(0, 1, m4)
        out(0, 0, (acc + m4 + md(M7)) * sc)

    def qkv_p2(g, c):
        sc = (sq if g == 0 else s1)[HM:TM, :]
        m2 = mm(xs1, wq, M2, g * 2 + c)
        acc = []
        for t in range(2):
            l, r = qkv_dst(g, c * 2 + t, 1), qkv_dst(g, c * 2 + t + 4, 1)
            l[...] = (l[...] + m2[:, _tile(t)]) * sc
            acc.append(r[...] - m2[:, _tile(t)])
        m6 = mm(xs1, wq, M6, g * 2 + c)
        for t in range(2):
            qkv_dst(g, c * 2 + t + 4, 1)[...] = (acc[t] + m6[:, _tile(t)]) * sc

    def window(ref, lead, r):
        return [ref[lead + (pl.ds(HALO + r - DIL * w, 8), slice(None))] for w in range(W)]

    def qk8(r, first):
        qs = [q[j, r:r + 8, :] for j in range(8)]
        CQ = opt['cq']
        if CQ == 3:
            qs = [after('qk2', t) for t in qs]
        elif CQ:
            qs = [after('qk', t) for t in qs] if CQ == 2 else [after('qk', qs[0])] + qs[1:]
        ks = [window(k, (j,), r) for j in range(8)]
        ls = []
        for w in range(W):
            p = _tree(jnp.add, [qs[j] * ks[j][w] for j in range(8)])
            if w == 0 and CQ == 3:
                last['qk2'] = pltpu.roll(p, 64, 1)
            if THREE:
                p = (p + pltpu.roll(p, 64, 1)) + (pltpu.roll(p, 32, 1) + pltpu.roll(p, 96, 1))
            else:
                p = p + pltpu.roll(p, 64, 1)
                p = p + pltpu.roll(p, 32, 1)
            if r - DIL * w < 0:
                p = jnp.where(jnp.logical_and(first, sub + (r - DIL * w) < 0), NEG, p)
            ls.append(p)
            if w == 0:
                last['qk'] = p
        m = _tree(jnp.maximum, ls)
        es = [jnp.exp2(l - m) for l in ls]
        sc = _tree(jnp.maximum, window(sv, (), r))
        so[r:r + 8, :] = sc
        den = _tree(jnp.add, es)
        inv = pltpu.reciprocal(den, approx=True)
        inv = inv * (2.0 - den * inv) * _pow2_inv(sc)
        for w in range(W):
            pr[w, r:r + 8, :] = es[w] * inv
        return inv

    def pv8(r):
        ps = [pr[w, r:r + 8, :] for w in range(W)]
        if CP:
            ps = [after('pv', t) for t in ps]
        outs = [_tree(jnp.add, [a * b for a, b in zip(ps, window(v, (j,), r))]) for j in range(8)]
        if CP and r % CP == 0:
            last['pv'] = outs[7]
        return jnp.concatenate(outs, axis=1)

    def pv16(half, r):
        r0 = half * HM + r
        (put_b if half else put_a)(os_, r, jnp.concatenate([pv8(r0), pv8(r0 + 8)], axis=0))

    def v_first(first):
        for j in range(8):
            v0 = jnp.broadcast_to(v[j, HALO:HALO + 1, :], (HALO, 128))
            v[j, 0:HALO, :] = jnp.where(first, v0, v[j, 0:HALO, :])

    def halo_save():
        sv[0:HALO, :] = sv[TM:TM + HALO, :]
        for j in range(8):
            k[j, 0:HALO, :] = k[j, TM:TM + HALO, :]
            v[j, 0:HALO, :] = v[j, TM:TM + HALO, :]

    def acc_x(base, half, j, val):
        rows = pl.ds(pl.multiple_of(base + half * HM, HM), HM)
        sc = so[half * HM:(half + 1) * HM, :]
        for t in range(2):
            r = x[rows, _tile(j + t)] + val[:, _tile(t)] * sc
            xt[half * HM:(half + 1) * HM, _tile(j + t)] = r
            if half:
                x[rows, _tile(j + t)] = r

    def wo_p1(base, c):
        cols = _tile(c * 2, 2)
        m3 = mm(os_, wo, M3, c)
        part[2, :, cols] = m3
        m5 = mm(os_, wo, M5, c)
        part[0, :, cols] = m5
        acc_x(base, 0, 4 + c * 2, m3 + m5)

    def wo_p2(base, c):
        cols = _tile(c * 2, 2)
        m1 = mm(os_, wo, M1, c)
        part[2, :, cols] = part[2, :, cols] + m1
        acc = m1 - part[0, :, cols]
        m4 = mm(os_, wo, M4, c)
        part[1, :, cols] = m4
        acc_x(base, 0, c * 2, acc + m4 + mm(os_, wo, M7, c))

    def wo_p3(base, c):
        cols = _tile(c * 2, 2)
        m2 = mm(os_, wo, M2, c)
        acc_x(base, 1, c * 2, part[1, :, cols] + m2)
        acc = part[2, :, cols] - m2
        acc_x(base, 1, 4 + c * 2, acc + mm(os_, wo, M6, c))

    def w1_pre(c):
        pre[0, :, _tile(c * 2, 2)] = mm(xs2, w1, M3, c)
        pre[1, :, _tile(c * 2, 2)] = mm(xs2, w1, M5, c)

    def w1_chunk(c):
        md = P(mm, xs2, w1, c=c)

        def act(z, half, side):
            rows = slice(half * HM, (half + 1) * HM)
            out = []
            for t in range(2):
                b = b1[0:1, _tile(side * 14 + c * 2 + t)]
                y = jnp.maximum(z[:, _tile(t)] * sg[rows, :] + gh[rows, :] * b, 0.0)
                out.append(y * y)
            return jnp.concatenate(out, axis=1)

        def out(i, val):
            put(hs, i, c * 2, slice(0, HM), val)
        if c < NPRE:
            m3, m5 = pre[0, :, _tile(c * 2, 2)], pre[1, :, _tile(c * 2, 2)]
        else:
            m3, m5 = md(M3), md(M5)
        h12 = act(m3 + m5, 0, 1)
        m4 = md(M4)
        acc1 = m4 - m5
        m2 = md(M2)
        h21 = act(m4 + m2, 1, 0)
        acc2 = m3 - m2
        m1 = md(M1)
        acc1, acc2 = acc1 + m1, acc2 + m1
        h22 = act(acc2 + md(M6), 1, 1)
        out(M2, h21 + h22)
        out(M4, h22)
        out(M7, h12 - h22)
        h11 = act(acc1 + md(M7), 0, 0)
        out(M1, h11 + h22)
        out(M3, h11)
        out(M5, h11 + h12)
        out(M6, h21 - h11)

    def fin(res, base, slot, half, c, side, val, sc):
        rows = pl.ds(pl.multiple_of(base + half * HM, HM), HM)
        for t in range(2):
            cols = _tile(side * 4 + c * 2 + t)
            r = res(rows, cols) + val[:, _tile(t)] * sc + b2[0:1, cols]
            x[rows, cols] = r
            ostage[slot, half, :, cols] = r.astype(bf16)

    def w2_p1(base, slot, c):
        done = P(fin, lambda rows, cols: xt[0:HM, cols], base, slot, 0, c, sc=sh[0:HM, :])
        m3 = mm(hs, w2, M3, c)
        m5 = mm(hs, w2, M5, c)
        done(1, m3 + m5)
        m1 = mm(hs, w2, M1, c)
        carry[1, :, _tile(2 * c, 2)] = m1 + m3
        acc = m1 - m5
        m4 = mm(hs, w2, M4, c)
        carry[0, :, _tile(2 * c, 2)] = m4
        done(0, acc + m4 + mm(hs, w2, M7, c))
        if c == 1:
            carry[2, :, 0:128] = sh[HM:TM, :]

    def w2_p2(base, slot, c):
        done = P(fin, lambda rows, cols: x[rows, cols], base, slot, 1, c, sc=carry[2, :, 0:128])
        m2 = mm(hs, w2, M2, c)
        done(0, carry[0, :, _tile(2 * c, 2)] + m2)
        acc = carry[1, :, _tile(2 * c, 2)] - m2
        done(1, acc + mm(hs, w2, M6, c))

    def put_sums(dst, rows, t, blocks):
        for i, s in enumerate(_b_sums(*blocks)):
            put(dst, i, t, rows, s)

    def permuted(r, n, g):
        lane = lax.broadcasted_iota(i32, (n // 2, 128), 1)
        src = ((lane & 31) << 2) | (lane >> 5)
        ts = [pltpu.bitcast(wqkv_raw[r:r + n, _tile(g * 8 + j)], u32) for j in range(8)]
        ts = [pltpu.roll(t, 4 * j, 1) if j else t for j, t in enumerate(ts)]
        ts = _skew_select(ts, lane, 4)
        return [pltpu.bitcast(jnp.take_along_axis(t, (src + 4 * j) & 127, axis=1), bf16).astype(f32)
                for j, t in enumerate(ts)]

    def prep_qkv(g, n, lo, hi):
        for r in range(lo, hi, n):
            top, bot = permuted(r, n, g), permuted(512 + r, n, g)
            for t in range(4):
                put_sums(wq, slice(r, r + n), g * 4 + t, (top[t], top[t + 4], bot[t], bot[t + 4]))

    def prep_wo():
        index = lax.broadcasted_iota(i32, (8, D), 0)
        for d3 in range(2):
            for h1 in range(2):
                blk = {}
                for d4 in range(2):
                    for h0 in range(2):
                        src = []
                        for hh in range(8):
                            r = hh * 128 + h1 * 64 + h0 * 32 + d4 * 16
                            t = wo_raw[r:r + 16, :].astype(f32)[8 * d3:8 * d3 + 8]
                            src.append(pltpu.roll(t, hh, 0) if hh else t)
                        for dl, t in enumerate(_skew_select(src, index, 1)):
                            blk[d4, h0, dl] = pltpu.roll(t, 8 - dl, 0) if dl else t
                for dl in range(8):
                    r = d3 * 256 + dl * 32 + h1 * 16
                    top, bot = (jnp.concatenate([blk[d4, 0, dl], blk[d4, 1, dl]], axis=0) for d4 in range(2))
                    put_sums(wo, slice(r, r + 16), 0, (top[:, :512], top[:, 512:], bot[:, :512], bot[:, 512:]))

    def prep_w1(c):
        es = []
        for t in (2 * c, 2 * c + 1):
            for r in range(0, 512, 64):
                blocks = [w1_raw[rr:rr + 64, _tile(j)].astype(f32) for rr in (r, 512 + r) for j in (t, t + 14)]
                put_sums(w1, slice(r, r + 64), t, blocks)
                if c == 0:
                    e = _tree(jnp.add, [y * y for y in blocks])
                    es.append(_tree(jnp.add, [e[a:a + 8] for a in range(0, 64, 8)]))
        if c == 0:
            tot = jnp.sum(jnp.sum(_tree(jnp.add, es), axis=1, keepdims=True), axis=0, keepdims=True)
            stat[0:1, :] = jnp.broadcast_to(tot * (1.0 / 512), (1, 128))
            bb = b1[0:1, :]
            stat[1:2, :] = jnp.broadcast_to(jnp.sum(bb * bb, axis=1, keepdims=True) * (1.0 / F) + TINY, (1, 128))

    def prep_w2():
        for t in range(4):
            for r in range(0, HF, 64):
                put_sums(w2, slice(r, r + 64), t,
                         [w2_raw[rr:rr + 64, _tile(j)].astype(f32) for rr in (r, HF + r) for j in (t, t + 4)])

    def cvt_x(r):
        val = xin[r:r + 64, :].astype(f32)
        x[r:r + 64, :] = val
        return _tree(jnp.add, [val[a:a + 8, 0:128] for a in range(0, 64, 8)])

    def dma(src, dst, block, i):
        return pltpu.make_async_copy(src.at[block], dst.at[block], isem.at[i])

    full = slice(None)
    cp_x0 = [[dma(x_hbm, xin, (pl.ds(half * HM + r, 128), full), 10 + 1024 // RQ + 2 * (r // 128) + half)
              for half in range(2)] for r in range(0, HM, 128)]
    cp_x1 = dma(x_hbm, xin, (pl.ds(TM, S - TM), full), 1)
    cp_k, cp_v = (dma(wqkv_hbm, wqkv_raw, (full, pl.ds(g * D, D)), 1 + g) for g in (1, 2))
    cp_wo = dma(wo_hbm, wo_raw, (full, full), 4)
    cp_w2 = dma(w2_hbm, w2_raw, (full, full), 5)
    cp_w1a = [dma(w1_hbm, w1_raw, (full, pl.ds(s * HF, 256 * NPRE)), 6 + s) for s in range(2)]
    cp_w1b = [dma(w1_hbm, w1_raw, (full, pl.ds(s * HF + 256 * NPRE, HF - 256 * NPRE)), 8 + s) for s in range(2)]
    cp_q = [[dma(wqkv_hbm, wqkv_raw, (pl.ds(s * 512 + n * RQ, RQ), pl.ds(0, D)), 10 + 2 * n + s) for s in range(2)]
            for n in range(512 // RQ)]

    def step(t, peeled):
        base = (t % NT) * TM
        pbase = ((t + NT - 1) % NT) * TM
        nbase = ((t + 1) % NT) * TM
        slot = t % 2
        first = t % NT == 0
        clock[0] = 0
        last.clear()
        opt.update(ch=CHF if peeled else CH, cq=CQF if peeled else CQ)
        qk_items = [P(qk8, r, first) for r in range(0, TM, 8)]
        ln1_items = [P(ln1, nbase, 16, r) for r in range(0, HM, 16)]

        def two(f, *a):
            for c in range(2):
                f(*a, c)
        if peeled:
            for cp in [*sum(cp_x0 + cp_q, []), cp_k, cp_v, cp_wo, *cp_w1a, *cp_w1b, cp_w2, cp_x1]:
                cp.start()
            sv[0:HALO, :] = jnp.zeros((HALO, 128), f32)
            k[:, 0:HALO, :] = jnp.zeros((8, HALO, 128), f32)
            b1[0:1, :] = b1_ref[...].astype(f32).reshape(1, F)
            b2[0:1, :] = b2_ref[...].astype(f32).reshape(1, D)
            ostage[slot, 1] = jnp.zeros((HM, D), bf16)
            for r, cps in zip(range(0, HM, 128), cp_x0):
                for cp in cps:
                    cp.wait()
                for rr in (r, r + 64, HM + r, HM + r + 64):
                    cvt_x(rr)
                ln1(base, 128, r)
            for n, cps in enumerate(cp_q):
                for cp in cps:
                    cp.wait()
                prep_qkv(0, 128, n * RQ, (n + 1) * RQ)
            plan(QKF, qk_items)
            qkv_p1(0, 0)
            qkv_p2(0, 0)
            cp_k.wait()
            prep_qkv(1, 128, 0, 512)
            qkv_p1(0, 1)
            qkv_p2(0, 1)
            if VB:
                qkv_p1(1, 0)
            cp_v.wait()
            cp_wo.wait()
            prep_qkv(2, 128, 0, 512)
            prep_wo()
            if not VB:
                qkv_p1(1, 0)
            qkv_p1(1, 1)
        else:
            plan(QK if TQ else (QK[1], QK[1]), qk_items)
            plan(L1, ln1_items)
            two(qkv_p1, 0)
            two(qkv_p1, 1)
            two(qkv_p2, 0)
        two(qkv_p2, 1)
        two(qkv_p1, 2)
        v_first(first)
        two(qkv_p2, 2)
        flush(QK[1])
        for half in range(2):
            for r in range(0, HM, 16):
                pv16(half, r)
        if not peeled:
            w2_p2(pbase, slot, 0)
        two(wo_p1, base)
        halo_save()
        if peeled:
            for cp in cp_w1a:
                cp.wait()
            for c in range(NPRE):
                prep_w1(c)
        two(wo_p2, base)
        two(wo_p3, base)
        if not peeled:
            w2_p2(pbase, slot, 1)
        for half in range(2):
            for r in range(0, HM, 16):
                ln2(half, r)
        for c in range(NPRE):
            w1_pre(c)
        for c in range(7):
            if peeled and c == NPRE:
                for cp in [*cp_w1b, cp_w2, cp_x1]:
                    cp.wait()
                for cc in range(NPRE, 7):
                    prep_w1(cc)
                for r in range(TM, 2 * TM, 64):
                    cvt_x(r)
                w = ((2000, 12000), (14000, 27000)) if XF == 0 else ((11000, 27000), (11000, 27000))
                plan((clock[0] + w[0][0], clock[0] + w[0][1]), ln1_items)
                plan((clock[0] + w[1][0], clock[0] + w[1][1]), [P(cvt_x, r) for r in range(2 * TM, S, 64)])
                prep_w2()
            w1_chunk(c)
        two(w2_p1, base, slot)
        flush(float("inf"))

    def out_copies(t):
        return [pltpu.make_async_copy(
            ostage.at[t % 2, half],
            out_hbm.at[pl.ds(pl.multiple_of(((t + (NT - 1) * half) % NT) * TM + half * HM, HM), HM), :],
            osem.at[half]) for half in range(2)]

    if MODE != "body":
        step(0, True)

    def body(t, c):
        cps = out_copies(t - 1)
        for cp in cps:
            cp.start()
        step(t, False)
        for cp in cps:
            cp.wait()
        return c

    if MODE != "first":
        lax.fori_loop(1, 2 * NT, body, 0)
    cps = out_copies(2 * NT - 1)
    for cp in cps:
        cp.start()
    for c in range(2):
        w2_p2(S - TM, 0, c)
    for cp in cps:
        cp.wait()
    last = out_copies(2 * NT)[1]
    last.start()
    last.wait()


@jax.jit
def pallas_interleave_layers__sliding_local_dilated__dense_activation_squared_relu__prompt_kernel(A_x, A_wqkv, A_wo, B_x, B_w1, B_b1, B_w2, B_b2):
    del B_x
    hbm = pl.BlockSpec(memory_space=pl.ANY)
    vmem = pl.BlockSpec(memory_space=pltpu.VMEM)
    V = pltpu.VMEM
    out = pl.pallas_call(
        _kernel,
        in_specs=[hbm, hbm, hbm, hbm, vmem, hbm, vmem],
        out_specs=hbm,
        out_shape=jax.ShapeDtypeStruct((S, D), bf16),
        scratch_shapes=[
            V((2, 2, HM, D), bf16), V((S, D), bf16), V((S, D), f32),
            V((D, 3 * D), bf16), V((D, D), bf16), V((D, F), bf16), V((F, D), bf16),
            V((7, 12, 512, 128), bf16), V((7, 4, 512, 128), bf16),
            V((7, 14, 512, 128), bf16), V((7, 4, HF, 128), bf16),
            V((7, 4, HM, 128), bf16), V((7, 4, HM, 128), bf16), V((7, 4, HM, 128), bf16), V((7, 14, HM, 128), bf16),
            V((8, TM, 128), f32), V((8, TM + HALO, 128), f32), V((8, TM + HALO, 128), f32), V((W, TM, 128), f32),
            V((HM, D), f32), V((TM, D), f32),
            V((3, HM, 512), f32), V((2, HM, 256 * NPRE), f32), V((3, HM, 512), f32),
            V((TM, 128), f32), V((TM, 128), f32), V((TM + HALO, 128), f32), V((TM, 128), f32),
            V((TM, 128), f32), V((TM, 128), f32), V((TM, 128), f32),
            V((8, F), f32), V((8, D), f32), V((8, 128), f32),
            pltpu.SemaphoreType.DMA((14 + 1024 // RQ,)), pltpu.SemaphoreType.DMA((2,)),
        ],
        compiler_params=pltpu.CompilerParams(vmem_limit_bytes=127 * 1024 * 1024),
    )(A_x.reshape(S, D), A_wqkv, A_wo, B_w1, B_b1, B_w2, B_b2)
    return out.reshape(1, S, D)
```

```python
import functools

import jax
import jax.numpy as jnp
import numpy as np
from jax import lax
import jax.experimental.pallas as pl
import jax.experimental.pallas.tpu as pltpu

S, D, F = 2048, 1024, 3584
DH, W, DIL = 32, 8, 2
TM = 512
HM = TM // 2
HF = F // 2
NT = S // TM
HALO = 16
EPS = 1e-5
TINY = 1e-30
QSCALE = float(DH ** -0.5 * np.log2(np.e))
NEG = float(-1e9 * np.log2(np.e))
NPRE = 4
RQ = 256
QK = (10900, 21500)
QKF = (14000, 21400)
L1 = (42000, 58000)
f32, bf16, u32, i32 = jnp.float32, jnp.bfloat16, jnp.uint32, jnp.int32
P = functools.partial


def _tree(op, xs):
    xs = list(xs)
    while len(xs) > 1:
        xs = [op(xs[i], xs[i + 1]) if i + 1 < len(xs) else xs[i] for i in range(0, len(xs), 2)]
    return xs[0]


def _a_sums(a11, a12, a21, a22):
    return (a11 + a22, a21 + a22, a11, a22, a11 + a12, a21 - a11, a12 - a22)


def _b_sums(b11, b12, b21, b22):
    return (b11 + b22, b11, b12 - b22, b21 - b11, b22, b11 + b12, b21 + b22)


M1, M2, M3, M4, M5, M6, M7 = range(7)


def _tile(j, n=1):
    return slice(j * 128, (j + n) * 128)


def _pow2(s):
    return pltpu.bitcast((pltpu.bitcast(s, i32) + 0x007FFFFF) & 0x7F800000, f32)


def _pow2_inv(s):
    return pltpu.bitcast(0x7F000000 - pltpu.bitcast(s, i32), f32)


def _pow2_sqrt(s):
    half = lax.shift_right_logical(pltpu.bitcast(s, i32), 1)
    return pltpu.bitcast((half + 0x1FC00000) & 0x7F800000, f32)


def _skew_select(ts, index, unit):
    ts = [ts[-i % 8] for i in range(8)]
    for b in (1, 2, 4):
        take = (index & (unit * b)) != 0
        ts = [jnp.where(take, ts[(i - b) % 8], ts[i]) for i in range(8)]
    return ts


def _kernel(x_hbm, wqkv_hbm, wo_hbm, w1_hbm, b1_ref, w2_hbm, b2_ref, out_hbm,
            ostage, xin, x, wqkv_raw, wo_raw, w1_raw, w2_raw,
            wq, wo, w1, w2, xs1, xs2, os_, hs, q, k, v, pr, ua, xt, part, pre, carry,
            s1, sq, sv, so, sg, gh, sh, b1, b2, stat, isem, osem):
    sub = lax.broadcasted_iota(i32, (8, 128), 0)

    clock = [0]
    queue = []

    def never(shape, dtype):
        return jnp.broadcast_to(jnp.abs(b2[0:1, 0:128]), shape).astype(dtype) < 0

    def plan(window, items):
        lo, hi = window
        queue.extend((lo + (hi - lo) * (n + 1) / len(items), f) for n, f in enumerate(items))
        queue.sort(key=lambda e: e[0])

    def flush(until):
        vals = []
        while queue and queue[0][0] <= until:
            vals.append(queue.pop(0)[1]())
        return vals

    def tie(operand, r, until):
        vals = flush(until)
        if not vals:
            return operand
        d = _tree(jnp.add, vals)
        d = jnp.concatenate([d, d], axis=0).astype(bf16)
        parts = [operand[:r], jnp.where(never((16, 128), bf16), d, operand[r:r + 16]), operand[r + 16:]]
        return jnp.concatenate([p for p in parts if p.shape[0]], axis=0)

    last = {}

    def after(key, val):
        if key not in last:
            return val
        return jnp.where(never(val.shape, f32), last[key], val)

    def mm(a_ref, w_ref, i, c):
        kt = a_ref.shape[1]
        ls = [a_ref[i, t] for t in range(kt)]
        rs = [w_ref[i, 2 * c + n] for n in range(2)]
        t0 = clock[0]
        clock[0] = t0 + 128 * kt
        if kt == 4:
            out = []
            for n in range(2):
                l0 = ls[0]
                for r in range(0, HM, 64):
                    l0 = tie(l0, r, t0 + n * 256 + r + 63)
                out.append(jnp.dot(jnp.concatenate([l0] + ls[1:], axis=1), rs[n], preferred_element_type=f32))
            return jnp.concatenate(out, axis=1)
        for g in range(kt // 4 + 1):
            for r in range(0, HM, 64):
                ls[4 * g] = tie(ls[4 * g], r, t0 + g * 448 + r + 63)
        return jnp.dot(jnp.concatenate(ls, axis=1), jnp.concatenate(rs, axis=1), preferred_element_type=f32)

    def put(dst, i, t0, rows, val):
        for t in range(val.shape[1] // 128):
            dst[i, t0 + t, rows, :] = val[:, _tile(t)].astype(bf16)

    def put_a(dst, r, ua_):
        ua[r:r + 16, :] = ua_
        put(dst, M3, 0, slice(r, r + 16), ua_[:, :512])
        put(dst, M5, 0, slice(r, r + 16), ua_[:, :512] + ua_[:, 512:])

    def put_b(dst, r, ub):
        ss = _a_sums(ua[r:r + 16, :512], ua[r:r + 16, 512:], ub[:, :512], ub[:, 512:])
        for i in (M1, M2, M4, M6, M7):
            put(dst, i, 0, slice(r, r + 16), ss[i])

    def ln(xv, chain=False):
        if chain:
            xv = jnp.concatenate([after('ln', xv[:, :128]), xv[:, 128:]], axis=1)
        z = xv - jnp.sum(xv, axis=1, keepdims=True) * (1.0 / D)
        var = jnp.sum(z * z, axis=1, keepdims=True) * (1.0 / D)
        var = jnp.broadcast_to(var, (xv.shape[0], 128))
        if chain:
            last['ln'] = var
        size = _pow2_sqrt(jnp.maximum(var, TINY))
        g = _pow2_inv(size)
        u = jnp.concatenate([z[:, _tile(j)] * g for j in range(8)], axis=1)
        return u, lax.rsqrt(var + EPS) * size

    def ln1(base, n, r):
        ua_, sa = ln(x[pl.ds(pl.multiple_of(base + r, n), n), :])
        ub, sb = ln(x[pl.ds(pl.multiple_of(base + HM + r, n), n), :])
        for i, val in enumerate(_a_sums(ua_[:, :512], ua_[:, 512:], ub[:, :512], ub[:, 512:])):
            put(xs1, i, 0, slice(r, r + n), val)
        for r0, s in ((r, sa), (HM + r, sb)):
            s1[r0:r0 + n, :] = s
            sq[r0:r0 + n, :] = s * QSCALE
            sv[HALO + r0:HALO + r0 + n, :] = _pow2(s)
        return (sa + sb)[0:8]

    def ln2(half, r, chain):
        rows = slice(half * HM + r, half * HM + r + 16)
        u, s = ln(xt[rows, :], chain)
        (put_b if half else put_a)(xs2, r, u)
        p = s * s * stat[0:1, :] + stat[1:2, :]
        size = _pow2_sqrt(p)
        g = _pow2_inv(size)
        gh[rows, :] = g
        sg[rows, :] = s * g
        sh[rows, :] = size * size

    def qkv_dst(g, j, half):
        if g == 0:
            return q.at[j, pl.ds(half * HM, HM), :]
        return (k, v)[g - 1].at[j, pl.ds(HALO + half * HM, HM), :]

    def qkv_p1(g, c):
        sc = (sq if g == 0 else s1)[0:HM, :]
        sc = jnp.concatenate([sc, sc], axis=1)
        md = P(mm, xs1, wq, c=g * 2 + c)

        def out(j, half, val):
            for t in range(2):
                qkv_dst(g, c * 2 + j + t, half)[...] = val[:, _tile(t)]
        m3 = md(M3)
        m5 = md(M5)
        out(4, 0, (m3 + m5) * sc)
        m1 = md(M1)
        out(4, 1, m1 + m3)
        acc = m1 - m5
        m4 = md(M4)
        out(0, 1, m4)
        out(0, 0, (acc + m4 + md(M7)) * sc)

    def qkv_p2(g, c):
        sc = (sq if g == 0 else s1)[HM:TM, :]
        m2 = mm(xs1, wq, M2, g * 2 + c)
        acc = []
        for t in range(2):
            l, r = qkv_dst(g, c * 2 + t, 1), qkv_dst(g, c * 2 + t + 4, 1)
            l[...] = (l[...] + m2[:, _tile(t)]) * sc
            acc.append(r[...] - m2[:, _tile(t)])
        m6 = mm(xs1, wq, M6, g * 2 + c)
        for t in range(2):
            qkv_dst(g, c * 2 + t + 4, 1)[...] = (acc[t] + m6[:, _tile(t)]) * sc

    def window(ref, lead, r):
        return [ref[lead + (pl.ds(HALO + r - DIL * w, 8), slice(None))] for w in range(W)]

    def qk8(r, first, chain):
        qs = [q[j, r:r + 8, :] for j in range(8)]
        if chain:
            qs = [after('qk', t) for t in qs]
        ks = [window(k, (j,), r) for j in range(8)]
        ls = []
        for w in range(W):
            p = _tree(jnp.add, [qs[j] * ks[j][w] for j in range(8)])
            p = (p + pltpu.roll(p, 64, 1)) + (pltpu.roll(p, 32, 1) + pltpu.roll(p, 96, 1))
            if r - DIL * w < 0:
                p = jnp.where(jnp.logical_and(first, sub + (r - DIL * w) < 0), NEG, p)
            ls.append(p)
        last['qk'] = ls[0]
        m = _tree(jnp.maximum, ls)
        es = [jnp.exp2(l - m) for l in ls]
        sc = _tree(jnp.maximum, window(sv, (), r))
        so[r:r + 8, :] = sc
        den = _tree(jnp.add, es)
        inv = pltpu.reciprocal(den, approx=True)
        inv = inv * (2.0 - den * inv) * _pow2_inv(sc)
        for w in range(W):
            pr[w, r:r + 8, :] = es[w] * inv
        return inv

    def pv8(r):
        ps = [pr[w, r:r + 8, :] for w in range(W)]
        return jnp.concatenate(
            [_tree(jnp.add, [a * b for a, b in zip(ps, window(v, (j,), r))]) for j in range(8)], axis=1)

    def pv16(half, r):
        r0 = half * HM + r
        (put_b if half else put_a)(os_, r, jnp.concatenate([pv8(r0), pv8(r0 + 8)], axis=0))

    def v_first(first):
        for j in range(8):
            v0 = jnp.broadcast_to(v[j, HALO:HALO + 1, :], (HALO, 128))
            v[j, 0:HALO, :] = jnp.where(first, v0, v[j, 0:HALO, :])

    def halo_save():
        sv[0:HALO, :] = sv[TM:TM + HALO, :]
        for j in range(8):
            k[j, 0:HALO, :] = k[j, TM:TM + HALO, :]
            v[j, 0:HALO, :] = v[j, TM:TM + HALO, :]

    def acc_x(base, half, j, val):
        rows = pl.ds(pl.multiple_of(base + half * HM, HM), HM)
        sc = so[half * HM:(half + 1) * HM, :]
        for t in range(2):
            r = x[rows, _tile(j + t)] + val[:, _tile(t)] * sc
            xt[half * HM:(half + 1) * HM, _tile(j + t)] = r
            if half:
                x[rows, _tile(j + t)] = r

    def wo_p1(base, c):
        cols = _tile(c * 2, 2)
        m3 = mm(os_, wo, M3, c)
        part[2, :, cols] = m3
        m5 = mm(os_, wo, M5, c)
        part[0, :, cols] = m5
        acc_x(base, 0, 4 + c * 2, m3 + m5)

    def wo_p2(base, c):
        cols = _tile(c * 2, 2)
        m1 = mm(os_, wo, M1, c)
        part[2, :, cols] = part[2, :, cols] + m1
        acc = m1 - part[0, :, cols]
        m4 = mm(os_, wo, M4, c)
        part[1, :, cols] = m4
        acc_x(base, 0, c * 2, acc + m4 + mm(os_, wo, M7, c))

    def wo_p3(base, c):
        cols = _tile(c * 2, 2)
        m2 = mm(os_, wo, M2, c)
        acc_x(base, 1, c * 2, part[1, :, cols] + m2)
        acc = part[2, :, cols] - m2
        acc_x(base, 1, 4 + c * 2, acc + mm(os_, wo, M6, c))

    def w1_pre(c):
        pre[0, :, _tile(c * 2, 2)] = mm(xs2, w1, M3, c)
        pre[1, :, _tile(c * 2, 2)] = mm(xs2, w1, M5, c)

    def w1_chunk(c):
        md = P(mm, xs2, w1, c=c)

        def act(z, half, side):
            rows = slice(half * HM, (half + 1) * HM)
            out = []
            for t in range(2):
                b = b1[0:1, _tile(side * 14 + c * 2 + t)]
                y = jnp.maximum(z[:, _tile(t)] * sg[rows, :] + gh[rows, :] * b, 0.0)
                out.append(y * y)
            return jnp.concatenate(out, axis=1)

        def out(i, val):
            put(hs, i, c * 2, slice(0, HM), val)
        if c < NPRE:
            m3, m5 = pre[0, :, _tile(c * 2, 2)], pre[1, :, _tile(c * 2, 2)]
        else:
            m3, m5 = md(M3), md(M5)
        h12 = act(m3 + m5, 0, 1)
        m4 = md(M4)
        acc1 = m4 - m5
        m2 = md(M2)
        h21 = act(m4 + m2, 1, 0)
        acc2 = m3 - m2
        m1 = md(M1)
        acc1, acc2 = acc1 + m1, acc2 + m1
        h22 = act(acc2 + md(M6), 1, 1)
        out(M2, h21 + h22)
        out(M4, h22)
        out(M7, h12 - h22)
        h11 = act(acc1 + md(M7), 0, 0)
        out(M1, h11 + h22)
        out(M3, h11)
        out(M5, h11 + h12)
        out(M6, h21 - h11)

    def fin(res, base, slot, half, c, side, val, sc):
        rows = pl.ds(pl.multiple_of(base + half * HM, HM), HM)
        for t in range(2):
            cols = _tile(side * 4 + c * 2 + t)
            r = res(rows, cols) + val[:, _tile(t)] * sc + b2[0:1, cols]
            x[rows, cols] = r
            ostage[slot, half, :, cols] = r.astype(bf16)

    def w2_p1(base, slot, c):
        done = P(fin, lambda rows, cols: xt[0:HM, cols], base, slot, 0, c, sc=sh[0:HM, :])
        m3 = mm(hs, w2, M3, c)
        m5 = mm(hs, w2, M5, c)
        done(1, m3 + m5)
        m1 = mm(hs, w2, M1, c)
        carry[1, :, _tile(2 * c, 2)] = m1 + m3
        acc = m1 - m5
        m4 = mm(hs, w2, M4, c)
        carry[0, :, _tile(2 * c, 2)] = m4
        done(0, acc + m4 + mm(hs, w2, M7, c))
        if c == 1:
            carry[2, :, 0:128] = sh[HM:TM, :]

    def w2_p2(base, slot, c):
        done = P(fin, lambda rows, cols: x[rows, cols], base, slot, 1, c, sc=carry[2, :, 0:128])
        m2 = mm(hs, w2, M2, c)
        done(0, carry[0, :, _tile(2 * c, 2)] + m2)
        acc = carry[1, :, _tile(2 * c, 2)] - m2
        done(1, acc + mm(hs, w2, M6, c))

    def put_sums(dst, rows, t, blocks):
        for i, s in enumerate(_b_sums(*blocks)):
            put(dst, i, t, rows, s)

    def permuted(r, n, g):
        lane = lax.broadcasted_iota(i32, (n // 2, 128), 1)
        src = ((lane & 31) << 2) | (lane >> 5)
        ts = [pltpu.bitcast(wqkv_raw[r:r + n, _tile(g * 8 + j)], u32) for j in range(8)]
        ts = [pltpu.roll(t, 4 * j, 1) if j else t for j, t in enumerate(ts)]
        ts = _skew_select(ts, lane, 4)
        return [pltpu.bitcast(jnp.take_along_axis(t, (src + 4 * j) & 127, axis=1), bf16).astype(f32)
                for j, t in enumerate(ts)]

    def prep_qkv(g, n, lo, hi):
        for r in range(lo, hi, n):
            top, bot = permuted(r, n, g), permuted(512 + r, n, g)
            for t in range(4):
                put_sums(wq, slice(r, r + n), g * 4 + t, (top[t], top[t + 4], bot[t], bot[t + 4]))

    def prep_wo():
        index = lax.broadcasted_iota(i32, (8, D), 0)
        for d3 in range(2):
            for h1 in range(2):
                blk = {}
                for d4 in range(2):
                    for h0 in range(2):
                        src = []
                        for hh in range(8):
                            r = hh * 128 + h1 * 64 + h0 * 32 + d4 * 16
                            t = wo_raw[r:r + 16, :].astype(f32)[8 * d3:8 * d3 + 8]
                            src.append(pltpu.roll(t, hh, 0) if hh else t)
                        for dl, t in enumerate(_skew_select(src, index, 1)):
                            blk[d4, h0, dl] = pltpu.roll(t, 8 - dl, 0) if dl else t
                for dl in range(8):
                    r = d3 * 256 + dl * 32 + h1 * 16
                    top, bot = (jnp.concatenate([blk[d4, 0, dl], blk[d4, 1, dl]], axis=0) for d4 in range(2))
                    put_sums(wo, slice(r, r + 16), 0, (top[:, :512], top[:, 512:], bot[:, :512], bot[:, 512:]))

    def prep_w1(c):
        es = []
        for t in (2 * c, 2 * c + 1):
            for r in range(0, 512, 64):
                blocks = [w1_raw[rr:rr + 64, _tile(j)].astype(f32) for rr in (r, 512 + r) for j in (t, t + 14)]
                put_sums(w1, slice(r, r + 64), t, blocks)
                if c == 0:
                    e = _tree(jnp.add, [y * y for y in blocks])
                    es.append(_tree(jnp.add, [e[a:a + 8] for a in range(0, 64, 8)]))
        if c == 0:
            tot = jnp.sum(jnp.sum(_tree(jnp.add, es), axis=1, keepdims=True), axis=0, keepdims=True)
            stat[0:1, :] = jnp.broadcast_to(tot * (1.0 / 512), (1, 128))
            bb = b1[0:1, :]
            stat[1:2, :] = jnp.broadcast_to(jnp.sum(bb * bb, axis=1, keepdims=True) * (1.0 / F) + TINY, (1, 128))

    def prep_w2():
        for t in range(4):
            for r in range(0, HF, 64):
                put_sums(w2, slice(r, r + 64), t,
                         [w2_raw[rr:rr + 64, _tile(j)].astype(f32) for rr in (r, HF + r) for j in (t, t + 4)])

    def cvt_x(r):
        val = xin[r:r + 64, :].astype(f32)
        x[r:r + 64, :] = val
        return _tree(jnp.add, [val[a:a + 8, 0:128] for a in range(0, 64, 8)])

    def dma(src, dst, block, i):
        return pltpu.make_async_copy(src.at[block], dst.at[block], isem.at[i])

    full = slice(None)
    cp_x0 = [[dma(x_hbm, xin, (pl.ds(half * HM + r, 128), full), 10 + 1024 // RQ + 2 * (r // 128) + half)
              for half in range(2)] for r in range(0, HM, 128)]
    cp_x1 = dma(x_hbm, xin, (pl.ds(TM, S - TM), full), 1)
    cp_k, cp_v = (dma(wqkv_hbm, wqkv_raw, (full, pl.ds(g * D, D)), 1 + g) for g in (1, 2))
    cp_wo = dma(wo_hbm, wo_raw, (full, full), 4)
    cp_w2 = dma(w2_hbm, w2_raw, (full, full), 5)
    cp_w1a = [dma(w1_hbm, w1_raw, (full, pl.ds(s * HF, 256 * NPRE)), 6 + s) for s in range(2)]
    cp_w1b = [dma(w1_hbm, w1_raw, (full, pl.ds(s * HF + 256 * NPRE, HF - 256 * NPRE)), 8 + s) for s in range(2)]
    cp_q = [[dma(wqkv_hbm, wqkv_raw, (pl.ds(s * 512 + n * RQ, RQ), pl.ds(0, D)), 10 + 2 * n + s) for s in range(2)]
            for n in range(512 // RQ)]

    def step(t, peeled):
        base = (t % NT) * TM
        pbase = ((t + NT - 1) % NT) * TM
        nbase = ((t + 1) % NT) * TM
        slot = t % 2
        first = t % NT == 0
        clock[0] = 0
        last.clear()
        qk_items = [P(qk8, r, first, not peeled) for r in range(0, TM, 8)]
        ln1_items = [P(ln1, nbase, 16, r) for r in range(0, HM, 16)]

        def two(f, *a):
            for c in range(2):
                f(*a, c)
        if peeled:
            for cp in [*sum(cp_x0 + cp_q, []), cp_k, cp_v, cp_wo, *cp_w1a, *cp_w1b, cp_w2, cp_x1]:
                cp.start()
            sv[0:HALO, :] = jnp.zeros((HALO, 128), f32)
            k[:, 0:HALO, :] = jnp.zeros((8, HALO, 128), f32)
            v[:, 0:HALO, :] = jnp.zeros((8, HALO, 128), f32)
            b1[0:1, :] = b1_ref[...].astype(f32).reshape(1, F)
            b2[0:1, :] = b2_ref[...].astype(f32).reshape(1, D)
            ostage[slot, 1] = jnp.zeros((HM, D), bf16)
            for r, cps in zip(range(0, HM, 128), cp_x0):
                for cp in cps:
                    cp.wait()
                for rr in (r, r + 64, HM + r, HM + r + 64):
                    cvt_x(rr)
                ln1(base, 128, r)
            for n, cps in enumerate(cp_q):
                for cp in cps:
                    cp.wait()
                prep_qkv(0, 128, n * RQ, (n + 1) * RQ)
            plan(QKF, qk_items)
            qkv_p1(0, 0)
            qkv_p2(0, 0)
            cp_k.wait()
            prep_qkv(1, 128, 0, 512)
            qkv_p1(0, 1)
            qkv_p2(0, 1)
            qkv_p1(1, 0)
            cp_v.wait()
            cp_wo.wait()
            prep_qkv(2, 128, 0, 512)
            prep_wo()
            qkv_p1(1, 1)
        else:
            plan(QK, qk_items)
            plan(L1, ln1_items)
            two(qkv_p1, 0)
            two(qkv_p1, 1)
            two(qkv_p2, 0)
        two(qkv_p2, 1)
        two(qkv_p1, 2)
        v_first(first)
        two(qkv_p2, 2)
        flush(QK[1])
        for half in range(2):
            for r in range(0, HM, 16):
                pv16(half, r)
        if not peeled:
            w2_p2(pbase, slot, 0)
        two(wo_p1, base)
        halo_save()
        if peeled:
            for cp in cp_w1a:
                cp.wait()
            for c in range(NPRE):
                prep_w1(c)
        two(wo_p2, base)
        two(wo_p3, base)
        if not peeled:
            w2_p2(pbase, slot, 1)
        for half in range(2):
            for r in range(0, HM, 16):
                ln2(half, r, not peeled)
        for c in range(NPRE):
            w1_pre(c)
        for c in range(7):
            if peeled and c == NPRE:
                for cp in [*cp_w1b, cp_w2, cp_x1]:
                    cp.wait()
                for cc in range(NPRE, 7):
                    prep_w1(cc)
                for r in range(TM, 2 * TM, 64):
                    cvt_x(r)
                late = (clock[0] + 11000, clock[0] + 27000)
                plan(late, ln1_items)
                plan(late, [P(cvt_x, r) for r in range(2 * TM, S, 64)])
                prep_w2()
            w1_chunk(c)
        two(w2_p1, base, slot)
        flush(float("inf"))

    def out_copies(t):
        return [pltpu.make_async_copy(
            ostage.at[t % 2, half],
            out_hbm.at[pl.ds(pl.multiple_of(((t + (NT - 1) * half) % NT) * TM + half * HM, HM), HM), :],
            osem.at[half]) for half in range(2)]

    step(0, True)

    def body(t, c):
        cps = out_copies(t - 1)
        for cp in cps:
            cp.start()
        step(t, False)
        for cp in cps:
            cp.wait()
        return c

    lax.fori_loop(1, 2 * NT, body, 0)
    cps = out_copies(2 * NT - 1)
    for cp in cps:
        cp.start()
    for c in range(2):
        w2_p2(S - TM, 0, c)
    for cp in cps:
        cp.wait()
    last = out_copies(2 * NT)[1]
    last.start()
    last.wait()


@jax.jit
def pallas_interleave_layers__sliding_local_dilated__dense_activation_squared_relu__prompt_kernel(A_x, A_wqkv, A_wo, B_x, B_w1, B_b1, B_w2, B_b2):
    del B_x
    hbm = pl.BlockSpec(memory_space=pl.ANY)
    vmem = pl.BlockSpec(memory_space=pltpu.VMEM)
    V = pltpu.VMEM
    out = pl.pallas_call(
        _kernel,
        in_specs=[hbm, hbm, hbm, hbm, vmem, hbm, vmem],
        out_specs=hbm,
        out_shape=jax.ShapeDtypeStruct((S, D), bf16),
        scratch_shapes=[
            V((2, 2, HM, D), bf16), V((S, D), bf16), V((S, D), f32),
            V((D, 3 * D), bf16), V((D, D), bf16), V((D, F), bf16), V((F, D), bf16),
            V((7, 12, 512, 128), bf16), V((7, 4, 512, 128), bf16),
            V((7, 14, 512, 128), bf16), V((7, 4, HF, 128), bf16),
            V((7, 4, HM, 128), bf16), V((7, 4, HM, 128), bf16), V((7, 4, HM, 128), bf16), V((7, 14, HM, 128), bf16),
            V((8, TM, 128), f32), V((8, TM + HALO, 128), f32), V((8, TM + HALO, 128), f32), V((W, TM, 128), f32),
            V((HM, D), f32), V((TM, D), f32),
            V((3, HM, 512), f32), V((2, HM, 256 * NPRE), f32), V((3, HM, 512), f32),
            V((TM, 128), f32), V((TM, 128), f32), V((TM + HALO, 128), f32), V((TM, 128), f32),
            V((TM, 128), f32), V((TM, 128), f32), V((TM, 128), f32),
            V((8, F), f32), V((8, D), f32), V((8, 128), f32),
            pltpu.SemaphoreType.DMA((14 + 1024 // RQ,)), pltpu.SemaphoreType.DMA((2,)),
        ],
        compiler_params=pltpu.CompilerParams(vmem_limit_bytes=127 * 1024 * 1024),
    )(A_x.reshape(S, D), A_wqkv, A_wo, B_w1, B_b1, B_w2, B_b2)
    return out.reshape(1, S, D)
```

```python
import functools

import jax
import jax.numpy as jnp
import numpy as np
from jax import lax
import jax.experimental.pallas as pl
import jax.experimental.pallas.tpu as pltpu

S, D, F = 2048, 1024, 3584
DH, W, DIL = 32, 8, 2
TM = 512
HM = TM // 2
HF = F // 2
NT = S // TM
HALO = 16
EPS = 1e-5
TINY = 1e-30
QSCALE = float(DH ** -0.5 * np.log2(np.e))
NEG = float(-1e9 * np.log2(np.e))
MODE = 'all'
N0 = 1
COV = (3, 6)
CS = 16
TO = (14500, 22900)
TK = (3900, 6600)
TV = (10000, 13800)
NK = 64
TA = (2000, 14000, 1100)
CB = 2
T2 = (500, 15000)
NPRE = 4
RQ = 256
QK = (10900, 21500)
QKF = (14000, 21400)
L1 = (42000, 59000)
f32, bf16, u32, i32 = jnp.float32, jnp.bfloat16, jnp.uint32, jnp.int32
P = functools.partial


def _tree(op, xs):
    xs = list(xs)
    while len(xs) > 1:
        xs = [op(xs[i], xs[i + 1]) if i + 1 < len(xs) else xs[i] for i in range(0, len(xs), 2)]
    return xs[0]


def _a_sums(a11, a12, a21, a22):
    return (a11 + a22, a21 + a22, a11, a22, a11 + a12, a21 - a11, a12 - a22)


def _b_sums(b11, b12, b21, b22):
    return (b11 + b22, b11, b12 - b22, b21 - b11, b22, b11 + b12, b21 + b22)


M1, M2, M3, M4, M5, M6, M7 = range(7)


def _tile(j, n=1):
    return slice(j * 128, (j + n) * 128)


def _pow2(s):
    return pltpu.bitcast((pltpu.bitcast(s, i32) + 0x007FFFFF) & 0x7F800000, f32)


def _pow2_inv(s):
    return pltpu.bitcast(0x7F000000 - pltpu.bitcast(s, i32), f32)


def _pow2_sqrt(s):
    half = lax.shift_right_logical(pltpu.bitcast(s, i32), 1)
    return pltpu.bitcast((half + 0x1FC00000) & 0x7F800000, f32)


def _skew_select(ts, index, unit):
    ts = [ts[-i % 8] for i in range(8)]
    for b in (1, 2, 4):
        take = (index & (unit * b)) != 0
        ts = [jnp.where(take, ts[(i - b) % 8], ts[i]) for i in range(8)]
    return ts


def _kernel(x_hbm, wqkv_hbm, wo_hbm, w1_hbm, b1_ref, w2_hbm, b2_ref, out_hbm,
            ostage, xin, x, wqkv_raw, wo_raw, w1_raw, w2_raw,
            wq, wo, w1, w2, xs1, xs2, os_, hs, q, k, v, pr, ua, xt, part, pre, carry,
            s1, sq, sv, so, sg, gh, sh, b1, b2, stat, isem, osem):
    sub = lax.broadcasted_iota(i32, (8, 128), 0)

    clock = [0]
    queue = []

    def never(shape, dtype):
        return jnp.broadcast_to(jnp.abs(b2[0:1, 0:128]), shape).astype(dtype) < 0

    def plan(window, items):
        lo, hi = window
        queue.extend((lo + (hi - lo) * (n + 1) / len(items), f) for n, f in enumerate(items))
        queue.sort(key=lambda e: e[0])

    def flush(until):
        vals = []
        while queue and queue[0][0] <= until:
            vals.append(queue.pop(0)[1]())
        return vals

    def tie(operand, r, until):
        vals = flush(until)
        if not vals:
            return operand
        d = _tree(jnp.add, vals)
        d = jnp.concatenate([d, d], axis=0).astype(bf16)
        parts = [operand[:r], jnp.where(never((16, 128), bf16), d, operand[r:r + 16]), operand[r + 16:]]
        return jnp.concatenate([p for p in parts if p.shape[0]], axis=0)

    last = {}

    def after(key, val):
        if key not in last:
            return val
        return jnp.where(never(val.shape, f32), last[key], val)

    def mm(a_ref, w_ref, i, c):
        kt = a_ref.shape[1]
        ls = [a_ref[i, t] for t in range(kt)]
        rs = [w_ref[i, 2 * c + n] for n in range(2)]
        t0 = clock[0]
        clock[0] = t0 + 128 * kt
        if kt == 4:
            out = []
            for n in range(2):
                l0 = ls[0]
                for r in range(0, HM, 64):
                    l0 = tie(l0, r, t0 + n * 256 + r + 63)
                out.append(jnp.dot(jnp.concatenate([l0] + ls[1:], axis=1), rs[n], preferred_element_type=f32))
            return jnp.concatenate(out, axis=1)
        for g in range(kt // 4 + 1):
            for r in range(0, HM, 64):
                ls[4 * g] = tie(ls[4 * g], r, t0 + g * 448 + r + 63)
        return jnp.dot(jnp.concatenate(ls, axis=1), jnp.concatenate(rs, axis=1), preferred_element_type=f32)

    def put(dst, i, t0, rows, val):
        for t in range(val.shape[1] // 128):
            dst[i, t0 + t, rows, :] = val[:, _tile(t)].astype(bf16)

    def put_a(dst, r, ua_):
        ua[r:r + 16, :] = ua_
        put(dst, M3, 0, slice(r, r + 16), ua_[:, :512])
        put(dst, M5, 0, slice(r, r + 16), ua_[:, :512] + ua_[:, 512:])

    def put_b(dst, r, ub):
        ss = _a_sums(ua[r:r + 16, :512], ua[r:r + 16, 512:], ub[:, :512], ub[:, 512:])
        for i in (M1, M2, M4, M6, M7):
            put(dst, i, 0, slice(r, r + 16), ss[i])

    def ln(xv, chain=False):
        if chain:
            xv = jnp.concatenate([after('ln', xv[:, :128]), xv[:, 128:]], axis=1)
        z = xv - jnp.sum(xv, axis=1, keepdims=True) * (1.0 / D)
        var = jnp.sum(z * z, axis=1, keepdims=True) * (1.0 / D)
        var = jnp.broadcast_to(var, (xv.shape[0], 128))
        if chain:
            last['ln'] = var
        size = _pow2_sqrt(jnp.maximum(var, TINY))
        g = _pow2_inv(size)
        u = jnp.concatenate([z[:, _tile(j)] * g for j in range(8)], axis=1)
        return u, lax.rsqrt(var + EPS) * size

    def ln1(base, n, r):
        ua_, sa = ln(x[pl.ds(pl.multiple_of(base + r, n), n), :])
        ub, sb = ln(x[pl.ds(pl.multiple_of(base + HM + r, n), n), :])
        for i, val in enumerate(_a_sums(ua_[:, :512], ua_[:, 512:], ub[:, :512], ub[:, 512:])):
            put(xs1, i, 0, slice(r, r + n), val)
        for r0, s in ((r, sa), (HM + r, sb)):
            s1[r0:r0 + n, :] = s
            sq[r0:r0 + n, :] = s * QSCALE
            sv[HALO + r0:HALO + r0 + n, :] = _pow2(s)
        return (sa + sb)[0:8]

    def ln2(half, r, chain):
        rows = slice(half * HM + r, half * HM + r + 16)
        u, s = ln(xt[rows, :], chain)
        (put_b if half else put_a)(xs2, r, u)
        p = s * s * stat[0:1, :] + stat[1:2, :]
        size = _pow2_sqrt(p)
        g = _pow2_inv(size)
        gh[rows, :] = g
        sg[rows, :] = s * g
        sh[rows, :] = size * size

    def qkv_dst(g, j, half):
        if g == 0:
            return q.at[j, pl.ds(half * HM, HM), :]
        return (k, v)[g - 1].at[j, pl.ds(HALO + half * HM, HM), :]

    def qkv_p1(g, c):
        sc = (sq if g == 0 else s1)[0:HM, :]
        sc = jnp.concatenate([sc, sc], axis=1)
        md = P(mm, xs1, wq, c=g * 2 + c)

        def out(j, half, val):
            for t in range(2):
                qkv_dst(g, c * 2 + j + t, half)[...] = val[:, _tile(t)]
        m3 = md(M3)
        m5 = md(M5)
        out(4, 0, (m3 + m5) * sc)
        m1 = md(M1)
        out(4, 1, m1 + m3)
        acc = m1 - m5
        m4 = md(M4)
        out(0, 1, m4)
        out(0, 0, (acc + m4 + md(M7)) * sc)

    def qkv_p2(g, c):
        sc = (sq if g == 0 else s1)[HM:TM, :]
        m2 = mm(xs1, wq, M2, g * 2 + c)
        acc = []
        for t in range(2):
            l, r = qkv_dst(g, c * 2 + t, 1), qkv_dst(g, c * 2 + t + 4, 1)
            l[...] = (l[...] + m2[:, _tile(t)]) * sc
            acc.append(r[...] - m2[:, _tile(t)])
        m6 = mm(xs1, wq, M6, g * 2 + c)
        for t in range(2):
            qkv_dst(g, c * 2 + t + 4, 1)[...] = (acc[t] + m6[:, _tile(t)]) * sc

    def window(ref, lead, r):
        return [ref[lead + (pl.ds(HALO + r - DIL * w, 8), slice(None))] for w in range(W)]

    def qk8(r, first, chain):
        qs = [q[j, r:r + 8, :] for j in range(8)]
        if chain:
            qs = [after('qk', t) for t in qs]
        ks = [window(k, (j,), r) for j in range(8)]
        ls = []
        for w in range(W):
            p = _tree(jnp.add, [qs[j] * ks[j][w] for j in range(8)])
            p = (p + pltpu.roll(p, 64, 1)) + (pltpu.roll(p, 32, 1) + pltpu.roll(p, 96, 1))
            if r - DIL * w < 0:
                p = jnp.where(jnp.logical_and(first, sub + (r - DIL * w) < 0), NEG, p)
            ls.append(p)
        last['qk'] = ls[0]
        m = _tree(jnp.maximum, ls)
        es = [jnp.exp2(l - m) for l in ls]
        sc = _tree(jnp.maximum, window(sv, (), r))
        so[r:r + 8, :] = sc
        den = _tree(jnp.add, es)
        inv = pltpu.reciprocal(den, approx=True)
        inv = inv * (2.0 - den * inv) * _pow2_inv(sc)
        for w in range(W):
            pr[w, r:r + 8, :] = es[w] * inv
        return inv

    def pv8(r):
        ps = [pr[w, r:r + 8, :] for w in range(W)]
        return jnp.concatenate(
            [_tree(jnp.add, [a * b for a, b in zip(ps, window(v, (j,), r))]) for j in range(8)], axis=1)

    def pv16(half, r):
        r0 = half * HM + r
        (put_b if half else put_a)(os_, r, jnp.concatenate([pv8(r0), pv8(r0 + 8)], axis=0))

    def v_first(first):
        for j in range(8):
            v0 = jnp.broadcast_to(v[j, HALO:HALO + 1, :], (HALO, 128))
            v[j, 0:HALO, :] = jnp.where(first, v0, v[j, 0:HALO, :])

    def halo_save():
        sv[0:HALO, :] = sv[TM:TM + HALO, :]
        for j in range(8):
            k[j, 0:HALO, :] = k[j, TM:TM + HALO, :]
            v[j, 0:HALO, :] = v[j, TM:TM + HALO, :]

    def acc_x(base, half, j, val):
        rows = pl.ds(pl.multiple_of(base + half * HM, HM), HM)
        sc = so[half * HM:(half + 1) * HM, :]
        for t in range(2):
            r = x[rows, _tile(j + t)] + val[:, _tile(t)] * sc
            xt[half * HM:(half + 1) * HM, _tile(j + t)] = r
            if half:
                x[rows, _tile(j + t)] = r

    def wo_p1(base, c):
        cols = _tile(c * 2, 2)
        m3 = mm(os_, wo, M3, c)
        part[2, :, cols] = m3
        m5 = mm(os_, wo, M5, c)
        part[0, :, cols] = m5
        acc_x(base, 0, 4 + c * 2, m3 + m5)

    def wo_p2(base, c):
        cols = _tile(c * 2, 2)
        m1 = mm(os_, wo, M1, c)
        part[2, :, cols] = part[2, :, cols] + m1
        acc = m1 - part[0, :, cols]
        m4 = mm(os_, wo, M4, c)
        part[1, :, cols] = m4
        acc_x(base, 0, c * 2, acc + m4 + mm(os_, wo, M7, c))

    def wo_p3(base, c):
        cols = _tile(c * 2, 2)
        m2 = mm(os_, wo, M2, c)
        acc_x(base, 1, c * 2, part[1, :, cols] + m2)
        acc = part[2, :, cols] - m2
        acc_x(base, 1, 4 + c * 2, acc + mm(os_, wo, M6, c))

    def w1_pre(c):
        pre[0, :, _tile(c * 2, 2)] = mm(xs2, w1, M3, c)
        pre[1, :, _tile(c * 2, 2)] = mm(xs2, w1, M5, c)

    def w1_chunk(c):
        md = P(mm, xs2, w1, c=c)

        def act(z, half, side):
            rows = slice(half * HM, (half + 1) * HM)
            out = []
            for t in range(2):
                b = b1[0:1, _tile(side * 14 + c * 2 + t)]
                y = jnp.maximum(z[:, _tile(t)] * sg[rows, :] + gh[rows, :] * b, 0.0)
                out.append(y * y)
            return jnp.concatenate(out, axis=1)

        def out(i, val):
            put(hs, i, c * 2, slice(0, HM), val)
        if c < NPRE:
            m3, m5 = pre[0, :, _tile(c * 2, 2)], pre[1, :, _tile(c * 2, 2)]
        else:
            m3, m5 = md(M3), md(M5)
        h12 = act(m3 + m5, 0, 1)
        m4 = md(M4)
        acc1 = m4 - m5
        m2 = md(M2)
        h21 = act(m4 + m2, 1, 0)
        acc2 = m3 - m2
        m1 = md(M1)
        acc1, acc2 = acc1 + m1, acc2 + m1
        h22 = act(acc2 + md(M6), 1, 1)
        out(M2, h21 + h22)
        out(M4, h22)
        out(M7, h12 - h22)
        h11 = act(acc1 + md(M7), 0, 0)
        out(M1, h11 + h22)
        out(M3, h11)
        out(M5, h11 + h12)
        out(M6, h21 - h11)

    def fin(res, base, slot, half, c, side, val, sc):
        rows = pl.ds(pl.multiple_of(base + half * HM, HM), HM)
        for t in range(2):
            cols = _tile(side * 4 + c * 2 + t)
            r = res(rows, cols) + val[:, _tile(t)] * sc + b2[0:1, cols]
            x[rows, cols] = r
            ostage[slot, half, :, cols] = r.astype(bf16)

    def w2_p1(base, slot, c):
        done = P(fin, lambda rows, cols: xt[0:HM, cols], base, slot, 0, c, sc=sh[0:HM, :])
        m3 = mm(hs, w2, M3, c)
        m5 = mm(hs, w2, M5, c)
        done(1, m3 + m5)
        m1 = mm(hs, w2, M1, c)
        carry[1, :, _tile(2 * c, 2)] = m1 + m3
        acc = m1 - m5
        m4 = mm(hs, w2, M4, c)
        carry[0, :, _tile(2 * c, 2)] = m4
        done(0, acc + m4 + mm(hs, w2, M7, c))
        if c == 1:
            carry[2, :, 0:128] = sh[HM:TM, :]

    def w2_p2(base, slot, c):
        done = P(fin, lambda rows, cols: x[rows, cols], base, slot, 1, c, sc=carry[2, :, 0:128])
        m2 = mm(hs, w2, M2, c)
        done(0, carry[0, :, _tile(2 * c, 2)] + m2)
        acc = carry[1, :, _tile(2 * c, 2)] - m2
        done(1, acc + mm(hs, w2, M6, c))

    def put_sums(dst, rows, t, blocks):
        bits = []
        for i, s in enumerate(_b_sums(*blocks)):
            put(dst, i, t, rows, s)
            if i in COV:
                bits += [pltpu.bitcast(s[a:a + 8, 0:128], i32) for a in range(0, s.shape[0], CS)]
        return pltpu.bitcast(_tree(jnp.bitwise_or, bits), f32)

    def permuted(r, n, g):
        lane = lax.broadcasted_iota(i32, (n // 2, 128), 1)
        src = ((lane & 31) << 2) | (lane >> 5)
        ts = [pltpu.bitcast(wqkv_raw[r:r + n, _tile(g * 8 + j)], u32) for j in range(8)]
        ts = [pltpu.roll(t, 4 * j, 1) if j else t for j, t in enumerate(ts)]
        ts = _skew_select(ts, lane, 4)
        return [pltpu.bitcast(jnp.take_along_axis(t, (src + 4 * j) & 127, axis=1), bf16).astype(f32)
                for j, t in enumerate(ts)]

    def prep_qkv(g, n, lo, hi):
        for r in range(lo, hi, n):
            top, bot = permuted(r, n, g), permuted(512 + r, n, g)
            out = [put_sums(wq, slice(r, r + n), g * 4 + t, (top[t], top[t + 4], bot[t], bot[t + 4]))
                   for t in range(4)]
        return _tree(jnp.maximum, out)

    def prep_wo(t, d3, h1):
        blk = {}
        for side in range(2):
            for d4 in range(2):
                for h0 in range(2):
                    src = []
                    for hh in range(8):
                        r = hh * 128 + h1 * 64 + h0 * 32 + d4 * 16
                        val = wo_raw[r:r + 16, _tile(t + 4 * side)].astype(f32)[8 * d3:8 * d3 + 8]
                        src.append(pltpu.roll(val, hh, 0) if hh else val)
                    for dl, val in enumerate(_skew_select(src, sub, 1)):
                        blk[d4, side, h0, dl] = pltpu.roll(val, 8 - dl, 0) if dl else val
        out = []
        for dl in range(8):
            r = d3 * 256 + dl * 32 + h1 * 16
            out.append(put_sums(wo, slice(r, r + 16), t,
                                [jnp.concatenate([blk[d4, side, 0, dl], blk[d4, side, 1, dl]], axis=0)
                                 for d4 in range(2) for side in range(2)]))
        return _tree(jnp.maximum, out)

    def prep_w1(c):
        es = []
        for t in (2 * c, 2 * c + 1):
            for r in range(0, 512, 64):
                blocks = [w1_raw[rr:rr + 64, _tile(j)].astype(f32) for rr in (r, 512 + r) for j in (t, t + 14)]
                put_sums(w1, slice(r, r + 64), t, blocks)
                if c == 0:
                    e = _tree(jnp.add, [y * y for y in blocks])
                    es.append(_tree(jnp.add, [e[a:a + 8] for a in range(0, 64, 8)]))
        if c == 0:
            tot = jnp.sum(jnp.sum(_tree(jnp.add, es), axis=1, keepdims=True), axis=0, keepdims=True)
            stat[0:1, :] = jnp.broadcast_to(tot * (1.0 / 512), (1, 128))
            bb = b1[0:1, :]
            stat[1:2, :] = jnp.broadcast_to(jnp.sum(bb * bb, axis=1, keepdims=True) * (1.0 / F) + TINY, (1, 128))

    def prep_w2(t, r):
        return put_sums(w2, slice(r, r + 64), t,
                        [w2_raw[rr:rr + 64, _tile(j)].astype(f32) for rr in (r, HF + r) for j in (t, t + 4)])

    def prep_w1_part(t, r):
        return put_sums(w1, slice(r, r + 64), t,
                        [w1_raw[rr:rr + 64, _tile(j)].astype(f32) for rr in (r, 512 + r) for j in (t, t + 14)])

    def cvt_x(r):
        val = xin[r:r + 64, :].astype(f32)
        x[r:r + 64, :] = val
        return _tree(jnp.add, [val[a:a + 8, 0:128] for a in range(0, 64, 8)])

    def dma(src, dst, block, i):
        return pltpu.make_async_copy(src.at[block], dst.at[block], isem.at[i])

    full = slice(None)
    cp_x0 = [[dma(x_hbm, xin, (pl.ds(half * HM + r, 128), full), 10 + 1024 // RQ + 2 * (r // 128) + half)
              for half in range(2)] for r in range(0, HM, 128)]
    cp_x1 = dma(x_hbm, xin, (pl.ds(TM, S - TM), full), 1)
    cp_k, cp_v = (dma(wqkv_hbm, wqkv_raw, (full, pl.ds(g * D, D)), 1 + g) for g in (1, 2))
    cp_wo = dma(wo_hbm, wo_raw, (full, full), 4)
    cp_w2 = dma(w2_hbm, w2_raw, (full, full), 5)
    cp_w1 = dma(w1_hbm, w1_raw, (full, full), 6)
    cp_q = [[dma(wqkv_hbm, wqkv_raw, (pl.ds(s * 512 + n * RQ, RQ), pl.ds(0, D)), 10 + 2 * n + s) for s in range(2)]
            for n in range(512 // RQ)]

    def step(t, peeled):
        base = (t % NT) * TM
        pbase = ((t + NT - 1) % NT) * TM
        nbase = ((t + 1) % NT) * TM
        slot = t % 2
        first = t % NT == 0
        clock[0] = 0
        last.clear()
        qk_items = [P(qk8, r, first, not peeled) for r in range(0, TM, 8)]
        ln1_items = [P(ln1, nbase, 16, r) for r in range(0, HM, 16)]

        def two(f, *a):
            for c in range(2):
                f(*a, c)
        if peeled:
            for cp in [*sum(cp_x0 + cp_q, []), cp_k, cp_v, cp_wo, cp_w1, cp_w2, cp_x1]:
                cp.start()
            sv[0:HALO, :] = jnp.zeros((HALO, 128), f32)
            k[:, 0:HALO, :] = jnp.zeros((8, HALO, 128), f32)
            v[:, 0:HALO, :] = jnp.zeros((8, HALO, 128), f32)
            b1[0:1, :] = b1_ref[...].astype(f32).reshape(1, F)
            b2[0:1, :] = b2_ref[...].astype(f32).reshape(1, D)
            ostage[slot, 1] = jnp.zeros((HM, D), bf16)
            for r, cps in zip(range(0, HM, 128), cp_x0):
                for cp in cps:
                    cp.wait()
                for rr in (r, r + 64, HM + r, HM + r + 64):
                    cvt_x(rr)
                ln1(base, 128, r)
            for n, cps in enumerate(cp_q):
                for cp in cps:
                    cp.wait()
                prep_qkv(0, 128, n * RQ, (n + 1) * RQ)
            plan(QKF, qk_items)
            qkv_p1(0, 0)
            qkv_p2(0, 0)
            cp_k.wait()
            if TK:
                plan(TK, [P(prep_qkv, 1, NK, r, r + NK) for r in range(0, 512, NK)])
            else:
                prep_qkv(1, 128, 0, 512)
            qkv_p1(0, 1)
            qkv_p2(0, 1)
            qkv_p1(1, 0)
            cp_v.wait()
            cp_wo.wait()
            if TV:
                plan(TV, [P(prep_qkv, 2, NK, r, r + NK) for r in range(0, 512, NK)])
            else:
                prep_qkv(2, 128, 0, 512)
            items = [P(prep_wo, tt, d3, h1) for tt in range(4) for d3 in range(2) for h1 in range(2)]
            if TO:
                plan(TO, items)
            else:
                for f in items:
                    f()
            qkv_p1(1, 1)
        else:
            plan(QK, qk_items)
            plan(L1, ln1_items)
            two(qkv_p1, 0)
            two(qkv_p1, 1)
            two(qkv_p2, 0)
        two(qkv_p2, 1)
        two(qkv_p1, 2)
        v_first(first)
        two(qkv_p2, 2)
        flush(QK[1])
        for half in range(2):
            for r in range(0, HM, 16):
                pv16(half, r)
        if not peeled:
            w2_p2(pbase, slot, 0)
        two(wo_p1, base)
        halo_save()
        if peeled:
            cp_w1.wait()
            for c in range(N0):
                prep_w1(c)
            plan((clock[0] + TA[0], clock[0] + TA[1]),
                 [P(prep_w1_part, tt, r) for tt in range(2 * N0, 14) for r in range(0, 512, 64)])
        two(wo_p2, base)
        two(wo_p3, base)
        if not peeled:
            w2_p2(pbase, slot, 1)
        for half in range(2):
            for r in range(0, HM, 16):
                ln2(half, r, not peeled)
        for c in range(NPRE):
            if peeled:
                flush(clock[0] + TA[2])
            w1_pre(c)
        for c in range(7):
            if peeled and c == CB:
                flush(float("inf"))
                cp_w2.wait()
                cp_x1.wait()
                plan((clock[0] + T2[0], clock[0] + T2[1]),
                     [P(prep_w2, tt, r) for tt in range(4) for r in range(0, HF, 64)])
            w1_chunk(c)
        if peeled:
            flush(float("inf"))
            for r in range(TM, 2 * TM, 64):
                cvt_x(r)
            late = (clock[0] + 1000, clock[0] + 16000)
            plan(late, ln1_items)
            plan(late, [P(cvt_x, r) for r in range(2 * TM, S, 64)])
        two(w2_p1, base, slot)
        flush(float("inf"))

    def out_copies(t):
        return [pltpu.make_async_copy(
            ostage.at[t % 2, half],
            out_hbm.at[pl.ds(pl.multiple_of(((t + (NT - 1) * half) % NT) * TM + half * HM, HM), HM), :],
            osem.at[half]) for half in range(2)]

    step(0, True)

    def body(t, c):
        cps = out_copies(t - 1)
        for cp in cps:
            cp.start()
        step(t, False)
        for cp in cps:
            cp.wait()
        return c

    if MODE != 'first':
        lax.fori_loop(1, 2 * NT, body, 0)
    cps = out_copies(2 * NT - 1)
    for cp in cps:
        cp.start()
    for c in range(2):
        w2_p2(S - TM, 0, c)
    for cp in cps:
        cp.wait()
    last = out_copies(2 * NT)[1]
    last.start()
    last.wait()


@jax.jit
def pallas_interleave_layers__sliding_local_dilated__dense_activation_squared_relu__prompt_kernel(A_x, A_wqkv, A_wo, B_x, B_w1, B_b1, B_w2, B_b2):
    del B_x
    hbm = pl.BlockSpec(memory_space=pl.ANY)
    vmem = pl.BlockSpec(memory_space=pltpu.VMEM)
    V = pltpu.VMEM
    out = pl.pallas_call(
        _kernel,
        in_specs=[hbm, hbm, hbm, hbm, vmem, hbm, vmem],
        out_specs=hbm,
        out_shape=jax.ShapeDtypeStruct((S, D), bf16),
        scratch_shapes=[
            V((2, 2, HM, D), bf16), V((S, D), bf16), V((S, D), f32),
            V((D, 3 * D), bf16), V((D, D), bf16), V((D, F), bf16), V((F, D), bf16),
            V((7, 12, 512, 128), bf16), V((7, 4, 512, 128), bf16),
            V((7, 14, 512, 128), bf16), V((7, 4, HF, 128), bf16),
            V((7, 4, HM, 128), bf16), V((7, 4, HM, 128), bf16), V((7, 4, HM, 128), bf16), V((7, 14, HM, 128), bf16),
            V((8, TM, 128), f32), V((8, TM + HALO, 128), f32), V((8, TM + HALO, 128), f32), V((W, TM, 128), f32),
            V((HM, D), f32), V((TM, D), f32),
            V((3, HM, 512), f32), V((2, HM, 256 * NPRE), f32), V((3, HM, 512), f32),
            V((TM, 128), f32), V((TM, 128), f32), V((TM + HALO, 128), f32), V((TM, 128), f32),
            V((TM, 128), f32), V((TM, 128), f32), V((TM, 128), f32),
            V((8, F), f32), V((8, D), f32), V((8, 128), f32),
            pltpu.SemaphoreType.DMA((14 + 1024 // RQ,)), pltpu.SemaphoreType.DMA((2,)),
        ],
        compiler_params=pltpu.CompilerParams(vmem_limit_bytes=127 * 1024 * 1024),
    )(A_x.reshape(S, D), A_wqkv, A_wo, B_w1, B_b1, B_w2, B_b2)
    return out.reshape(1, S, D)
```

```python
import functools

import jax
import jax.numpy as jnp
import numpy as np
from jax import lax
import jax.experimental.pallas as pl
import jax.experimental.pallas.tpu as pltpu

S, D, F = 2048, 1024, 3584
DH, W, DIL = 32, 8, 2
TM = 512
HM = TM // 2
HF = F // 2
NT = S // TM
HALO = 16
EPS = 1e-5
TINY = 1e-30
QSCALE = float(DH ** -0.5 * np.log2(np.e))
NEG = float(-1e9 * np.log2(np.e))
MODE = 'all'
N0 = 1
COV = (3, 6)
CS = 16
TO = (14500, 22900)
TK = (3900, 6600)
TV = (10000, 13800)
NK = 64
TA = (2000, 14000, 1100)
CB = 2
T2 = (500, 15000)
NPRE = 4
RQ = 256
QK = (10850, 21500)
QKF = (14000, 21400)
L1 = (42000, 59000)
f32, bf16, u32, i32 = jnp.float32, jnp.bfloat16, jnp.uint32, jnp.int32
P = functools.partial


def _tree(op, xs):
    xs = list(xs)
    while len(xs) > 1:
        xs = [op(xs[i], xs[i + 1]) if i + 1 < len(xs) else xs[i] for i in range(0, len(xs), 2)]
    return xs[0]


def _a_sums(a11, a12, a21, a22):
    return (a11 + a22, a21 + a22, a11, a22, a11 + a12, a21 - a11, a12 - a22)


def _b_sums(b11, b12, b21, b22):
    return (b11 + b22, b11, b12 - b22, b21 - b11, b22, b11 + b12, b21 + b22)


M1, M2, M3, M4, M5, M6, M7 = range(7)


def _tile(j, n=1):
    if isinstance(j, int):
        return slice(j * 128, (j + n) * 128)
    return pl.ds(pl.multiple_of(j * 128, 128), n * 128)


def _pow2(s):
    return pltpu.bitcast((pltpu.bitcast(s, i32) + 0x007FFFFF) & 0x7F800000, f32)


def _pow2_inv(s):
    return pltpu.bitcast(0x7F000000 - pltpu.bitcast(s, i32), f32)


def _pow2_sqrt(s):
    half = lax.shift_right_logical(pltpu.bitcast(s, i32), 1)
    return pltpu.bitcast((half + 0x1FC00000) & 0x7F800000, f32)


def _skew_select(ts, index, unit):
    ts = [ts[-i % 8] for i in range(8)]
    for b in (1, 2, 4):
        take = (index & (unit * b)) != 0
        ts = [jnp.where(take, ts[(i - b) % 8], ts[i]) for i in range(8)]
    return ts


def _kernel(x_hbm, wqkv_hbm, wo_hbm, w1_hbm, b1_ref, w2_hbm, b2_ref, out_hbm,
            ostage, xin, x, wqkv_raw, wo_raw, w1_raw, w2_raw,
            wq, wo, w1, w2, xs1, xs2, os_, hs, q, k, v, pr, ua, xt, part, pre, carry,
            s1, sq, sv, so, sg, gh, sh, b1, b2, stat, isem, osem):
    sub = lax.broadcasted_iota(i32, (8, 128), 0)

    clock = [0]
    queue = []

    def never(shape, dtype):
        return jnp.broadcast_to(jnp.abs(b2[0:1, 0:128]), shape).astype(dtype) < 0

    def plan(window, items):
        lo, hi = window
        queue.extend((lo + (hi - lo) * (n + 1) / len(items), f) for n, f in enumerate(items))
        queue.sort(key=lambda e: e[0])

    def flush(until):
        vals = []
        while queue and queue[0][0] <= until:
            vals.append(queue.pop(0)[1]())
        return vals

    def tie(operand, r, until):
        vals = flush(until)
        if not vals:
            return operand
        d = _tree(jnp.add, vals)
        d = jnp.concatenate([d, d], axis=0).astype(bf16)
        parts = [operand[:r], jnp.where(never((16, 128), bf16), d, operand[r:r + 16]), operand[r + 16:]]
        return jnp.concatenate([p for p in parts if p.shape[0]], axis=0)

    last = {}

    def after(key, val):
        if key not in last:
            return val
        return jnp.where(never(val.shape, f32), last[key], val)

    def mm(a_ref, w_ref, i, c):
        kt = a_ref.shape[1]
        ls = [a_ref[i, t] for t in range(kt)]
        rs = [w_ref[i, 2 * c + n] for n in range(2)]
        t0 = clock[0]
        clock[0] = t0 + 128 * kt
        if kt == 4:
            out = []
            for n in range(2):
                l0 = ls[0]
                for r in range(0, HM, 64):
                    l0 = tie(l0, r, t0 + n * 256 + r + 63)
                out.append(jnp.dot(jnp.concatenate([l0] + ls[1:], axis=1), rs[n], preferred_element_type=f32))
            return jnp.concatenate(out, axis=1)
        for g in range(kt // 4 + 1):
            for r in range(0, HM, 64):
                ls[4 * g] = tie(ls[4 * g], r, t0 + g * 448 + r + 63)
        return jnp.dot(jnp.concatenate(ls, axis=1), jnp.concatenate(rs, axis=1), preferred_element_type=f32)

    def put(dst, i, t0, rows, val):
        for t in range(val.shape[1] // 128):
            dst[i, t0 + t, rows, :] = val[:, _tile(t)].astype(bf16)

    def put_a(dst, r, ua_):
        ua[r:r + 16, :] = ua_
        put(dst, M3, 0, slice(r, r + 16), ua_[:, :512])
        put(dst, M5, 0, slice(r, r + 16), ua_[:, :512] + ua_[:, 512:])

    def put_b(dst, r, ub):
        ss = _a_sums(ua[r:r + 16, :512], ua[r:r + 16, 512:], ub[:, :512], ub[:, 512:])
        for i in (M1, M2, M4, M6, M7):
            put(dst, i, 0, slice(r, r + 16), ss[i])

    def ln(xv, chain=False):
        if chain:
            xv = jnp.concatenate([after('ln', xv[:, :128]), xv[:, 128:]], axis=1)
        z = xv - jnp.sum(xv, axis=1, keepdims=True) * (1.0 / D)
        var = jnp.sum(z * z, axis=1, keepdims=True) * (1.0 / D)
        var = jnp.broadcast_to(var, (xv.shape[0], 128))
        if chain:
            last['ln'] = var
        size = _pow2_sqrt(jnp.maximum(var, TINY))
        g = _pow2_inv(size)
        u = jnp.concatenate([z[:, _tile(j)] * g for j in range(8)], axis=1)
        return u, lax.rsqrt(var + EPS) * size

    def ln1(base, n, r):
        ua_, sa = ln(x[pl.ds(pl.multiple_of(base + r, n), n), :])
        ub, sb = ln(x[pl.ds(pl.multiple_of(base + HM + r, n), n), :])
        for i, val in enumerate(_a_sums(ua_[:, :512], ua_[:, 512:], ub[:, :512], ub[:, 512:])):
            put(xs1, i, 0, slice(r, r + n), val)
        for r0, s in ((r, sa), (HM + r, sb)):
            s1[r0:r0 + n, :] = s
            sq[r0:r0 + n, :] = s * QSCALE
            sv[HALO + r0:HALO + r0 + n, :] = _pow2(s)
        return (sa + sb)[0:8]

    def ln2(half, r, chain):
        rows = slice(half * HM + r, half * HM + r + 16)
        u, s = ln(xt[rows, :], chain)
        (put_b if half else put_a)(xs2, r, u)
        p = s * s * stat[0:1, :] + stat[1:2, :]
        size = _pow2_sqrt(p)
        g = _pow2_inv(size)
        gh[rows, :] = g
        sg[rows, :] = s * g
        sh[rows, :] = size * size

    def qkv_dst(g, j, half):
        if g == 0:
            return q.at[j, pl.ds(half * HM, HM), :]
        return (k, v)[g - 1].at[j, pl.ds(HALO + half * HM, HM), :]

    def qkv_p1(g, c):
        sc = (sq if g == 0 else s1)[0:HM, :]
        sc = jnp.concatenate([sc, sc], axis=1)
        md = P(mm, xs1, wq, c=g * 2 + c)

        def out(j, half, val):
            for t in range(2):
                qkv_dst(g, c * 2 + j + t, half)[...] = val[:, _tile(t)]
        m3 = md(M3)
        m5 = md(M5)
        out(4, 0, (m3 + m5) * sc)
        m1 = md(M1)
        out(4, 1, m1 + m3)
        acc = m1 - m5
        m4 = md(M4)
        out(0, 1, m4)
        out(0, 0, (acc + m4 + md(M7)) * sc)

    def qkv_p2(g, c):
        sc = (sq if g == 0 else s1)[HM:TM, :]
        m2 = mm(xs1, wq, M2, g * 2 + c)
        acc = []
        for t in range(2):
            l, r = qkv_dst(g, c * 2 + t, 1), qkv_dst(g, c * 2 + t + 4, 1)
            l[...] = (l[...] + m2[:, _tile(t)]) * sc
            acc.append(r[...] - m2[:, _tile(t)])
        m6 = mm(xs1, wq, M6, g * 2 + c)
        for t in range(2):
            qkv_dst(g, c * 2 + t + 4, 1)[...] = (acc[t] + m6[:, _tile(t)]) * sc

    def window(ref, lead, r):
        return [ref[lead + (pl.ds(HALO + r - DIL * w, 8), slice(None))] for w in range(W)]

    def qk8(r, first, chain):
        qs = [q[j, r:r + 8, :] for j in range(8)]
        if chain:
            qs = [after('qk', t) for t in qs]
        ks = [window(k, (j,), r) for j in range(8)]
        ls = []
        for w in range(W):
            p = _tree(jnp.add, [qs[j] * ks[j][w] for j in range(8)])
            p = (p + pltpu.roll(p, 64, 1)) + (pltpu.roll(p, 32, 1) + pltpu.roll(p, 96, 1))
            if r - DIL * w < 0:
                p = jnp.where(jnp.logical_and(first, sub + (r - DIL * w) < 0), NEG, p)
            ls.append(p)
        last['qk'] = ls[0]
        m = _tree(jnp.maximum, ls)
        es = [jnp.exp2(l - m) for l in ls]
        sc = _tree(jnp.maximum, window(sv, (), r))
        so[r:r + 8, :] = sc
        den = _tree(jnp.add, es)
        inv = pltpu.reciprocal(den, approx=True)
        inv = inv * (2.0 - den * inv) * _pow2_inv(sc)
        for w in range(W):
            pr[w, r:r + 8, :] = es[w] * inv
        return inv

    def pv8(r):
        ps = [pr[w, r:r + 8, :] for w in range(W)]
        return jnp.concatenate(
            [_tree(jnp.add, [a * b for a, b in zip(ps, window(v, (j,), r))]) for j in range(8)], axis=1)

    def pv16(half, r):
        r0 = half * HM + r
        (put_b if half else put_a)(os_, r, jnp.concatenate([pv8(r0), pv8(r0 + 8)], axis=0))

    def v_first(first):
        for j in range(8):
            v0 = jnp.broadcast_to(v[j, HALO:HALO + 1, :], (HALO, 128))
            v[j, 0:HALO, :] = jnp.where(first, v0, v[j, 0:HALO, :])

    def halo_save():
        sv[0:HALO, :] = sv[TM:TM + HALO, :]
        for j in range(8):
            k[j, 0:HALO, :] = k[j, TM:TM + HALO, :]
            v[j, 0:HALO, :] = v[j, TM:TM + HALO, :]

    def acc_x(base, half, j, val):
        rows = pl.ds(pl.multiple_of(base + half * HM, HM), HM)
        sc = so[half * HM:(half + 1) * HM, :]
        for t in range(2):
            r = x[rows, _tile(j + t)] + val[:, _tile(t)] * sc
            xt[half * HM:(half + 1) * HM, _tile(j + t)] = r
            if half:
                x[rows, _tile(j + t)] = r

    def wo_p1(base, c):
        cols = _tile(c * 2, 2)
        m3 = mm(os_, wo, M3, c)
        part[2, :, cols] = m3
        m5 = mm(os_, wo, M5, c)
        part[0, :, cols] = m5
        acc_x(base, 0, 4 + c * 2, m3 + m5)

    def wo_p2(base, c):
        cols = _tile(c * 2, 2)
        m1 = mm(os_, wo, M1, c)
        part[2, :, cols] = part[2, :, cols] + m1
        acc = m1 - part[0, :, cols]
        m4 = mm(os_, wo, M4, c)
        part[1, :, cols] = m4
        acc_x(base, 0, c * 2, acc + m4 + mm(os_, wo, M7, c))

    def wo_p3(base, c):
        cols = _tile(c * 2, 2)
        m2 = mm(os_, wo, M2, c)
        acc_x(base, 1, c * 2, part[1, :, cols] + m2)
        acc = part[2, :, cols] - m2
        acc_x(base, 1, 4 + c * 2, acc + mm(os_, wo, M6, c))

    def w1_pre(c):
        pre[0, :, _tile(c * 2, 2)] = mm(xs2, w1, M3, c)
        pre[1, :, _tile(c * 2, 2)] = mm(xs2, w1, M5, c)

    def w1_chunk(c):
        md = P(mm, xs2, w1, c=c)

        def act(z, half, side):
            rows = slice(half * HM, (half + 1) * HM)
            out = []
            for t in range(2):
                b = b1[0:1, _tile(side * 14 + c * 2 + t)]
                y = jnp.maximum(z[:, _tile(t)] * sg[rows, :] + gh[rows, :] * b, 0.0)
                out.append(y * y)
            return jnp.concatenate(out, axis=1)

        def out(i, val):
            put(hs, i, c * 2, slice(0, HM), val)
        if c < NPRE:
            m3, m5 = pre[0, :, _tile(c * 2, 2)], pre[1, :, _tile(c * 2, 2)]
        else:
            m3, m5 = md(M3), md(M5)
        h12 = act(m3 + m5, 0, 1)
        m4 = md(M4)
        acc1 = m4 - m5
        m2 = md(M2)
        h21 = act(m4 + m2, 1, 0)
        acc2 = m3 - m2
        m1 = md(M1)
        acc1, acc2 = acc1 + m1, acc2 + m1
        h22 = act(acc2 + md(M6), 1, 1)
        out(M2, h21 + h22)
        out(M4, h22)
        out(M7, h12 - h22)
        h11 = act(acc1 + md(M7), 0, 0)
        out(M1, h11 + h22)
        out(M3, h11)
        out(M5, h11 + h12)
        out(M6, h21 - h11)

    def fin(res, base, slot, half, c, side, val, sc):
        rows = pl.ds(pl.multiple_of(base + half * HM, HM), HM)
        for t in range(2):
            cols = _tile(side * 4 + c * 2 + t)
            r = res(rows, cols) + val[:, _tile(t)] * sc + b2[0:8, cols][0:1]
            x[rows, cols] = r
            ostage[slot, half, :, cols] = r.astype(bf16)

    def w2_p1(base, slot, c):
        done = P(fin, lambda rows, cols: xt[0:HM, cols], base, slot, 0, c, sc=sh[0:HM, :])
        m3 = mm(hs, w2, M3, c)
        m5 = mm(hs, w2, M5, c)
        done(1, m3 + m5)
        m1 = mm(hs, w2, M1, c)
        carry[1, :, _tile(2 * c, 2)] = m1 + m3
        acc = m1 - m5
        m4 = mm(hs, w2, M4, c)
        carry[0, :, _tile(2 * c, 2)] = m4
        done(0, acc + m4 + mm(hs, w2, M7, c))
        if c == 1:
            carry[2, :, 0:128] = sh[HM:TM, :]

    def w2_p2(base, slot, c):
        done = P(fin, lambda rows, cols: x[rows, cols], base, slot, 1, c, sc=carry[2, :, 0:128])
        m2 = mm(hs, w2, M2, c)
        done(0, carry[0, :, _tile(2 * c, 2)] + m2)
        acc = carry[1, :, _tile(2 * c, 2)] - m2
        done(1, acc + mm(hs, w2, M6, c))

    def put_sums(dst, rows, t, blocks):
        bits = []
        for i, s in enumerate(_b_sums(*blocks)):
            put(dst, i, t, rows, s)
            if i in COV:
                bits += [pltpu.bitcast(s[a:a + 8, 0:128], i32) for a in range(0, s.shape[0], CS)]
        return pltpu.bitcast(_tree(jnp.bitwise_or, bits), f32)

    def permuted(r, n, g):
        lane = lax.broadcasted_iota(i32, (n // 2, 128), 1)
        src = ((lane & 31) << 2) | (lane >> 5)
        ts = [pltpu.bitcast(wqkv_raw[r:r + n, _tile(g * 8 + j)], u32) for j in range(8)]
        ts = [pltpu.roll(t, 4 * j, 1) if j else t for j, t in enumerate(ts)]
        ts = _skew_select(ts, lane, 4)
        return [pltpu.bitcast(jnp.take_along_axis(t, (src + 4 * j) & 127, axis=1), bf16).astype(f32)
                for j, t in enumerate(ts)]

    def prep_qkv(g, n, lo, hi):
        for r in range(lo, hi, n):
            top, bot = permuted(r, n, g), permuted(512 + r, n, g)
            out = [put_sums(wq, slice(r, r + n), g * 4 + t, (top[t], top[t + 4], bot[t], bot[t + 4]))
                   for t in range(4)]
        return _tree(jnp.maximum, out)

    def prep_wo(t, d3, h1):
        blk = {}
        for side in range(2):
            for d4 in range(2):
                for h0 in range(2):
                    src = []
                    for hh in range(8):
                        r = hh * 128 + h1 * 64 + h0 * 32 + d4 * 16
                        val = wo_raw[r:r + 16, _tile(t + 4 * side)].astype(f32)[8 * d3:8 * d3 + 8]
                        src.append(pltpu.roll(val, hh, 0) if hh else val)
                    for dl, val in enumerate(_skew_select(src, sub, 1)):
                        blk[d4, side, h0, dl] = pltpu.roll(val, 8 - dl, 0) if dl else val
        out = []
        for dl in range(8):
            r = d3 * 256 + dl * 32 + h1 * 16
            out.append(put_sums(wo, slice(r, r + 16), t,
                                [jnp.concatenate([blk[d4, side, 0, dl], blk[d4, side, 1, dl]], axis=0)
                                 for d4 in range(2) for side in range(2)]))
        return _tree(jnp.maximum, out)

    def prep_w1(c):
        es = []
        for t in (2 * c, 2 * c + 1):
            for r in range(0, 512, 64):
                blocks = [w1_raw[rr:rr + 64, _tile(j)].astype(f32) for rr in (r, 512 + r) for j in (t, t + 14)]
                put_sums(w1, slice(r, r + 64), t, blocks)
                if c == 0:
                    e = _tree(jnp.add, [y * y for y in blocks])
                    es.append(_tree(jnp.add, [e[a:a + 8] for a in range(0, 64, 8)]))
        if c == 0:
            tot = jnp.sum(jnp.sum(_tree(jnp.add, es), axis=1, keepdims=True), axis=0, keepdims=True)
            stat[0:1, :] = jnp.broadcast_to(tot * (1.0 / 512), (1, 128))
            bb = b1[0:1, :]
            stat[1:2, :] = jnp.broadcast_to(jnp.sum(bb * bb, axis=1, keepdims=True) * (1.0 / F) + TINY, (1, 128))

    def prep_w2(t, r):
        return put_sums(w2, slice(r, r + 64), t,
                        [w2_raw[rr:rr + 64, _tile(j)].astype(f32) for rr in (r, HF + r) for j in (t, t + 4)])

    def prep_w1_part(t, r):
        return put_sums(w1, slice(r, r + 64), t,
                        [w1_raw[rr:rr + 64, _tile(j)].astype(f32) for rr in (r, 512 + r) for j in (t, t + 14)])

    def cvt_x(r):
        val = xin[r:r + 64, :].astype(f32)
        x[r:r + 64, :] = val
        return _tree(jnp.add, [val[a:a + 8, 0:128] for a in range(0, 64, 8)])

    def dma(src, dst, block, i):
        return pltpu.make_async_copy(src.at[block], dst.at[block], isem.at[i])

    full = slice(None)
    cp_x0 = [[dma(x_hbm, xin, (pl.ds(half * HM + r, 128), full), 10 + 1024 // RQ + 2 * (r // 128) + half)
              for half in range(2)] for r in range(0, HM, 128)]
    cp_x1 = dma(x_hbm, xin, (pl.ds(TM, S - TM), full), 1)
    cp_k, cp_v = (dma(wqkv_hbm, wqkv_raw, (full, pl.ds(g * D, D)), 1 + g) for g in (1, 2))
    cp_wo = dma(wo_hbm, wo_raw, (full, full), 4)
    cp_w2 = dma(w2_hbm, w2_raw, (full, full), 5)
    cp_w1 = dma(w1_hbm, w1_raw, (full, full), 6)
    cp_q = [[dma(wqkv_hbm, wqkv_raw, (pl.ds(s * 512 + n * RQ, RQ), pl.ds(0, D)), 10 + 2 * n + s) for s in range(2)]
            for n in range(512 // RQ)]

    def step(t, peeled):
        base = (t % NT) * TM
        pbase = ((t + NT - 1) % NT) * TM
        nbase = ((t + 1) % NT) * TM
        slot = t % 2
        first = t % NT == 0
        clock[0] = 0
        last.clear()
        qk_items = [P(qk8, r, first, not peeled) for r in range(0, TM, 8)]
        ln1_items = [P(ln1, nbase, 16, r) for r in range(0, HM, 16)]

        def two(f, *a):
            for c in range(2):
                f(*a, c)
        if peeled:
            for cp in [*sum(cp_x0 + cp_q, []), cp_k, cp_v, cp_wo, cp_w1, cp_w2, cp_x1]:
                cp.start()
            sv[0:HALO, :] = jnp.zeros((HALO, 128), f32)
            k[:, 0:HALO, :] = jnp.zeros((8, HALO, 128), f32)
            v[:, 0:HALO, :] = jnp.zeros((8, HALO, 128), f32)
            b1[0:1, :] = b1_ref[...].astype(f32).reshape(1, F)
            b2[0:1, :] = b2_ref[...].astype(f32).reshape(1, D)
            ostage[slot, 1] = jnp.zeros((HM, D), bf16)
            for r, cps in zip(range(0, HM, 128), cp_x0):
                for cp in cps:
                    cp.wait()
                for rr in (r, r + 64, HM + r, HM + r + 64):
                    cvt_x(rr)
                ln1(base, 128, r)
            for n, cps in enumerate(cp_q):
                for cp in cps:
                    cp.wait()
                prep_qkv(0, 128, n * RQ, (n + 1) * RQ)
            plan(QKF, qk_items)
            qkv_p1(0, 0)
            qkv_p2(0, 0)
            cp_k.wait()
            if TK:
                plan(TK, [P(prep_qkv, 1, NK, r, r + NK) for r in range(0, 512, NK)])
            else:
                prep_qkv(1, 128, 0, 512)
            qkv_p1(0, 1)
            qkv_p2(0, 1)
            qkv_p1(1, 0)
            cp_v.wait()
            cp_wo.wait()
            if TV:
                plan(TV, [P(prep_qkv, 2, NK, r, r + NK) for r in range(0, 512, NK)])
            else:
                prep_qkv(2, 128, 0, 512)
            items = [P(prep_wo, tt, d3, h1) for tt in range(4) for d3 in range(2) for h1 in range(2)]
            if TO:
                plan(TO, items)
            else:
                for f in items:
                    f()
            qkv_p1(1, 1)
        else:
            plan(QK, qk_items)
            plan(L1, ln1_items)
            two(qkv_p1, 0)
            two(qkv_p1, 1)
            two(qkv_p2, 0)
        two(qkv_p2, 1)
        two(qkv_p1, 2)
        v_first(first)
        two(qkv_p2, 2)
        flush(QK[1])
        for half in range(2):
            for r in range(0, HM, 16):
                pv16(half, r)
        if not peeled:
            w2_p2(pbase, slot, 0)
        two(wo_p1, base)
        halo_save()
        if peeled:
            cp_w1.wait()
            for c in range(N0):
                prep_w1(c)
            plan((clock[0] + TA[0], clock[0] + TA[1]),
                 [P(prep_w1_part, tt, r) for tt in range(2 * N0, 14) for r in range(0, 512, 64)])
        two(wo_p2, base)
        two(wo_p3, base)
        if not peeled:
            w2_p2(pbase, slot, 1)
        for half in range(2):
            for r in range(0, HM, 16):
                ln2(half, r, not peeled)
        for c in range(NPRE):
            if peeled:
                flush(clock[0] + TA[2])
            w1_pre(c)
        for c in range(7):
            if peeled and c == CB:
                flush(float("inf"))
                cp_w2.wait()
                cp_x1.wait()
                plan((clock[0] + T2[0], clock[0] + T2[1]),
                     [P(prep_w2, tt, r) for tt in range(4) for r in range(0, HF, 64)])
            w1_chunk(c)
        if peeled:
            flush(float("inf"))
            for r in range(TM, 2 * TM, 64):
                cvt_x(r)
            late = (clock[0] + 1000, clock[0] + 16000)
            plan(late, ln1_items)
            plan(late, [P(cvt_x, r) for r in range(2 * TM, S, 64)])
        two(w2_p1, base, slot)
        flush(float("inf"))

    def out_copies(t):
        return [pltpu.make_async_copy(
            ostage.at[t % 2, half],
            out_hbm.at[pl.ds(pl.multiple_of(((t + (NT - 1) * half) % NT) * TM + half * HM, HM), HM), :],
            osem.at[half]) for half in range(2)]

    step(0, True)

    def body(t, c):
        cps = out_copies(t - 1)
        for cp in cps:
            cp.start()
        step(t, False)
        for cp in cps:
            cp.wait()
        return c

    if MODE != 'first':
        lax.fori_loop(1, 2 * NT, body, 0)
    cps = out_copies(2 * NT - 1)
    for cp in cps:
        cp.start()
    lax.fori_loop(0, 2, lambda c, _: w2_p2(S - TM, 0, c), None)
    for cp in cps:
        cp.wait()
    last = out_copies(2 * NT)[1]
    last.start()
    last.wait()


@jax.jit
def pallas_interleave_layers__sliding_local_dilated__dense_activation_squared_relu__prompt_kernel(A_x, A_wqkv, A_wo, B_x, B_w1, B_b1, B_w2, B_b2):
    del B_x
    hbm = pl.BlockSpec(memory_space=pl.ANY)
    vmem = pl.BlockSpec(memory_space=pltpu.VMEM)
    V = pltpu.VMEM
    out = pl.pallas_call(
        _kernel,
        in_specs=[hbm, hbm, hbm, hbm, vmem, hbm, vmem],
        out_specs=hbm,
        out_shape=jax.ShapeDtypeStruct((S, D), bf16),
        scratch_shapes=[
            V((2, 2, HM, D), bf16), V((S, D), bf16), V((S, D), f32),
            V((D, 3 * D), bf16), V((D, D), bf16), V((D, F), bf16), V((F, D), bf16),
            V((7, 12, 512, 128), bf16), V((7, 4, 512, 128), bf16),
            V((7, 14, 512, 128), bf16), V((7, 4, HF, 128), bf16),
            V((7, 4, HM, 128), bf16), V((7, 4, HM, 128), bf16), V((7, 4, HM, 128), bf16), V((7, 14, HM, 128), bf16),
            V((8, TM, 128), f32), V((8, TM + HALO, 128), f32), V((8, TM + HALO, 128), f32), V((W, TM, 128), f32),
            V((HM, D), f32), V((TM, D), f32),
            V((3, HM, 512), f32), V((2, HM, 256 * NPRE), f32), V((3, HM, 512), f32),
            V((TM, 128), f32), V((TM, 128), f32), V((TM + HALO, 128), f32), V((TM, 128), f32),
            V((TM, 128), f32), V((TM, 128), f32), V((TM, 128), f32),
            V((8, F), f32), V((8, D), f32), V((8, 128), f32),
            pltpu.SemaphoreType.DMA((14 + 1024 // RQ,)), pltpu.SemaphoreType.DMA((2,)),
        ],
        compiler_params=pltpu.CompilerParams(vmem_limit_bytes=127 * 1024 * 1024),
    )(A_x.reshape(S, D), A_wqkv, A_wo, B_w1, B_b1, B_w2, B_b2)
    return out.reshape(1, S, D)
```

```python
import functools

import jax
import jax.numpy as jnp
import numpy as np
from jax import lax
import jax.experimental.pallas as pl
import jax.experimental.pallas.tpu as pltpu

S, D, F = 2048, 1024, 3584
DH, W, DIL = 32, 8, 2
TM = 512
HM = TM // 2
HF = F // 2
NT = S // TM
HALO = 16
EPS = 1e-5
TINY = 1e-30
QSCALE = float(DH ** -0.5 * np.log2(np.e))
NEG = float(-1e9 * np.log2(np.e))
NPRE = 4
RQ = 256
QK = (10850, 21500)
QKF = (14000, 21400)
L1 = (42000, 59000)
TK = (3900, 6600)
TV = (10000, 13800)
TO = (12500, 21400)
TA = (2000, 2000)
T2 = (500, 15000)
CB = 2
f32, bf16, u32, i32 = jnp.float32, jnp.bfloat16, jnp.uint32, jnp.int32
P = functools.partial


def _tree(op, xs):
    xs = list(xs)
    while len(xs) > 1:
        xs = [op(xs[i], xs[i + 1]) if i + 1 < len(xs) else xs[i] for i in range(0, len(xs), 2)]
    return xs[0]


def _a_sums(a11, a12, a21, a22):
    return (a11 + a22, a21 + a22, a11, a22, a11 + a12, a21 - a11, a12 - a22)


def _b_sums(b11, b12, b21, b22):
    return (b11 + b22, b11, b12 - b22, b21 - b11, b22, b11 + b12, b21 + b22)


M1, M2, M3, M4, M5, M6, M7 = range(7)


def _tile(j, n=1):
    if isinstance(j, int):
        return slice(j * 128, (j + n) * 128)
    return pl.ds(pl.multiple_of(j * 128, 128), n * 128)


def _pow2(s):
    return pltpu.bitcast((pltpu.bitcast(s, i32) + 0x007FFFFF) & 0x7F800000, f32)


def _pow2_inv(s):
    return pltpu.bitcast(0x7F000000 - pltpu.bitcast(s, i32), f32)


def _pow2_sqrt(s):
    half = lax.shift_right_logical(pltpu.bitcast(s, i32), 1)
    return pltpu.bitcast((half + 0x1FC00000) & 0x7F800000, f32)


def _skew_select(ts, index, unit):
    ts = [ts[-i % 8] for i in range(8)]
    for b in (1, 2, 4):
        take = (index & (unit * b)) != 0
        ts = [jnp.where(take, ts[(i - b) % 8], ts[i]) for i in range(8)]
    return ts


def _kernel(x_hbm, wqkv_hbm, wo_hbm, w1_hbm, b1_ref, w2_hbm, b2_ref, out_hbm,
            ostage, xin, x, wqkv_raw, wo_raw, w1_raw, w2_raw,
            wq, wo, w1, w2, xs1, xs2, os_, hs, q, k, v, pr, ua, xt, part, pre, carry,
            s1, sq, sv, so, sg, gh, sh, b1, b2, stat, isem, osem):
    sub = lax.broadcasted_iota(i32, (8, 128), 0)

    clock = [0]
    queue = []

    def never(shape, dtype):
        return jnp.broadcast_to(jnp.abs(b2[0:1, 0:128]), shape).astype(dtype) < 0

    def plan(window, items):
        lo, hi = window
        entries = [(lo + (hi - lo) * (n + 1) / len(items), f) for n, f in enumerate(items)]
        queue.extend(entries)
        queue.sort(key=lambda e: e[0])
        return entries

    def finish(entries):
        for e in entries:
            if e in queue:
                queue.remove(e)
                e[1]()

    def flush(until):
        vals = []
        while queue and queue[0][0] <= until:
            vals.append(queue.pop(0)[1]())
        return vals

    def tie(operand, r, until):
        vals = flush(until)
        if not vals:
            return operand
        d = _tree(jnp.add, vals)
        d = jnp.concatenate([d, d], axis=0).astype(bf16)
        parts = [operand[:r], jnp.where(never((16, 128), bf16), d, operand[r:r + 16]), operand[r + 16:]]
        return jnp.concatenate([p for p in parts if p.shape[0]], axis=0)

    last = {}

    def after(key, val):
        if key not in last:
            return val
        return jnp.where(never(val.shape, f32), last[key], val)

    def mm(a_ref, w_ref, i, c):
        kt = a_ref.shape[1]
        ls = [a_ref[i, t] for t in range(kt)]
        rs = [w_ref[i, 2 * c + n] for n in range(2)]
        t0 = clock[0]
        clock[0] = t0 + 128 * kt
        if kt == 4:
            out = []
            for n in range(2):
                l0 = ls[0]
                for r in range(0, HM, 64):
                    l0 = tie(l0, r, t0 + n * 256 + r + 63)
                out.append(jnp.dot(jnp.concatenate([l0] + ls[1:], axis=1), rs[n], preferred_element_type=f32))
            return jnp.concatenate(out, axis=1)
        for g in range(kt // 4 + 1):
            for r in range(0, HM, 64):
                ls[4 * g] = tie(ls[4 * g], r, t0 + g * 448 + r + 63)
        return jnp.dot(jnp.concatenate(ls, axis=1), jnp.concatenate(rs, axis=1), preferred_element_type=f32)

    def put(dst, i, t0, rows, val):
        for t in range(val.shape[1] // 128):
            dst[i, t0 + t, rows, :] = val[:, _tile(t)].astype(bf16)

    def put_a(dst, r, ua_):
        ua[r:r + 16, :] = ua_
        put(dst, M3, 0, slice(r, r + 16), ua_[:, :512])
        put(dst, M5, 0, slice(r, r + 16), ua_[:, :512] + ua_[:, 512:])

    def put_b(dst, r, ub):
        ss = _a_sums(ua[r:r + 16, :512], ua[r:r + 16, 512:], ub[:, :512], ub[:, 512:])
        for i in (M1, M2, M4, M6, M7):
            put(dst, i, 0, slice(r, r + 16), ss[i])

    def ln(xv, chain=False):
        if chain:
            xv = jnp.concatenate([after('ln', xv[:, :128]), xv[:, 128:]], axis=1)
        z = xv - jnp.sum(xv, axis=1, keepdims=True) * (1.0 / D)
        var = jnp.sum(z * z, axis=1, keepdims=True) * (1.0 / D)
        var = jnp.broadcast_to(var, (xv.shape[0], 128))
        if chain:
            last['ln'] = var
        size = _pow2_sqrt(jnp.maximum(var, TINY))
        g = _pow2_inv(size)
        u = jnp.concatenate([z[:, _tile(j)] * g for j in range(8)], axis=1)
        return u, lax.rsqrt(var + EPS) * size

    def ln1(base, n, r):
        ua_, sa = ln(x[pl.ds(pl.multiple_of(base + r, n), n), :])
        ub, sb = ln(x[pl.ds(pl.multiple_of(base + HM + r, n), n), :])
        for i, val in enumerate(_a_sums(ua_[:, :512], ua_[:, 512:], ub[:, :512], ub[:, 512:])):
            put(xs1, i, 0, slice(r, r + n), val)
        for r0, s in ((r, sa), (HM + r, sb)):
            s1[r0:r0 + n, :] = s
            sq[r0:r0 + n, :] = s * QSCALE
            sv[HALO + r0:HALO + r0 + n, :] = _pow2(s)
        return (sa + sb)[0:8]

    def ln2(half, r, chain):
        rows = slice(half * HM + r, half * HM + r + 16)
        u, s = ln(xt[rows, :], chain)
        (put_b if half else put_a)(xs2, r, u)
        p = s * s * stat[0:1, :] + stat[1:2, :]
        size = _pow2_sqrt(p)
        g = _pow2_inv(size)
        gh[rows, :] = g
        sg[rows, :] = s * g
        sh[rows, :] = size * size

    def qkv_dst(g, j, half):
        if g == 0:
            return q.at[j, pl.ds(half * HM, HM), :]
        return (k, v)[g - 1].at[j, pl.ds(HALO + half * HM, HM), :]

    def qkv_p1(g, c):
        sc = (sq if g == 0 else s1)[0:HM, :]
        sc = jnp.concatenate([sc, sc], axis=1)
        md = P(mm, xs1, wq, c=g * 2 + c)

        def out(j, half, val):
            for t in range(2):
                qkv_dst(g, c * 2 + j + t, half)[...] = val[:, _tile(t)]
        m3 = md(M3)
        m5 = md(M5)
        out(4, 0, (m3 + m5) * sc)
        m1 = md(M1)
        out(4, 1, m1 + m3)
        acc = m1 - m5
        m4 = md(M4)
        out(0, 1, m4)
        out(0, 0, (acc + m4 + md(M7)) * sc)

    def qkv_p2(g, c):
        sc = (sq if g == 0 else s1)[HM:TM, :]
        m2 = mm(xs1, wq, M2, g * 2 + c)
        acc = []
        for t in range(2):
            l, r = qkv_dst(g, c * 2 + t, 1), qkv_dst(g, c * 2 + t + 4, 1)
            l[...] = (l[...] + m2[:, _tile(t)]) * sc
            acc.append(r[...] - m2[:, _tile(t)])
        m6 = mm(xs1, wq, M6, g * 2 + c)
        for t in range(2):
            qkv_dst(g, c * 2 + t + 4, 1)[...] = (acc[t] + m6[:, _tile(t)]) * sc

    def window(ref, lead, r):
        return [ref[lead + (pl.ds(HALO + r - DIL * w, 8), slice(None))] for w in range(W)]

    def qk8(r, first, chain):
        qs = [q[j, r:r + 8, :] for j in range(8)]
        if chain:
            qs = [after('qk', t) for t in qs]
        ks = [window(k, (j,), r) for j in range(8)]
        ls = []
        for w in range(W):
            p = _tree(jnp.add, [qs[j] * ks[j][w] for j in range(8)])
            p = (p + pltpu.roll(p, 64, 1)) + (pltpu.roll(p, 32, 1) + pltpu.roll(p, 96, 1))
            if r - DIL * w < 0:
                p = jnp.where(jnp.logical_and(first, sub + (r - DIL * w) < 0), NEG, p)
            ls.append(p)
        last['qk'] = ls[0]
        m = _tree(jnp.maximum, ls)
        es = [jnp.exp2(l - m) for l in ls]
        sc = _tree(jnp.maximum, window(sv, (), r))
        so[r:r + 8, :] = sc
        den = _tree(jnp.add, es)
        inv = pltpu.reciprocal(den, approx=True)
        inv = inv * (2.0 - den * inv) * _pow2_inv(sc)
        for w in range(W):
            pr[w, r:r + 8, :] = es[w] * inv
        return inv

    def pv8(r):
        ps = [pr[w, r:r + 8, :] for w in range(W)]
        return jnp.concatenate(
            [_tree(jnp.add, [a * b for a, b in zip(ps, window(v, (j,), r))]) for j in range(8)], axis=1)

    def pv16(half, r):
        r0 = half * HM + r
        (put_b if half else put_a)(os_, r, jnp.concatenate([pv8(r0), pv8(r0 + 8)], axis=0))

    def v_first(first):
        for j in range(8):
            v0 = jnp.broadcast_to(v[j, HALO:HALO + 1, :], (HALO, 128))
            v[j, 0:HALO, :] = jnp.where(first, v0, v[j, 0:HALO, :])

    def halo_save():
        sv[0:HALO, :] = sv[TM:TM + HALO, :]
        for j in range(8):
            k[j, 0:HALO, :] = k[j, TM:TM + HALO, :]
            v[j, 0:HALO, :] = v[j, TM:TM + HALO, :]

    def acc_x(base, half, j, val):
        rows = pl.ds(pl.multiple_of(base + half * HM, HM), HM)
        sc = so[half * HM:(half + 1) * HM, :]
        for t in range(2):
            r = x[rows, _tile(j + t)] + val[:, _tile(t)] * sc
            xt[half * HM:(half + 1) * HM, _tile(j + t)] = r
            if half:
                x[rows, _tile(j + t)] = r

    def wo_p1(base, c):
        cols = _tile(c * 2, 2)
        m3 = mm(os_, wo, M3, c)
        part[2, :, cols] = m3
        m5 = mm(os_, wo, M5, c)
        part[0, :, cols] = m5
        acc_x(base, 0, 4 + c * 2, m3 + m5)

    def wo_p2(base, c):
        cols = _tile(c * 2, 2)
        m1 = mm(os_, wo, M1, c)
        part[2, :, cols] = part[2, :, cols] + m1
        acc = m1 - part[0, :, cols]
        m4 = mm(os_, wo, M4, c)
        part[1, :, cols] = m4
        acc_x(base, 0, c * 2, acc + m4 + mm(os_, wo, M7, c))

    def wo_p3(base, c):
        cols = _tile(c * 2, 2)
        m2 = mm(os_, wo, M2, c)
        acc_x(base, 1, c * 2, part[1, :, cols] + m2)
        acc = part[2, :, cols] - m2
        acc_x(base, 1, 4 + c * 2, acc + mm(os_, wo, M6, c))

    def w1_pre(c):
        pre[0, :, _tile(c * 2, 2)] = mm(xs2, w1, M3, c)
        pre[1, :, _tile(c * 2, 2)] = mm(xs2, w1, M5, c)

    def w1_chunk(c):
        md = P(mm, xs2, w1, c=c)

        def act(z, half, side):
            rows = slice(half * HM, (half + 1) * HM)
            out = []
            for t in range(2):
                b = b1[0:1, _tile(side * 14 + c * 2 + t)]
                y = jnp.maximum(z[:, _tile(t)] * sg[rows, :] + gh[rows, :] * b, 0.0)
                out.append(y * y)
            return jnp.concatenate(out, axis=1)

        def out(i, val):
            put(hs, i, c * 2, slice(0, HM), val)
        if c < NPRE:
            m3, m5 = pre[0, :, _tile(c * 2, 2)], pre[1, :, _tile(c * 2, 2)]
        else:
            m3, m5 = md(M3), md(M5)
        h12 = act(m3 + m5, 0, 1)
        m4 = md(M4)
        acc1 = m4 - m5
        m2 = md(M2)
        h21 = act(m4 + m2, 1, 0)
        acc2 = m3 - m2
        m1 = md(M1)
        acc1, acc2 = acc1 + m1, acc2 + m1
        h22 = act(acc2 + md(M6), 1, 1)
        out(M2, h21 + h22)
        out(M4, h22)
        out(M7, h12 - h22)
        h11 = act(acc1 + md(M7), 0, 0)
        out(M1, h11 + h22)
        out(M3, h11)
        out(M5, h11 + h12)
        out(M6, h21 - h11)

    def fin(res, base, slot, half, c, side, val, sc):
        rows = pl.ds(pl.multiple_of(base + half * HM, HM), HM)
        for t in range(2):
            cols = _tile(side * 4 + c * 2 + t)
            r = res(rows, cols) + val[:, _tile(t)] * sc + b2[0:8, cols][0:1]
            x[rows, cols] = r
            ostage[slot, half, :, cols] = r.astype(bf16)

    def w2_p1(base, slot, c):
        done = P(fin, lambda rows, cols: xt[0:HM, cols], base, slot, 0, c, sc=sh[0:HM, :])
        m3 = mm(hs, w2, M3, c)
        m5 = mm(hs, w2, M5, c)
        done(1, m3 + m5)
        m1 = mm(hs, w2, M1, c)
        carry[1, :, _tile(2 * c, 2)] = m1 + m3
        acc = m1 - m5
        m4 = mm(hs, w2, M4, c)
        carry[0, :, _tile(2 * c, 2)] = m4
        done(0, acc + m4 + mm(hs, w2, M7, c))
        if c == 1:
            carry[2, :, 0:128] = sh[HM:TM, :]

    def w2_p2(base, slot, c):
        done = P(fin, lambda rows, cols: x[rows, cols], base, slot, 1, c, sc=carry[2, :, 0:128])
        m2 = mm(hs, w2, M2, c)
        done(0, carry[0, :, _tile(2 * c, 2)] + m2)
        acc = carry[1, :, _tile(2 * c, 2)] - m2
        done(1, acc + mm(hs, w2, M6, c))

    def put_sums(dst, rows, t, blocks):
        bits = []
        for i, s in enumerate(_b_sums(*blocks)):
            put(dst, i, t, rows, s)
            if i in (M4, M7):
                bits += [pltpu.bitcast(s[a:a + 8, 0:128], i32) for a in range(0, s.shape[0], 16)]
        return pltpu.bitcast(_tree(jnp.bitwise_or, bits), f32)

    def permuted(r, n, g):
        lane = lax.broadcasted_iota(i32, (n // 2, 128), 1)
        src = ((lane & 31) << 2) | (lane >> 5)
        ts = [pltpu.bitcast(wqkv_raw[r:r + n, _tile(g * 8 + j)], u32) for j in range(8)]
        ts = [pltpu.roll(t, 4 * j, 1) if j else t for j, t in enumerate(ts)]
        ts = _skew_select(ts, lane, 4)
        return [pltpu.bitcast(jnp.take_along_axis(t, (src + 4 * j) & 127, axis=1), bf16).astype(f32)
                for j, t in enumerate(ts)]

    def prep_qkv(g, n, r):
        top, bot = permuted(r, n, g), permuted(512 + r, n, g)
        return _tree(jnp.maximum, [
            put_sums(wq, slice(r, r + n), g * 4 + t, (top[t], top[t + 4], bot[t], bot[t + 4])) for t in range(4)])

    def prep_wo(t, d3, h1):
        blk = {}
        for side in range(2):
            for d4 in range(2):
                for h0 in range(2):
                    src = []
                    for hh in range(8):
                        r = hh * 128 + h1 * 64 + h0 * 32 + d4 * 16
                        val = wo_raw[r:r + 16, _tile(t + 4 * side)].astype(f32)[8 * d3:8 * d3 + 8]
                        src.append(pltpu.roll(val, hh, 0) if hh else val)
                    for dl, val in enumerate(_skew_select(src, sub, 1)):
                        blk[d4, side, h0, dl] = pltpu.roll(val, 8 - dl, 0) if dl else val
        out = []
        for dl in range(8):
            r = d3 * 256 + dl * 32 + h1 * 16
            out.append(put_sums(wo, slice(r, r + 16), t,
                                [jnp.concatenate([blk[d4, side, 0, dl], blk[d4, side, 1, dl]], axis=0)
                                 for d4 in range(2) for side in range(2)]))
        return _tree(jnp.maximum, out)

    def w1_blocks(t, r):
        return [w1_raw[rr:rr + 64, _tile(j)].astype(f32) for rr in (r, 512 + r) for j in (t, t + 14)]

    def prep_w1(t, r):
        return put_sums(w1, slice(r, r + 64), t, w1_blocks(t, r))

    def prep_w1_first():
        es = []
        for t in range(2):
            for r in range(0, 512, 64):
                blocks = w1_blocks(t, r)
                put_sums(w1, slice(r, r + 64), t, blocks)
                e = _tree(jnp.add, [y * y for y in blocks])
                es.append(_tree(jnp.add, [e[a:a + 8] for a in range(0, 64, 8)]))
        tot = jnp.sum(jnp.sum(_tree(jnp.add, es), axis=1, keepdims=True), axis=0, keepdims=True)
        stat[0:1, :] = jnp.broadcast_to(tot * (1.0 / 512), (1, 128))
        bb = b1[0:1, :]
        stat[1:2, :] = jnp.broadcast_to(jnp.sum(bb * bb, axis=1, keepdims=True) * (1.0 / F) + TINY, (1, 128))

    def prep_w2(t, r):
        return put_sums(w2, slice(r, r + 64), t,
                        [w2_raw[rr:rr + 64, _tile(j)].astype(f32) for rr in (r, HF + r) for j in (t, t + 4)])

    def cvt_x(r):
        val = xin[r:r + 64, :].astype(f32)
        x[r:r + 64, :] = val
        return _tree(jnp.add, [val[a:a + 8, 0:128] for a in range(0, 64, 8)])

    def dma(src, dst, block, i):
        return pltpu.make_async_copy(src.at[block], dst.at[block], isem.at[i])

    full = slice(None)
    cp_x0 = [[dma(x_hbm, xin, (pl.ds(half * HM + r, 128), full), 10 + 1024 // RQ + 2 * (r // 128) + half)
              for half in range(2)] for r in range(0, HM, 128)]
    cp_x1 = dma(x_hbm, xin, (pl.ds(TM, S - TM), full), 1)
    cp_k, cp_v = (dma(wqkv_hbm, wqkv_raw, (full, pl.ds(g * D, D)), 1 + g) for g in (1, 2))
    cp_wo = dma(wo_hbm, wo_raw, (full, full), 4)
    cp_w2 = dma(w2_hbm, w2_raw, (full, full), 5)
    cp_w1 = dma(w1_hbm, w1_raw, (full, full), 6)
    cp_q = [[dma(wqkv_hbm, wqkv_raw, (pl.ds(s * 512 + n * RQ, RQ), pl.ds(0, D)), 10 + 2 * n + s) for s in range(2)]
            for n in range(512 // RQ)]

    def step(t, peeled):
        base = (t % NT) * TM
        pbase = ((t + NT - 1) % NT) * TM
        nbase = ((t + 1) % NT) * TM
        slot = t % 2
        first = t % NT == 0
        clock[0] = 0
        last.clear()
        qk_items = [P(qk8, r, first, not peeled) for r in range(0, TM, 8)]
        ln1_items = [P(ln1, nbase, 16, r) for r in range(0, HM, 16)]

        def two(f, *a):
            for c in range(2):
                f(*a, c)
        if peeled:
            for cp in [*sum(cp_x0 + cp_q, []), cp_k, cp_v, cp_wo, cp_w1, cp_w2, cp_x1]:
                cp.start()
            sv[0:HALO, :] = jnp.zeros((HALO, 128), f32)
            k[:, 0:HALO, :] = jnp.zeros((8, HALO, 128), f32)
            v[:, 0:HALO, :] = jnp.zeros((8, HALO, 128), f32)
            b1[0:1, :] = b1_ref[...].astype(f32).reshape(1, F)
            b2[0:1, :] = b2_ref[...].astype(f32).reshape(1, D)
            ostage[slot, 1] = jnp.zeros((HM, D), bf16)
            for r, cps in zip(range(0, HM, 128), cp_x0):
                for cp in cps:
                    cp.wait()
                for rr in (r, r + 64, HM + r, HM + r + 64):
                    cvt_x(rr)
                ln1(base, 128, r)
            for n, cps in enumerate(cp_q):
                for cp in cps:
                    cp.wait()
                for r in range(n * RQ, (n + 1) * RQ, 128):
                    prep_qkv(0, 128, r)
            attn = plan(QKF, qk_items)
            qkv_p1(0, 0)
            qkv_p2(0, 0)
            cp_k.wait()
            job = plan(TK, [P(prep_qkv, 1, 64, r) for r in range(0, 512, 64)])
            qkv_p1(0, 1)
            qkv_p2(0, 1)
            finish(job)
            qkv_p1(1, 0)
            cp_v.wait()
            cp_wo.wait()
            job = plan(TV, [P(prep_qkv, 2, 64, r) for r in range(0, 512, 64)])
            job_wo = plan(TO, [P(prep_wo, tt, d3, h1) for tt in range(4) for d3 in range(2) for h1 in range(2)])
            qkv_p1(1, 1)
            two(qkv_p2, 1)
            finish(job)
        else:
            attn = plan(QK, qk_items)
            job_ln1 = plan(L1, ln1_items)
            two(qkv_p1, 0)
            two(qkv_p1, 1)
            two(qkv_p2, 0)
            two(qkv_p2, 1)
        two(qkv_p1, 2)
        v_first(first)
        two(qkv_p2, 2)
        finish(attn)
        for half in range(2):
            for r in range(0, HM, 16):
                pv16(half, r)
        if peeled:
            finish(job_wo)
        else:
            w2_p2(pbase, slot, 0)
        two(wo_p1, base)
        halo_save()
        if peeled:
            cp_w1.wait()
            prep_w1_first()
            jobs = {}
            for c in range(1, 7):
                lo = clock[0] + TA[0] + (c - 1) * TA[1]
                jobs[c] = plan((lo, lo + TA[1]), [P(prep_w1, tt, r) for tt in (2 * c, 2 * c + 1) for r in range(0, 512, 64)])
        two(wo_p2, base)
        two(wo_p3, base)
        if not peeled:
            w2_p2(pbase, slot, 1)
        for half in range(2):
            for r in range(0, HM, 16):
                ln2(half, r, not peeled)
        for c in range(NPRE):
            if peeled and c:
                finish(jobs[c])
            w1_pre(c)
        for c in range(7):
            if peeled and c == CB:
                for cc in jobs:
                    finish(jobs[cc])
                cp_w2.wait()
                cp_x1.wait()
                job = plan((clock[0] + T2[0], clock[0] + T2[1]),
                           [P(prep_w2, tt, r) for tt in range(4) for r in range(0, HF, 64)])
            w1_chunk(c)
        if peeled:
            finish(job)
            for r in range(TM, 2 * TM, 64):
                cvt_x(r)
            late = (clock[0] + 1000, clock[0] + 16000)
            job_ln1 = plan(late, ln1_items)
            job = plan(late, [P(cvt_x, r) for r in range(2 * TM, S, 64)])
        else:
            finish(job_ln1)
        two(w2_p1, base, slot)
        if peeled:
            finish(job_ln1)
            finish(job)
        assert not queue

    def out_copies(t):
        return [pltpu.make_async_copy(
            ostage.at[t % 2, half],
            out_hbm.at[pl.ds(pl.multiple_of(((t + (NT - 1) * half) % NT) * TM + half * HM, HM), HM), :],
            osem.at[half]) for half in range(2)]

    step(0, True)

    def body(t, c):
        cps = out_copies(t - 1)
        for cp in cps:
            cp.start()
        step(t, False)
        for cp in cps:
            cp.wait()
        return c

    lax.fori_loop(1, 2 * NT, body, 0)
    cps = out_copies(2 * NT - 1)
    for cp in cps:
        cp.start()
    lax.fori_loop(0, 2, lambda c, _: w2_p2(S - TM, 0, c), None)
    for cp in cps:
        cp.wait()
    last = out_copies(2 * NT)[1]
    last.start()
    last.wait()


@jax.jit
def pallas_interleave_layers__sliding_local_dilated__dense_activation_squared_relu__prompt_kernel(A_x, A_wqkv, A_wo, B_x, B_w1, B_b1, B_w2, B_b2):
    del B_x
    hbm = pl.BlockSpec(memory_space=pl.ANY)
    vmem = pl.BlockSpec(memory_space=pltpu.VMEM)
    V = pltpu.VMEM
    out = pl.pallas_call(
        _kernel,
        in_specs=[hbm, hbm, hbm, hbm, vmem, hbm, vmem],
        out_specs=hbm,
        out_shape=jax.ShapeDtypeStruct((S, D), bf16),
        scratch_shapes=[
            V((2, 2, HM, D), bf16), V((S, D), bf16), V((S, D), f32),
            V((D, 3 * D), bf16), V((D, D), bf16), V((D, F), bf16), V((F, D), bf16),
            V((7, 12, 512, 128), bf16), V((7, 4, 512, 128), bf16),
            V((7, 14, 512, 128), bf16), V((7, 4, HF, 128), bf16),
            V((7, 4, HM, 128), bf16), V((7, 4, HM, 128), bf16), V((7, 4, HM, 128), bf16), V((7, 14, HM, 128), bf16),
            V((8, TM, 128), f32), V((8, TM + HALO, 128), f32), V((8, TM + HALO, 128), f32), V((W, TM, 128), f32),
            V((HM, D), f32), V((TM, D), f32),
            V((3, HM, 512), f32), V((2, HM, 256 * NPRE), f32), V((3, HM, 512), f32),
            V((TM, 128), f32), V((TM, 128), f32), V((TM + HALO, 128), f32), V((TM, 128), f32),
            V((TM, 128), f32), V((TM, 128), f32), V((TM, 128), f32),
            V((8, F), f32), V((8, D), f32), V((8, 128), f32),
            pltpu.SemaphoreType.DMA((14 + 1024 // RQ,)), pltpu.SemaphoreType.DMA((2,)),
        ],
        compiler_params=pltpu.CompilerParams(vmem_limit_bytes=127 * 1024 * 1024),
    )(A_x.reshape(S, D), A_wqkv, A_wo, B_w1, B_b1, B_w2, B_b2)
    return out.reshape(1, S, D)
```

```python
import functools

import jax
import jax.numpy as jnp
import numpy as np
from jax import lax
import jax.experimental.pallas as pl
import jax.experimental.pallas.tpu as pltpu

S, D, F = 2048, 1024, 3584
DH, W, DIL = 32, 8, 2
TM = 512
HM = TM // 2
HF = F // 2
NT = S // TM
HALO = 16
EPS = 1e-5
TINY = 1e-30
QSCALE = float(DH ** -0.5 * np.log2(np.e))
NEG = float(-1e9 * np.log2(np.e))
NPRE = 4
RQ = 256
QK = (10850, 21500)
QKF = (14000, 21400)
L1 = (42000, 59000)
TK = (3900, 6600)
TV = (10000, 13800)
TO = (12500, 21400)
TA = (2000, 2000)
T2 = (500, 15000)
CB = 2
f32, bf16, u32, i32 = jnp.float32, jnp.bfloat16, jnp.uint32, jnp.int32
P = functools.partial


def _tree(op, xs):
    xs = list(xs)
    while len(xs) > 1:
        xs = [op(xs[i], xs[i + 1]) if i + 1 < len(xs) else xs[i] for i in range(0, len(xs), 2)]
    return xs[0]


def _a_sums(a11, a12, a21, a22):
    return (a11 + a22, a21 + a22, a11, a22, a11 + a12, a21 - a11, a12 - a22)


def _b_sums(b11, b12, b21, b22):
    return (b11 + b22, b11, b12 - b22, b21 - b11, b22, b11 + b12, b21 + b22)


M1, M2, M3, M4, M5, M6, M7 = range(7)


def _tile(j, n=1):
    if isinstance(j, int):
        return slice(j * 128, (j + n) * 128)
    return pl.ds(pl.multiple_of(j * 128, 128), n * 128)


def _pow2(s):
    return pltpu.bitcast((pltpu.bitcast(s, i32) + 0x007FFFFF) & 0x7F800000, f32)


def _pow2_inv(s):
    return pltpu.bitcast(0x7F000000 - pltpu.bitcast(s, i32), f32)


def _pow2_sqrt(s):
    half = lax.shift_right_logical(pltpu.bitcast(s, i32), 1)
    return pltpu.bitcast((half + 0x1FC00000) & 0x7F800000, f32)


def _skew_select(ts, index, unit):
    ts = [ts[-i % 8] for i in range(8)]
    for b in (1, 2, 4):
        take = (index & (unit * b)) != 0
        ts = [jnp.where(take, ts[(i - b) % 8], ts[i]) for i in range(8)]
    return ts


def _kernel(x_hbm, wqkv_hbm, wo_hbm, w1_hbm, b1_ref, w2_hbm, b2_ref, out_hbm,
            ostage, xin, x, wqkv_raw, wo_raw, w1_raw, w2_raw,
            wq, wo, w1, w2, xs1, xs2, os_, hs, q, k, v, pr, ua, xt, part, pre, carry,
            s1, sq, sv, so, sg, gh, sh, b1, b2, stat, isem, osem):
    sub = lax.broadcasted_iota(i32, (8, 128), 0)

    clock = [0]
    queue = []

    def never(shape, dtype):
        return jnp.broadcast_to(jnp.abs(b2[0:1, 0:128]), shape).astype(dtype) < 0

    def plan(window, items):
        lo, hi = window
        entries = [(lo + (hi - lo) * (n + 1) / len(items), f) for n, f in enumerate(items)]
        queue.extend(entries)
        queue.sort(key=lambda e: e[0])
        return entries

    def finish(entries):
        for e in entries:
            if e in queue:
                queue.remove(e)
                e[1]()

    def flush(until):
        vals = []
        while queue and queue[0][0] <= until:
            vals.append(queue.pop(0)[1]())
        return vals

    def tie(operand, r, until):
        vals = flush(until)
        if not vals:
            return operand
        d = _tree(jnp.add, vals)
        d = jnp.concatenate([d, d], axis=0).astype(bf16)
        parts = [operand[:r], jnp.where(never((16, 128), bf16), d, operand[r:r + 16]), operand[r + 16:]]
        return jnp.concatenate([p for p in parts if p.shape[0]], axis=0)

    last = {}

    def after(key, val):
        if key not in last:
            return val
        return jnp.where(never(val.shape, f32), last[key], val)

    def mm(a_ref, w_ref, i, c):
        kt = a_ref.shape[1]
        ls = [a_ref[i, t] for t in range(kt)]
        rs = [w_ref[i, 2 * c + n] for n in range(2)]
        t0 = clock[0]
        clock[0] = t0 + 128 * kt
        if kt == 4:
            out = []
            for n in range(2):
                l0 = ls[0]
                for r in range(0, HM, 64):
                    l0 = tie(l0, r, t0 + n * 256 + r + 63)
                out.append(jnp.dot(jnp.concatenate([l0] + ls[1:], axis=1), rs[n], preferred_element_type=f32))
            return jnp.concatenate(out, axis=1)
        for g in range(kt // 4 + 1):
            for r in range(0, HM, 64):
                ls[4 * g] = tie(ls[4 * g], r, t0 + g * 448 + r + 63)
        return jnp.dot(jnp.concatenate(ls, axis=1), jnp.concatenate(rs, axis=1), preferred_element_type=f32)

    def put(dst, i, t0, rows, val):
        for t in range(val.shape[1] // 128):
            dst[i, t0 + t, rows, :] = val[:, _tile(t)].astype(bf16)

    def put_a(dst, r, ua_):
        ua[r:r + 16, :] = ua_
        put(dst, M3, 0, slice(r, r + 16), ua_[:, :512])
        put(dst, M5, 0, slice(r, r + 16), ua_[:, :512] + ua_[:, 512:])

    def put_b(dst, r, ub):
        ss = _a_sums(ua[r:r + 16, :512], ua[r:r + 16, 512:], ub[:, :512], ub[:, 512:])
        for i in (M1, M2, M4, M6, M7):
            put(dst, i, 0, slice(r, r + 16), ss[i])

    def ln(xv, chain=False):
        if chain:
            xv = jnp.concatenate([after('ln', xv[:, :128]), xv[:, 128:]], axis=1)
        z = xv - jnp.sum(xv, axis=1, keepdims=True) * (1.0 / D)
        var = jnp.sum(z * z, axis=1, keepdims=True) * (1.0 / D)
        var = jnp.broadcast_to(var, (xv.shape[0], 128))
        if chain:
            last['ln'] = var
        size = _pow2_sqrt(jnp.maximum(var, TINY))
        g = _pow2_inv(size)
        u = jnp.concatenate([z[:, _tile(j)] * g for j in range(8)], axis=1)
        return u, lax.rsqrt(var + EPS) * size

    def ln1(base, n, r):
        ua_, sa = ln(x[pl.ds(pl.multiple_of(base + r, n), n), :])
        ub, sb = ln(x[pl.ds(pl.multiple_of(base + HM + r, n), n), :])
        for i, val in enumerate(_a_sums(ua_[:, :512], ua_[:, 512:], ub[:, :512], ub[:, 512:])):
            put(xs1, i, 0, slice(r, r + n), val)
        for r0, s in ((r, sa), (HM + r, sb)):
            s1[r0:r0 + n, :] = s
            sq[r0:r0 + n, :] = s * QSCALE
            sv[HALO + r0:HALO + r0 + n, :] = _pow2(s)
        return (sa + sb)[0:8]

    def ln2(half, r, chain):
        rows = slice(half * HM + r, half * HM + r + 16)
        u, s = ln(xt[rows, :], chain)
        (put_b if half else put_a)(xs2, r, u)
        p = s * s * stat[0:1, :] + stat[1:2, :]
        size = _pow2_sqrt(p)
        g = _pow2_inv(size)
        gh[rows, :] = g
        sg[rows, :] = s * g
        sh[rows, :] = size * size

    def qkv_dst(g, j, half):
        if g == 0:
            return q.at[j, pl.ds(half * HM, HM), :]
        return (k, v)[g - 1].at[j, pl.ds(HALO + half * HM, HM), :]

    def qkv_p1(g, c):
        sc = (sq if g == 0 else s1)[0:HM, :]
        sc = jnp.concatenate([sc, sc], axis=1)
        md = P(mm, xs1, wq, c=g * 2 + c)

        def out(j, half, val):
            for t in range(2):
                qkv_dst(g, c * 2 + j + t, half)[...] = val[:, _tile(t)]
        m3 = md(M3)
        m5 = md(M5)
        out(4, 0, (m3 + m5) * sc)
        m1 = md(M1)
        out(4, 1, m1 + m3)
        acc = m1 - m5
        m4 = md(M4)
        out(0, 1, m4)
        out(0, 0, (acc + m4 + md(M7)) * sc)

    def qkv_p2(g, c):
        sc = (sq if g == 0 else s1)[HM:TM, :]
        m2 = mm(xs1, wq, M2, g * 2 + c)
        acc = []
        for t in range(2):
            l, r = qkv_dst(g, c * 2 + t, 1), qkv_dst(g, c * 2 + t + 4, 1)
            l[...] = (l[...] + m2[:, _tile(t)]) * sc
            acc.append(r[...] - m2[:, _tile(t)])
        m6 = mm(xs1, wq, M6, g * 2 + c)
        for t in range(2):
            qkv_dst(g, c * 2 + t + 4, 1)[...] = (acc[t] + m6[:, _tile(t)]) * sc

    def window(ref, lead, r):
        return [ref[lead + (pl.ds(HALO + r - DIL * w, 8), slice(None))] for w in range(W)]

    def qk8(r, first, chain):
        qs = [q[j, r:r + 8, :] for j in range(8)]
        if chain:
            qs = [after('qk', t) for t in qs]
        ks = [window(k, (j,), r) for j in range(8)]
        ls = []
        for w in range(W):
            p = _tree(jnp.add, [qs[j] * ks[j][w] for j in range(8)])
            p = (p + pltpu.roll(p, 64, 1)) + (pltpu.roll(p, 32, 1) + pltpu.roll(p, 96, 1))
            if r - DIL * w < 0:
                p = jnp.where(jnp.logical_and(first, sub + (r - DIL * w) < 0), NEG, p)
            ls.append(p)
        last['qk'] = ls[0]
        m = _tree(jnp.maximum, ls)
        es = [jnp.exp2(l - m) for l in ls]
        sc = _tree(jnp.maximum, window(sv, (), r))
        so[r:r + 8, :] = sc
        den = _tree(jnp.add, es)
        inv = pltpu.reciprocal(den, approx=True)
        inv = inv * (2.0 - den * inv) * _pow2_inv(sc)
        for w in range(W):
            pr[w, r:r + 8, :] = es[w] * inv
        return inv

    def pv8(r):
        ps = [pr[w, r:r + 8, :] for w in range(W)]
        return jnp.concatenate(
            [_tree(jnp.add, [a * b for a, b in zip(ps, window(v, (j,), r))]) for j in range(8)], axis=1)

    def pv16(half, r):
        r0 = half * HM + r
        (put_b if half else put_a)(os_, r, jnp.concatenate([pv8(r0), pv8(r0 + 8)], axis=0))

    def v_first(first):
        for j in range(8):
            v0 = jnp.broadcast_to(v[j, HALO:HALO + 1, :], (HALO, 128))
            v[j, 0:HALO, :] = jnp.where(first, v0, v[j, 0:HALO, :])

    def halo_save():
        sv[0:HALO, :] = sv[TM:TM + HALO, :]
        for j in range(8):
            k[j, 0:HALO, :] = k[j, TM:TM + HALO, :]
            v[j, 0:HALO, :] = v[j, TM:TM + HALO, :]

    def acc_x(base, half, j, val):
        rows = pl.ds(pl.multiple_of(base + half * HM, HM), HM)
        sc = so[half * HM:(half + 1) * HM, :]
        for t in range(2):
            r = x[rows, _tile(j + t)] + val[:, _tile(t)] * sc
            xt[half * HM:(half + 1) * HM, _tile(j + t)] = r
            if half:
                x[rows, _tile(j + t)] = r

    def wo_p1(base, c):
        cols = _tile(c * 2, 2)
        m3 = mm(os_, wo, M3, c)
        part[2, :, cols] = m3
        m5 = mm(os_, wo, M5, c)
        part[0, :, cols] = m5
        acc_x(base, 0, 4 + c * 2, m3 + m5)

    def wo_p2(base, c):
        cols = _tile(c * 2, 2)
        m1 = mm(os_, wo, M1, c)
        part[2, :, cols] = part[2, :, cols] + m1
        acc = m1 - part[0, :, cols]
        m4 = mm(os_, wo, M4, c)
        part[1, :, cols] = m4
        acc_x(base, 0, c * 2, acc + m4 + mm(os_, wo, M7, c))

    def wo_p3(base, c):
        cols = _tile(c * 2, 2)
        m2 = mm(os_, wo, M2, c)
        acc_x(base, 1, c * 2, part[1, :, cols] + m2)
        acc = part[2, :, cols] - m2
        acc_x(base, 1, 4 + c * 2, acc + mm(os_, wo, M6, c))

    def w1_pre(c):
        pre[0, :, _tile(c * 2, 2)] = mm(xs2, w1, M3, c)
        pre[1, :, _tile(c * 2, 2)] = mm(xs2, w1, M5, c)

    def w1_chunk(c):
        md = P(mm, xs2, w1, c=c)

        def act(z, half, side):
            rows = slice(half * HM, (half + 1) * HM)
            out = []
            for t in range(2):
                b = b1[0:1, _tile(side * 14 + c * 2 + t)]
                y = jnp.maximum(z[:, _tile(t)] * sg[rows, :] + gh[rows, :] * b, 0.0)
                out.append(y * y)
            return jnp.concatenate(out, axis=1)

        def out(i, val):
            put(hs, i, c * 2, slice(0, HM), val)
        if c < NPRE:
            m3, m5 = pre[0, :, _tile(c * 2, 2)], pre[1, :, _tile(c * 2, 2)]
        else:
            m3, m5 = md(M3), md(M5)
        h12 = act(m3 + m5, 0, 1)
        m4 = md(M4)
        acc1 = m4 - m5
        m2 = md(M2)
        h21 = act(m4 + m2, 1, 0)
        acc2 = m3 - m2
        m1 = md(M1)
        acc1, acc2 = acc1 + m1, acc2 + m1
        h22 = act(acc2 + md(M6), 1, 1)
        out(M2, h21 + h22)
        out(M4, h22)
        out(M7, h12 - h22)
        h11 = act(acc1 + md(M7), 0, 0)
        out(M1, h11 + h22)
        out(M3, h11)
        out(M5, h11 + h12)
        out(M6, h21 - h11)

    def fin(res, base, slot, half, c, side, val, sc):
        rows = pl.ds(pl.multiple_of(base + half * HM, HM), HM)
        for t in range(2):
            cols = _tile(side * 4 + c * 2 + t)
            r = res(rows, cols) + val[:, _tile(t)] * sc + b2[:, cols][0:1]
            x[rows, cols] = r
            ostage[slot, half, :, cols] = r.astype(bf16)

    def w2_p1(base, slot, c):
        done = P(fin, lambda rows, cols: xt[0:HM, cols], base, slot, 0, c, sc=sh[0:HM, :])
        m3 = mm(hs, w2, M3, c)
        m5 = mm(hs, w2, M5, c)
        done(1, m3 + m5)
        m1 = mm(hs, w2, M1, c)
        carry[1, :, _tile(2 * c, 2)] = m1 + m3
        acc = m1 - m5
        m4 = mm(hs, w2, M4, c)
        carry[0, :, _tile(2 * c, 2)] = m4
        done(0, acc + m4 + mm(hs, w2, M7, c))
        if c == 1:
            carry[2, :, 0:128] = sh[HM:TM, :]

    def w2_p2(base, slot, c):
        done = P(fin, lambda rows, cols: x[rows, cols], base, slot, 1, c, sc=carry[2, :, 0:128])
        m2 = mm(hs, w2, M2, c)
        done(0, carry[0, :, _tile(2 * c, 2)] + m2)
        acc = carry[1, :, _tile(2 * c, 2)] - m2
        done(1, acc + mm(hs, w2, M6, c))

    def put_sums(dst, rows, t, blocks):
        bits = []
        for i, s in enumerate(_b_sums(*blocks)):
            put(dst, i, t, rows, s)
            if i in (M4, M7):
                bits += [pltpu.bitcast(s[a:a + 8, 0:128], i32) for a in range(0, s.shape[0], 16)]
        return pltpu.bitcast(_tree(jnp.bitwise_or, bits), f32)

    def permuted(r, n, g):
        lane = lax.broadcasted_iota(i32, (n // 2, 128), 1)
        src = ((lane & 31) << 2) | (lane >> 5)
        ts = [pltpu.bitcast(wqkv_raw[r:r + n, _tile(g * 8 + j)], u32) for j in range(8)]
        ts = [pltpu.roll(t, 4 * j, 1) if j else t for j, t in enumerate(ts)]
        ts = _skew_select(ts, lane, 4)
        return [pltpu.bitcast(jnp.take_along_axis(t, (src + 4 * j) & 127, axis=1), bf16).astype(f32)
                for j, t in enumerate(ts)]

    def prep_qkv(g, n, r):
        top, bot = permuted(r, n, g), permuted(512 + r, n, g)
        return _tree(jnp.maximum, [
            put_sums(wq, slice(r, r + n), g * 4 + t, (top[t], top[t + 4], bot[t], bot[t + 4])) for t in range(4)])

    def prep_wo(t, d3, h1):
        blk = {}
        for side in range(2):
            for d4 in range(2):
                for h0 in range(2):
                    src = []
                    for hh in range(8):
                        r = hh * 128 + h1 * 64 + h0 * 32 + d4 * 16
                        val = wo_raw[r:r + 16, _tile(t + 4 * side)].astype(f32)[8 * d3:8 * d3 + 8]
                        src.append(pltpu.roll(val, hh, 0) if hh else val)
                    for dl, val in enumerate(_skew_select(src, sub, 1)):
                        blk[d4, side, h0, dl] = pltpu.roll(val, 8 - dl, 0) if dl else val
        out = []
        for dl in range(8):
            r = d3 * 256 + dl * 32 + h1 * 16
            out.append(put_sums(wo, slice(r, r + 16), t,
                                [jnp.concatenate([blk[d4, side, 0, dl], blk[d4, side, 1, dl]], axis=0)
                                 for d4 in range(2) for side in range(2)]))
        return _tree(jnp.maximum, out)

    def w1_blocks(t, r):
        return [w1_raw[rr:rr + 64, _tile(j)].astype(f32) for rr in (r, 512 + r) for j in (t, t + 14)]

    def prep_w1(t, r):
        return put_sums(w1, slice(r, r + 64), t, w1_blocks(t, r))

    def prep_w1_first():
        es = []
        for t in range(2):
            for r in range(0, 512, 64):
                blocks = w1_blocks(t, r)
                put_sums(w1, slice(r, r + 64), t, blocks)
                e = _tree(jnp.add, [y * y for y in blocks])
                es.append(_tree(jnp.add, [e[a:a + 8] for a in range(0, 64, 8)]))
        tot = jnp.sum(jnp.sum(_tree(jnp.add, es), axis=1, keepdims=True), axis=0, keepdims=True)
        stat[0:1, :] = jnp.broadcast_to(tot * (1.0 / 512), (1, 128))
        bb = b1[0:1, :]
        stat[1:2, :] = jnp.broadcast_to(jnp.sum(bb * bb, axis=1, keepdims=True) * (1.0 / F) + TINY, (1, 128))

    def prep_w2(t, r):
        return put_sums(w2, slice(r, r + 64), t,
                        [w2_raw[rr:rr + 64, _tile(j)].astype(f32) for rr in (r, HF + r) for j in (t, t + 4)])

    def cvt_x(r):
        val = xin[r:r + 64, :].astype(f32)
        x[r:r + 64, :] = val
        return _tree(jnp.add, [val[a:a + 8, 0:128] for a in range(0, 64, 8)])

    def dma(src, dst, block, i):
        return pltpu.make_async_copy(src.at[block], dst.at[block], isem.at[i])

    full = slice(None)
    cp_x0 = [[dma(x_hbm, xin, (pl.ds(half * HM + r, 128), full), 10 + 1024 // RQ + 2 * (r // 128) + half)
              for half in range(2)] for r in range(0, HM, 128)]
    cp_x1 = dma(x_hbm, xin, (pl.ds(TM, S - TM), full), 1)
    cp_k, cp_v = (dma(wqkv_hbm, wqkv_raw, (full, pl.ds(g * D, D)), 1 + g) for g in (1, 2))
    cp_wo = dma(wo_hbm, wo_raw, (full, full), 4)
    cp_w2 = dma(w2_hbm, w2_raw, (full, full), 5)
    cp_w1 = dma(w1_hbm, w1_raw, (full, full), 6)
    cp_q = [[dma(wqkv_hbm, wqkv_raw, (pl.ds(s * 512 + n * RQ, RQ), pl.ds(0, D)), 10 + 2 * n + s) for s in range(2)]
            for n in range(512 // RQ)]

    def step(t, peeled):
        base = (t % NT) * TM
        pbase = ((t + NT - 1) % NT) * TM
        nbase = ((t + 1) % NT) * TM
        slot = t % 2
        first = t % NT == 0
        clock[0] = 0
        last.clear()
        qk_items = [P(qk8, r, first, not peeled) for r in range(0, TM, 8)]
        ln1_items = [P(ln1, nbase, 16, r) for r in range(0, HM, 16)]

        def two(f, *a):
            for c in range(2):
                f(*a, c)
        if peeled:
            for cp in [*sum(cp_x0 + cp_q, []), cp_k, cp_v, cp_wo, cp_w1, cp_w2, cp_x1]:
                cp.start()
            sv[0:HALO, :] = jnp.zeros((HALO, 128), f32)
            k[:, 0:HALO, :] = jnp.zeros((8, HALO, 128), f32)
            v[:, 0:HALO, :] = jnp.zeros((8, HALO, 128), f32)
            b1[0:1, :] = b1_ref[...].astype(f32).reshape(1, F)
            b2[...] = jnp.broadcast_to(b2_ref[...].astype(f32).reshape(1, D), (8, D))
            ostage[slot, 1] = jnp.zeros((HM, D), bf16)
            for r, cps in zip(range(0, HM, 128), cp_x0):
                for cp in cps:
                    cp.wait()
                for rr in (r, r + 64, HM + r, HM + r + 64):
                    cvt_x(rr)
                ln1(base, 128, r)
            for n, cps in enumerate(cp_q):
                for cp in cps:
                    cp.wait()
                for r in range(n * RQ, (n + 1) * RQ, 128):
                    prep_qkv(0, 128, r)
            attn = plan(QKF, qk_items)
            qkv_p1(0, 0)
            qkv_p2(0, 0)
            cp_k.wait()
            job = plan(TK, [P(prep_qkv, 1, 64, r) for r in range(0, 512, 64)])
            qkv_p1(0, 1)
            qkv_p2(0, 1)
            finish(job)
            qkv_p1(1, 0)
            cp_v.wait()
            cp_wo.wait()
            job = plan(TV, [P(prep_qkv, 2, 64, r) for r in range(0, 512, 64)])
            job_wo = plan(TO, [P(prep_wo, tt, d3, h1) for tt in range(4) for d3 in range(2) for h1 in range(2)])
            qkv_p1(1, 1)
            two(qkv_p2, 1)
            finish(job)
        else:
            attn = plan(QK, qk_items)
            job_ln1 = plan(L1, ln1_items)
            two(qkv_p1, 0)
            two(qkv_p1, 1)
            two(qkv_p2, 0)
            two(qkv_p2, 1)
        two(qkv_p1, 2)
        v_first(first)
        two(qkv_p2, 2)
        finish(attn)
        for half in range(2):
            for r in range(0, HM, 16):
                pv16(half, r)
        if peeled:
            finish(job_wo)
        else:
            w2_p2(pbase, slot, 0)
        two(wo_p1, base)
        halo_save()
        if peeled:
            cp_w1.wait()
            prep_w1_first()
            jobs = {}
            for c in range(1, 7):
                lo = clock[0] + TA[0] + (c - 1) * TA[1]
                jobs[c] = plan((lo, lo + TA[1]), [P(prep_w1, tt, r) for tt in (2 * c, 2 * c + 1) for r in range(0, 512, 64)])
        two(wo_p2, base)
        two(wo_p3, base)
        if not peeled:
            w2_p2(pbase, slot, 1)
        for half in range(2):
            for r in range(0, HM, 16):
                ln2(half, r, not peeled)
        for c in range(NPRE):
            if peeled and c:
                finish(jobs[c])
            w1_pre(c)
        for c in range(7):
            if peeled and c == CB:
                for cc in jobs:
                    finish(jobs[cc])
                cp_w2.wait()
                cp_x1.wait()
                job = plan((clock[0] + T2[0], clock[0] + T2[1]),
                           [P(prep_w2, tt, r) for tt in range(4) for r in range(0, HF, 64)])
            w1_chunk(c)
        if peeled:
            finish(job)
            for r in range(TM, 2 * TM, 64):
                cvt_x(r)
            late = (clock[0] + 1000, clock[0] + 16000)
            job_ln1 = plan(late, ln1_items)
            job = plan(late, [P(cvt_x, r) for r in range(2 * TM, S, 64)])
        else:
            finish(job_ln1)
        two(w2_p1, base, slot)
        if peeled:
            finish(job_ln1)
            finish(job)
        assert not queue

    def out_copies(t):
        return [pltpu.make_async_copy(
            ostage.at[t % 2, half],
            out_hbm.at[pl.ds(pl.multiple_of(((t + (NT - 1) * half) % NT) * TM + half * HM, HM), HM), :],
            osem.at[half]) for half in range(2)]

    step(0, True)

    def body(t, c):
        cps = out_copies(t - 1)
        for cp in cps:
            cp.start()
        step(t, False)
        for cp in cps:
            cp.wait()
        return c

    lax.fori_loop(1, 2 * NT, body, 0)
    cps = out_copies(2 * NT - 1)
    for cp in cps:
        cp.start()

    def last_copies(c):
        return [pltpu.make_async_copy(ostage.at[0, 1, :, _tile(4 * side + 2 * c, 2)],
                                      out_hbm.at[pl.ds(S - HM, HM), _tile(4 * side + 2 * c, 2)],
                                      osem.at[2 + 2 * c + side]) for side in range(2)]

    def last_rows(c, _):
        w2_p2(S - TM, 0, c)
        for cp in last_copies(c):
            cp.start()

    lax.fori_loop(0, 2, last_rows, None)
    for cp in cps + last_copies(0) + last_copies(1):
        cp.wait()


@jax.jit
def pallas_interleave_layers__sliding_local_dilated__dense_activation_squared_relu__prompt_kernel(A_x, A_wqkv, A_wo, B_x, B_w1, B_b1, B_w2, B_b2):
    del B_x
    hbm = pl.BlockSpec(memory_space=pl.ANY)
    vmem = pl.BlockSpec(memory_space=pltpu.VMEM)
    V = pltpu.VMEM
    out = pl.pallas_call(
        _kernel,
        in_specs=[hbm, hbm, hbm, hbm, vmem, hbm, vmem],
        out_specs=hbm,
        out_shape=jax.ShapeDtypeStruct((S, D), bf16),
        scratch_shapes=[
            V((2, 2, HM, D), bf16), V((S, D), bf16), V((S, D), f32),
            V((D, 3 * D), bf16), V((D, D), bf16), V((D, F), bf16), V((F, D), bf16),
            V((7, 12, 512, 128), bf16), V((7, 4, 512, 128), bf16),
            V((7, 14, 512, 128), bf16), V((7, 4, HF, 128), bf16),
            V((7, 4, HM, 128), bf16), V((7, 4, HM, 128), bf16), V((7, 4, HM, 128), bf16), V((7, 14, HM, 128), bf16),
            V((8, TM, 128), f32), V((8, TM + HALO, 128), f32), V((8, TM + HALO, 128), f32), V((W, TM, 128), f32),
            V((HM, D), f32), V((TM, D), f32),
            V((3, HM, 512), f32), V((2, HM, 256 * NPRE), f32), V((3, HM, 512), f32),
            V((TM, 128), f32), V((TM, 128), f32), V((TM + HALO, 128), f32), V((TM, 128), f32),
            V((TM, 128), f32), V((TM, 128), f32), V((TM, 128), f32),
            V((8, F), f32), V((8, D), f32), V((8, 128), f32),
            pltpu.SemaphoreType.DMA((14 + 1024 // RQ,)), pltpu.SemaphoreType.DMA((6,)),
        ],
        compiler_params=pltpu.CompilerParams(vmem_limit_bytes=127 * 1024 * 1024),
    )(A_x.reshape(S, D), A_wqkv, A_wo, B_w1, B_b1, B_w2, B_b2)
    return out.reshape(1, S, D)
```

```python
import functools

import jax
import jax.numpy as jnp
import numpy as np
from jax import lax
import jax.experimental.pallas as pl
import jax.experimental.pallas.tpu as pltpu

S, D, F = 2048, 1024, 3584
DH, W, DIL = 32, 8, 2
TM = 512
HM = TM // 2
HF = F // 2
NT = S // TM
HALO = 16
EPS = 1e-5
TINY = 1e-30
QSCALE = float(DH ** -0.5 * np.log2(np.e))
NEG = float(-1e9 * np.log2(np.e))
NPRE = 4
RQ = 256
QK = (10850, 21500)
QKF = (14000, 21400)
L1 = (42000, 59000)
TK = (3900, 6600)
TV = (10000, 13800)
TO = (12500, 21400)
TA = (2000, 2000)
T2 = (500, 15000)
MODE = 'all'
RL = 0
CV1 = ()
G1 = 0
G2 = (1000, 16000)
CB = 2
f32, bf16, u32, i32 = jnp.float32, jnp.bfloat16, jnp.uint32, jnp.int32
P = functools.partial


def _tree(op, xs):
    xs = list(xs)
    while len(xs) > 1:
        xs = [op(xs[i], xs[i + 1]) if i + 1 < len(xs) else xs[i] for i in range(0, len(xs), 2)]
    return xs[0]


def _a_sums(a11, a12, a21, a22):
    return (a11 + a22, a21 + a22, a11, a22, a11 + a12, a21 - a11, a12 - a22)


def _b_sums(b11, b12, b21, b22):
    return (b11 + b22, b11, b12 - b22, b21 - b11, b22, b11 + b12, b21 + b22)


M1, M2, M3, M4, M5, M6, M7 = range(7)


def _tile(j, n=1):
    if isinstance(j, int):
        return slice(j * 128, (j + n) * 128)
    return pl.ds(pl.multiple_of(j * 128, 128), n * 128)


def _pow2(s):
    return pltpu.bitcast((pltpu.bitcast(s, i32) + 0x007FFFFF) & 0x7F800000, f32)


def _pow2_inv(s):
    return pltpu.bitcast(0x7F000000 - pltpu.bitcast(s, i32), f32)


def _pow2_sqrt(s):
    half = lax.shift_right_logical(pltpu.bitcast(s, i32), 1)
    return pltpu.bitcast((half + 0x1FC00000) & 0x7F800000, f32)


def _skew_select(ts, index, unit):
    ts = [ts[-i % 8] for i in range(8)]
    for b in (1, 2, 4):
        take = (index & (unit * b)) != 0
        ts = [jnp.where(take, ts[(i - b) % 8], ts[i]) for i in range(8)]
    return ts


def _kernel(x_hbm, wqkv_hbm, wo_hbm, w1_hbm, b1_ref, w2_hbm, b2_ref, out_hbm,
            ostage, xin, x, wqkv_raw, wo_raw, w1_raw, w2_raw,
            wq, wo, w1, w2, xs1, xs2, os_, hs, q, k, v, pr, ua, xt, part, pre, carry,
            s1, sq, sv, so, sg, gh, sh, b1, b2, stat, isem, osem):
    sub = lax.broadcasted_iota(i32, (8, 128), 0)

    clock = [0]
    queue = []

    def never(shape, dtype):
        return jnp.broadcast_to(jnp.abs(b2[0:1, 0:128]), shape).astype(dtype) < 0

    def plan(window, items):
        lo, hi = window
        entries = [(lo + (hi - lo) * (n + 1) / len(items), f) for n, f in enumerate(items)]
        queue.extend(entries)
        queue.sort(key=lambda e: e[0])
        return entries

    def finish(entries):
        for e in entries:
            if e in queue:
                queue.remove(e)
                e[1]()

    def flush(until):
        vals = []
        while queue and queue[0][0] <= until:
            vals.append(queue.pop(0)[1]())
        return vals

    def tie(operand, r, until):
        vals = flush(until)
        if not vals:
            return operand
        d = _tree(jnp.add, vals)
        d = jnp.concatenate([d, d], axis=0).astype(bf16)
        parts = [operand[:r], jnp.where(never((16, 128), bf16), d, operand[r:r + 16]), operand[r + 16:]]
        return jnp.concatenate([p for p in parts if p.shape[0]], axis=0)

    last = {}
    recent = []

    def after(key, val):
        if key not in last:
            return val
        return jnp.where(never(val.shape, f32), last[key], val)

    def mm(a_ref, w_ref, i, c):
        kt = a_ref.shape[1]
        ls = [a_ref[i, t] for t in range(kt)]
        rs = [w_ref[i, 2 * c + n] for n in range(2)]
        t0 = clock[0]
        clock[0] = t0 + 128 * kt
        if kt == 4:
            out = []
            for n in range(2):
                l0 = ls[0]
                for r in range(0, HM, 64):
                    l0 = tie(l0, r, t0 + n * 256 + r + 63)
                out.append(jnp.dot(jnp.concatenate([l0] + ls[1:], axis=1), rs[n], preferred_element_type=f32))
            recent.append(out[1][HM - 16:])
            return jnp.concatenate(out, axis=1)
        for g in range(kt // 4 + 1):
            for r in range(0, HM, 64):
                ls[4 * g] = tie(ls[4 * g], r, t0 + g * 448 + r + 63)
        return jnp.dot(jnp.concatenate(ls, axis=1), jnp.concatenate(rs, axis=1), preferred_element_type=f32)

    def put(dst, i, t0, rows, val):
        for t in range(val.shape[1] // 128):
            dst[i, t0 + t, rows, :] = val[:, _tile(t)].astype(bf16)

    def put_a(dst, r, ua_):
        ua[r:r + 16, :] = ua_
        put(dst, M3, 0, slice(r, r + 16), ua_[:, :512])
        put(dst, M5, 0, slice(r, r + 16), ua_[:, :512] + ua_[:, 512:])

    def put_b(dst, r, ub):
        ss = _a_sums(ua[r:r + 16, :512], ua[r:r + 16, 512:], ub[:, :512], ub[:, 512:])
        for i in (M1, M2, M4, M6, M7):
            put(dst, i, 0, slice(r, r + 16), ss[i])

    def ln(xv, chain=False, key='ln'):
        if chain:
            xv = jnp.concatenate([after(key, xv[:, :128]), xv[:, 128:]], axis=1)
        z = xv - jnp.sum(xv, axis=1, keepdims=True) * (1.0 / D)
        var = jnp.sum(z * z, axis=1, keepdims=True) * (1.0 / D)
        var = jnp.broadcast_to(var, (xv.shape[0], 128))
        if chain and not (RL and key == 'ln1'):
            last[key] = var
        size = _pow2_sqrt(jnp.maximum(var, TINY))
        g = _pow2_inv(size)
        u = jnp.concatenate([z[:, _tile(j)] * g for j in range(8)], axis=1)
        return u, lax.rsqrt(var + EPS) * size

    def ln1(base, n, r, chain=False):
        if chain and RL:
            last['ln1'] = recent[-RL]
        ua_, sa = ln(x[pl.ds(pl.multiple_of(base + r, n), n), :], chain, 'ln1')
        ub, sb = ln(x[pl.ds(pl.multiple_of(base + HM + r, n), n), :], chain, 'ln1')
        ss = _a_sums(ua_[:, :512], ua_[:, 512:], ub[:, :512], ub[:, 512:])
        for i, val in enumerate(ss):
            put(xs1, i, 0, slice(r, r + n), val)
        for r0, s in ((r, sa), (HM + r, sb)):
            s1[r0:r0 + n, :] = s
            sq[r0:r0 + n, :] = s * QSCALE
            sv[HALO + r0:HALO + r0 + n, :] = _pow2(s)
        if CV1 and chain:
            tok = _tree(jnp.maximum, [ss[i][:, _tile(t)] for i in CV1 for t in range(4)])
            if not RL:
                last['ln1'] = tok
            return jnp.maximum(tok[0:8], tok[8:16])
        return (sa + sb)[0:8]

    def ln2(half, r, chain):
        rows = slice(half * HM + r, half * HM + r + 16)
        u, s = ln(xt[rows, :], chain)
        (put_b if half else put_a)(xs2, r, u)
        p = s * s * stat[0:1, :] + stat[1:2, :]
        size = _pow2_sqrt(p)
        g = _pow2_inv(size)
        gh[rows, :] = g
        sg[rows, :] = s * g
        sh[rows, :] = size * size

    def qkv_dst(g, j, half):
        if g == 0:
            return q.at[j, pl.ds(half * HM, HM), :]
        return (k, v)[g - 1].at[j, pl.ds(HALO + half * HM, HM), :]

    def qkv_p1(g, c):
        sc = (sq if g == 0 else s1)[0:HM, :]
        sc = jnp.concatenate([sc, sc], axis=1)
        md = P(mm, xs1, wq, c=g * 2 + c)

        def out(j, half, val):
            for t in range(2):
                qkv_dst(g, c * 2 + j + t, half)[...] = val[:, _tile(t)]
        m3 = md(M3)
        m5 = md(M5)
        out(4, 0, (m3 + m5) * sc)
        m1 = md(M1)
        out(4, 1, m1 + m3)
        acc = m1 - m5
        m4 = md(M4)
        out(0, 1, m4)
        out(0, 0, (acc + m4 + md(M7)) * sc)

    def qkv_p2(g, c):
        sc = (sq if g == 0 else s1)[HM:TM, :]
        m2 = mm(xs1, wq, M2, g * 2 + c)
        acc = []
        for t in range(2):
            l, r = qkv_dst(g, c * 2 + t, 1), qkv_dst(g, c * 2 + t + 4, 1)
            l[...] = (l[...] + m2[:, _tile(t)]) * sc
            acc.append(r[...] - m2[:, _tile(t)])
        m6 = mm(xs1, wq, M6, g * 2 + c)
        for t in range(2):
            qkv_dst(g, c * 2 + t + 4, 1)[...] = (acc[t] + m6[:, _tile(t)]) * sc

    def window(ref, lead, r):
        return [ref[lead + (pl.ds(HALO + r - DIL * w, 8), slice(None))] for w in range(W)]

    def qk8(r, first, chain):
        qs = [q[j, r:r + 8, :] for j in range(8)]
        if chain:
            qs = [after('qk', t) for t in qs]
        ks = [window(k, (j,), r) for j in range(8)]
        ls = []
        for w in range(W):
            p = _tree(jnp.add, [qs[j] * ks[j][w] for j in range(8)])
            p = (p + pltpu.roll(p, 64, 1)) + (pltpu.roll(p, 32, 1) + pltpu.roll(p, 96, 1))
            if r - DIL * w < 0:
                p = jnp.where(jnp.logical_and(first, sub + (r - DIL * w) < 0), NEG, p)
            ls.append(p)
        last['qk'] = ls[0]
        m = _tree(jnp.maximum, ls)
        es = [jnp.exp2(l - m) for l in ls]
        sc = _tree(jnp.maximum, window(sv, (), r))
        so[r:r + 8, :] = sc
        den = _tree(jnp.add, es)
        inv = pltpu.reciprocal(den, approx=True)
        inv = inv * (2.0 - den * inv) * _pow2_inv(sc)
        for w in range(W):
            pr[w, r:r + 8, :] = es[w] * inv
        return inv

    def pv8(r):
        ps = [pr[w, r:r + 8, :] for w in range(W)]
        return jnp.concatenate(
            [_tree(jnp.add, [a * b for a, b in zip(ps, window(v, (j,), r))]) for j in range(8)], axis=1)

    def pv16(half, r):
        r0 = half * HM + r
        (put_b if half else put_a)(os_, r, jnp.concatenate([pv8(r0), pv8(r0 + 8)], axis=0))

    def v_first(first):
        for j in range(8):
            v0 = jnp.broadcast_to(v[j, HALO:HALO + 1, :], (HALO, 128))
            v[j, 0:HALO, :] = jnp.where(first, v0, v[j, 0:HALO, :])

    def halo_save():
        sv[0:HALO, :] = sv[TM:TM + HALO, :]
        for j in range(8):
            k[j, 0:HALO, :] = k[j, TM:TM + HALO, :]
            v[j, 0:HALO, :] = v[j, TM:TM + HALO, :]

    def acc_x(base, half, j, val):
        rows = pl.ds(pl.multiple_of(base + half * HM, HM), HM)
        sc = so[half * HM:(half + 1) * HM, :]
        for t in range(2):
            r = x[rows, _tile(j + t)] + val[:, _tile(t)] * sc
            xt[half * HM:(half + 1) * HM, _tile(j + t)] = r
            if half:
                x[rows, _tile(j + t)] = r

    def wo_p1(base, c):
        cols = _tile(c * 2, 2)
        m3 = mm(os_, wo, M3, c)
        part[2, :, cols] = m3
        m5 = mm(os_, wo, M5, c)
        part[0, :, cols] = m5
        acc_x(base, 0, 4 + c * 2, m3 + m5)

    def wo_p2(base, c):
        cols = _tile(c * 2, 2)
        m1 = mm(os_, wo, M1, c)
        part[2, :, cols] = part[2, :, cols] + m1
        acc = m1 - part[0, :, cols]
        m4 = mm(os_, wo, M4, c)
        part[1, :, cols] = m4
        acc_x(base, 0, c * 2, acc + m4 + mm(os_, wo, M7, c))

    def wo_p3(base, c):
        cols = _tile(c * 2, 2)
        m2 = mm(os_, wo, M2, c)
        acc_x(base, 1, c * 2, part[1, :, cols] + m2)
        acc = part[2, :, cols] - m2
        acc_x(base, 1, 4 + c * 2, acc + mm(os_, wo, M6, c))

    def w1_pre(c):
        pre[0, :, _tile(c * 2, 2)] = mm(xs2, w1, M3, c)
        pre[1, :, _tile(c * 2, 2)] = mm(xs2, w1, M5, c)

    def w1_chunk(c):
        md = P(mm, xs2, w1, c=c)

        def act(z, half, side):
            rows = slice(half * HM, (half + 1) * HM)
            out = []
            for t in range(2):
                b = b1[0:1, _tile(side * 14 + c * 2 + t)]
                y = jnp.maximum(z[:, _tile(t)] * sg[rows, :] + gh[rows, :] * b, 0.0)
                out.append(y * y)
            return jnp.concatenate(out, axis=1)

        def out(i, val):
            put(hs, i, c * 2, slice(0, HM), val)
        if c < NPRE:
            m3, m5 = pre[0, :, _tile(c * 2, 2)], pre[1, :, _tile(c * 2, 2)]
        else:
            m3, m5 = md(M3), md(M5)
        h12 = act(m3 + m5, 0, 1)
        m4 = md(M4)
        acc1 = m4 - m5
        m2 = md(M2)
        h21 = act(m4 + m2, 1, 0)
        acc2 = m3 - m2
        m1 = md(M1)
        acc1, acc2 = acc1 + m1, acc2 + m1
        h22 = act(acc2 + md(M6), 1, 1)
        out(M2, h21 + h22)
        out(M4, h22)
        out(M7, h12 - h22)
        h11 = act(acc1 + md(M7), 0, 0)
        if c == G1:
            last['ln1'] = h11[0:16, 0:128]
        out(M1, h11 + h22)
        out(M3, h11)
        out(M5, h11 + h12)
        out(M6, h21 - h11)

    def fin(res, base, slot, half, c, side, val, sc):
        rows = pl.ds(pl.multiple_of(base + half * HM, HM), HM)
        for t in range(2):
            cols = _tile(side * 4 + c * 2 + t)
            r = res(rows, cols) + val[:, _tile(t)] * sc + b2[:, cols][0:1]
            x[rows, cols] = r
            ostage[slot, half, :, cols] = r.astype(bf16)

    def w2_p1(base, slot, c):
        done = P(fin, lambda rows, cols: xt[0:HM, cols], base, slot, 0, c, sc=sh[0:HM, :])
        m3 = mm(hs, w2, M3, c)
        m5 = mm(hs, w2, M5, c)
        done(1, m3 + m5)
        m1 = mm(hs, w2, M1, c)
        carry[1, :, _tile(2 * c, 2)] = m1 + m3
        acc = m1 - m5
        m4 = mm(hs, w2, M4, c)
        carry[0, :, _tile(2 * c, 2)] = m4
        done(0, acc + m4 + mm(hs, w2, M7, c))
        if c == 1:
            carry[2, :, 0:128] = sh[HM:TM, :]

    def w2_p2(base, slot, c):
        done = P(fin, lambda rows, cols: x[rows, cols], base, slot, 1, c, sc=carry[2, :, 0:128])
        m2 = mm(hs, w2, M2, c)
        done(0, carry[0, :, _tile(2 * c, 2)] + m2)
        acc = carry[1, :, _tile(2 * c, 2)] - m2
        done(1, acc + mm(hs, w2, M6, c))

    def put_sums(dst, rows, t, blocks):
        bits = []
        for i, s in enumerate(_b_sums(*blocks)):
            put(dst, i, t, rows, s)
            if i in (M4, M7):
                bits += [pltpu.bitcast(s[a:a + 8, 0:128], i32) for a in range(0, s.shape[0], 16)]
        return pltpu.bitcast(_tree(jnp.bitwise_or, bits), f32)

    def permuted(r, n, g):
        lane = lax.broadcasted_iota(i32, (n // 2, 128), 1)
        src = ((lane & 31) << 2) | (lane >> 5)
        ts = [pltpu.bitcast(wqkv_raw[r:r + n, _tile(g * 8 + j)], u32) for j in range(8)]
        ts = [pltpu.roll(t, 4 * j, 1) if j else t for j, t in enumerate(ts)]
        ts = _skew_select(ts, lane, 4)
        return [pltpu.bitcast(jnp.take_along_axis(t, (src + 4 * j) & 127, axis=1), bf16).astype(f32)
                for j, t in enumerate(ts)]

    def prep_qkv(g, n, r):
        top, bot = permuted(r, n, g), permuted(512 + r, n, g)
        return _tree(jnp.maximum, [
            put_sums(wq, slice(r, r + n), g * 4 + t, (top[t], top[t + 4], bot[t], bot[t + 4])) for t in range(4)])

    def prep_wo(t, d3, h1):
        blk = {}
        for side in range(2):
            for d4 in range(2):
                for h0 in range(2):
                    src = []
                    for hh in range(8):
                        r = hh * 128 + h1 * 64 + h0 * 32 + d4 * 16
                        val = wo_raw[r:r + 16, _tile(t + 4 * side)].astype(f32)[8 * d3:8 * d3 + 8]
                        src.append(pltpu.roll(val, hh, 0) if hh else val)
                    for dl, val in enumerate(_skew_select(src, sub, 1)):
                        blk[d4, side, h0, dl] = pltpu.roll(val, 8 - dl, 0) if dl else val
        out = []
        for dl in range(8):
            r = d3 * 256 + dl * 32 + h1 * 16
            out.append(put_sums(wo, slice(r, r + 16), t,
                                [jnp.concatenate([blk[d4, side, 0, dl], blk[d4, side, 1, dl]], axis=0)
                                 for d4 in range(2) for side in range(2)]))
        return _tree(jnp.maximum, out)

    def w1_blocks(t, r):
        return [w1_raw[rr:rr + 64, _tile(j)].astype(f32) for rr in (r, 512 + r) for j in (t, t + 14)]

    def prep_w1(t, r):
        return put_sums(w1, slice(r, r + 64), t, w1_blocks(t, r))

    def prep_w1_first():
        es = []
        for t in range(2):
            for r in range(0, 512, 64):
                blocks = w1_blocks(t, r)
                put_sums(w1, slice(r, r + 64), t, blocks)
                e = _tree(jnp.add, [y * y for y in blocks])
                es.append(_tree(jnp.add, [e[a:a + 8] for a in range(0, 64, 8)]))
        tot = jnp.sum(jnp.sum(_tree(jnp.add, es), axis=1, keepdims=True), axis=0, keepdims=True)
        stat[0:1, :] = jnp.broadcast_to(tot * (1.0 / 512), (1, 128))
        bb = b1[0:1, :]
        stat[1:2, :] = jnp.broadcast_to(jnp.sum(bb * bb, axis=1, keepdims=True) * (1.0 / F) + TINY, (1, 128))

    def prep_w2(t, r):
        return put_sums(w2, slice(r, r + 64), t,
                        [w2_raw[rr:rr + 64, _tile(j)].astype(f32) for rr in (r, HF + r) for j in (t, t + 4)])

    def cvt_x(r):
        val = xin[r:r + 64, :].astype(f32)
        x[r:r + 64, :] = val
        return _tree(jnp.add, [val[a:a + 8, 0:128] for a in range(0, 64, 8)])

    def dma(src, dst, block, i):
        return pltpu.make_async_copy(src.at[block], dst.at[block], isem.at[i])

    full = slice(None)
    cp_x0 = [[dma(x_hbm, xin, (pl.ds(half * HM + r, 128), full), 10 + 1024 // RQ + 2 * (r // 128) + half)
              for half in range(2)] for r in range(0, HM, 128)]
    cp_x1 = dma(x_hbm, xin, (pl.ds(TM, S - TM), full), 1)
    cp_k, cp_v = (dma(wqkv_hbm, wqkv_raw, (full, pl.ds(g * D, D)), 1 + g) for g in (1, 2))
    cp_wo = dma(wo_hbm, wo_raw, (full, full), 4)
    cp_w2 = dma(w2_hbm, w2_raw, (full, full), 5)
    cp_w1 = dma(w1_hbm, w1_raw, (full, full), 6)
    cp_q = [[dma(wqkv_hbm, wqkv_raw, (pl.ds(s * 512 + n * RQ, RQ), pl.ds(0, D)), 10 + 2 * n + s) for s in range(2)]
            for n in range(512 // RQ)]

    def step(t, peeled):
        base = (t % NT) * TM
        pbase = ((t + NT - 1) % NT) * TM
        nbase = ((t + 1) % NT) * TM
        slot = t % 2
        first = t % NT == 0
        clock[0] = 0
        last.clear()
        qk_items = [P(qk8, r, first, not peeled) for r in range(0, TM, 8)]
        ln1_items = [P(ln1, nbase, 16, r, G1 is not None and not peeled) for r in range(0, HM, 16)]

        def two(f, *a):
            for c in range(2):
                f(*a, c)
        if peeled:
            for cp in [*sum(cp_x0 + cp_q, []), cp_k, cp_v, cp_wo, cp_w1, cp_w2, cp_x1]:
                cp.start()
            sv[0:HALO, :] = jnp.zeros((HALO, 128), f32)
            k[:, 0:HALO, :] = jnp.zeros((8, HALO, 128), f32)
            v[:, 0:HALO, :] = jnp.zeros((8, HALO, 128), f32)
            b1[0:1, :] = b1_ref[...].astype(f32).reshape(1, F)
            b2[...] = jnp.broadcast_to(b2_ref[...].astype(f32).reshape(1, D), (8, D))
            ostage[slot, 1] = jnp.zeros((HM, D), bf16)
            for r, cps in zip(range(0, HM, 128), cp_x0):
                for cp in cps:
                    cp.wait()
                for rr in (r, r + 64, HM + r, HM + r + 64):
                    cvt_x(rr)
                ln1(base, 128, r)
            for n, cps in enumerate(cp_q):
                for cp in cps:
                    cp.wait()
                for r in range(n * RQ, (n + 1) * RQ, 128):
                    prep_qkv(0, 128, r)
            attn = plan(QKF, qk_items)
            qkv_p1(0, 0)
            qkv_p2(0, 0)
            cp_k.wait()
            job = plan(TK, [P(prep_qkv, 1, 64, r) for r in range(0, 512, 64)])
            qkv_p1(0, 1)
            qkv_p2(0, 1)
            finish(job)
            qkv_p1(1, 0)
            cp_v.wait()
            cp_wo.wait()
            job = plan(TV, [P(prep_qkv, 2, 64, r) for r in range(0, 512, 64)])
            job_wo = plan(TO, [P(prep_wo, tt, d3, h1) for tt in range(4) for d3 in range(2) for h1 in range(2)])
            qkv_p1(1, 1)
            two(qkv_p2, 1)
            finish(job)
        else:
            attn = plan(QK, qk_items)
            if G1 is None:
                job_ln1 = plan(L1, ln1_items)
            two(qkv_p1, 0)
            two(qkv_p1, 1)
            two(qkv_p2, 0)
            two(qkv_p2, 1)
        two(qkv_p1, 2)
        v_first(first)
        two(qkv_p2, 2)
        finish(attn)
        for half in range(2):
            for r in range(0, HM, 16):
                pv16(half, r)
        if peeled:
            finish(job_wo)
        else:
            w2_p2(pbase, slot, 0)
        two(wo_p1, base)
        halo_save()
        if peeled:
            cp_w1.wait()
            prep_w1_first()
            jobs = {}
            for c in range(1, 7):
                lo = clock[0] + TA[0] + (c - 1) * TA[1]
                jobs[c] = plan((lo, lo + TA[1]), [P(prep_w1, tt, r) for tt in (2 * c, 2 * c + 1) for r in range(0, 512, 64)])
        two(wo_p2, base)
        two(wo_p3, base)
        if not peeled:
            w2_p2(pbase, slot, 1)
        for half in range(2):
            for r in range(0, HM, 16):
                ln2(half, r, not peeled)
        for c in range(NPRE):
            if peeled and c:
                finish(jobs[c])
            w1_pre(c)
        for c in range(7):
            if peeled and c == CB:
                for cc in jobs:
                    finish(jobs[cc])
                cp_w2.wait()
                cp_x1.wait()
                job = plan((clock[0] + T2[0], clock[0] + T2[1]),
                           [P(prep_w2, tt, r) for tt in range(4) for r in range(0, HF, 64)])
            w1_chunk(c)
            if c == G1 and not peeled:
                job_ln1 = plan((clock[0] + G2[0], clock[0] + G2[1]), ln1_items)
        if peeled:
            finish(job)
            for r in range(TM, 2 * TM, 64):
                cvt_x(r)
            late = (clock[0] + 1000, clock[0] + 16000)
            job_ln1 = plan(late, ln1_items)
            job = plan(late, [P(cvt_x, r) for r in range(2 * TM, S, 64)])
        else:
            finish(job_ln1)
        two(w2_p1, base, slot)
        if peeled:
            finish(job_ln1)
            finish(job)
        assert not queue

    def out_copies(t):
        return [pltpu.make_async_copy(
            ostage.at[t % 2, half],
            out_hbm.at[pl.ds(pl.multiple_of(((t + (NT - 1) * half) % NT) * TM + half * HM, HM), HM), :],
            osem.at[half]) for half in range(2)]

    if MODE != 'body':
        step(0, True)

    def body(t, c):
        cps = out_copies(t - 1)
        for cp in cps:
            cp.start()
        step(t, False)
        for cp in cps:
            cp.wait()
        return c

    lax.fori_loop(1, 2 * NT, body, 0)
    cps = out_copies(2 * NT - 1)
    for cp in cps:
        cp.start()

    def last_copies(c):
        return [pltpu.make_async_copy(ostage.at[0, 1, :, _tile(4 * side + 2 * c, 2)],
                                      out_hbm.at[pl.ds(S - HM, HM), _tile(4 * side + 2 * c, 2)],
                                      osem.at[2 + 2 * c + side]) for side in range(2)]

    def last_rows(c, _):
        w2_p2(S - TM, 0, c)
        for cp in last_copies(c):
            cp.start()

    lax.fori_loop(0, 2, last_rows, None)
    for cp in cps + last_copies(0) + last_copies(1):
        cp.wait()


@jax.jit
def pallas_interleave_layers__sliding_local_dilated__dense_activation_squared_relu__prompt_kernel(A_x, A_wqkv, A_wo, B_x, B_w1, B_b1, B_w2, B_b2):
    del B_x
    hbm = pl.BlockSpec(memory_space=pl.ANY)
    vmem = pl.BlockSpec(memory_space=pltpu.VMEM)
    V = pltpu.VMEM
    out = pl.pallas_call(
        _kernel,
        in_specs=[hbm, hbm, hbm, hbm, vmem, hbm, vmem],
        out_specs=hbm,
        out_shape=jax.ShapeDtypeStruct((S, D), bf16),
        scratch_shapes=[
            V((2, 2, HM, D), bf16), V((S, D), bf16), V((S, D), f32),
            V((D, 3 * D), bf16), V((D, D), bf16), V((D, F), bf16), V((F, D), bf16),
            V((7, 12, 512, 128), bf16), V((7, 4, 512, 128), bf16),
            V((7, 14, 512, 128), bf16), V((7, 4, HF, 128), bf16),
            V((7, 4, HM, 128), bf16), V((7, 4, HM, 128), bf16), V((7, 4, HM, 128), bf16), V((7, 14, HM, 128), bf16),
            V((8, TM, 128), f32), V((8, TM + HALO, 128), f32), V((8, TM + HALO, 128), f32), V((W, TM, 128), f32),
            V((HM, D), f32), V((TM, D), f32),
            V((3, HM, 512), f32), V((2, HM, 256 * NPRE), f32), V((3, HM, 512), f32),
            V((TM, 128), f32), V((TM, 128), f32), V((TM + HALO, 128), f32), V((TM, 128), f32),
            V((TM, 128), f32), V((TM, 128), f32), V((TM, 128), f32),
            V((8, F), f32), V((8, D), f32), V((8, 128), f32),
            pltpu.SemaphoreType.DMA((14 + 1024 // RQ,)), pltpu.SemaphoreType.DMA((6,)),
        ],
        compiler_params=pltpu.CompilerParams(vmem_limit_bytes=127 * 1024 * 1024),
    )(A_x.reshape(S, D), A_wqkv, A_wo, B_w1, B_b1, B_w2, B_b2)
    return out.reshape(1, S, D)
```

```python
import functools

import jax
import jax.numpy as jnp
import numpy as np
from jax import lax
import jax.experimental.pallas as pl
import jax.experimental.pallas.tpu as pltpu

S, D, F = 2048, 1024, 3584
DH, W, DIL = 32, 8, 2
TM = 512
HM = TM // 2
HF = F // 2
NT = S // TM
HALO = 16
EPS = 1e-5
TINY = 1e-30
QSCALE = float(DH ** -0.5 * np.log2(np.e))
NEG = float(-1e9 * np.log2(np.e))
NPRE = 4
RQ = 256
QK = (10850, 21500)
QKF = (14000, 21400)
L1 = (1000, 16000)
TK = (3900, 6600)
TV = (10000, 13800)
TO = (12500, 21400)
TA = (2000, 2000)
T2 = (500, 15000)
CB = 2
f32, bf16, u32, i32 = jnp.float32, jnp.bfloat16, jnp.uint32, jnp.int32
P = functools.partial


def _tree(op, xs):
    xs = list(xs)
    while len(xs) > 1:
        xs = [op(xs[i], xs[i + 1]) if i + 1 < len(xs) else xs[i] for i in range(0, len(xs), 2)]
    return xs[0]


def _a_sums(a11, a12, a21, a22):
    return (a11 + a22, a21 + a22, a11, a22, a11 + a12, a21 - a11, a12 - a22)


def _b_sums(b11, b12, b21, b22):
    return (b11 + b22, b11, b12 - b22, b21 - b11, b22, b11 + b12, b21 + b22)


M1, M2, M3, M4, M5, M6, M7 = range(7)


def _tile(j, n=1):
    if isinstance(j, int):
        return slice(j * 128, (j + n) * 128)
    return pl.ds(pl.multiple_of(j * 128, 128), n * 128)


def _pow2(s):
    return pltpu.bitcast((pltpu.bitcast(s, i32) + 0x007FFFFF) & 0x7F800000, f32)


def _pow2_inv(s):
    return pltpu.bitcast(0x7F000000 - pltpu.bitcast(s, i32), f32)


def _pow2_sqrt(s):
    half = lax.shift_right_logical(pltpu.bitcast(s, i32), 1)
    return pltpu.bitcast((half + 0x1FC00000) & 0x7F800000, f32)


def _skew_select(ts, index, unit):
    ts = [ts[-i % 8] for i in range(8)]
    for b in (1, 2, 4):
        take = (index & (unit * b)) != 0
        ts = [jnp.where(take, ts[(i - b) % 8], ts[i]) for i in range(8)]
    return ts


def _kernel(x_hbm, wqkv_hbm, wo_hbm, w1_hbm, b1_ref, w2_hbm, b2_ref, out_hbm,
            ostage, xin, x, wqkv_raw, wo_raw, w1_raw, w2_raw,
            wq, wo, w1, w2, xs1, xs2, os_, hs, q, k, v, pr, ua, xt, part, pre, carry,
            s1, sq, sv, so, sg, gh, sh, b1, b2, stat, isem, osem):
    sub = lax.broadcasted_iota(i32, (8, 128), 0)

    clock = [0]
    queue = []

    def never(shape, dtype):
        return jnp.broadcast_to(jnp.abs(b2[0:1, 0:128]), shape).astype(dtype) < 0

    def plan(window, items):
        lo, hi = window
        entries = [(lo + (hi - lo) * (n + 1) / len(items), f) for n, f in enumerate(items)]
        queue.extend(entries)
        queue.sort(key=lambda e: e[0])
        return entries

    def finish(entries):
        for e in entries:
            if e in queue:
                queue.remove(e)
                e[1]()

    def flush(until):
        vals = []
        while queue and queue[0][0] <= until:
            vals.append(queue.pop(0)[1]())
        return vals

    def tie(operand, r, until):
        vals = flush(until)
        if not vals:
            return operand
        d = _tree(jnp.add, vals)
        d = jnp.concatenate([d, d], axis=0).astype(bf16)
        parts = [operand[:r], jnp.where(never((16, 128), bf16), d, operand[r:r + 16]), operand[r + 16:]]
        return jnp.concatenate([p for p in parts if p.shape[0]], axis=0)

    last = {}

    def after(key, val):
        if key not in last:
            return val
        return jnp.where(never(val.shape, f32), last[key], val)

    def mm(a_ref, w_ref, i, c):
        kt = a_ref.shape[1]
        ls = [a_ref[i, t] for t in range(kt)]
        rs = [w_ref[i, 2 * c + n] for n in range(2)]
        t0 = clock[0]
        clock[0] = t0 + 128 * kt
        if kt == 4:
            out = []
            for n in range(2):
                l0 = ls[0]
                for r in range(0, HM, 64):
                    l0 = tie(l0, r, t0 + n * 256 + r + 63)
                out.append(jnp.dot(jnp.concatenate([l0] + ls[1:], axis=1), rs[n], preferred_element_type=f32))
            return jnp.concatenate(out, axis=1)
        for g in range(kt // 4 + 1):
            for r in range(0, HM, 64):
                ls[4 * g] = tie(ls[4 * g], r, t0 + g * 448 + r + 63)
        return jnp.dot(jnp.concatenate(ls, axis=1), jnp.concatenate(rs, axis=1), preferred_element_type=f32)

    def put(dst, i, t0, rows, val):
        for t in range(val.shape[1] // 128):
            dst[i, t0 + t, rows, :] = val[:, _tile(t)].astype(bf16)

    def put_a(dst, r, ua_):
        ua[r:r + 16, :] = ua_
        put(dst, M3, 0, slice(r, r + 16), ua_[:, :512])
        put(dst, M5, 0, slice(r, r + 16), ua_[:, :512] + ua_[:, 512:])

    def put_b(dst, r, ub):
        ss = _a_sums(ua[r:r + 16, :512], ua[r:r + 16, 512:], ub[:, :512], ub[:, 512:])
        for i in (M1, M2, M4, M6, M7):
            put(dst, i, 0, slice(r, r + 16), ss[i])

    def ln(xv, chain=False, key='ln'):
        if chain:
            xv = jnp.concatenate([after(key, xv[:, :128]), xv[:, 128:]], axis=1)
        z = xv - jnp.sum(xv, axis=1, keepdims=True) * (1.0 / D)
        var = jnp.sum(z * z, axis=1, keepdims=True) * (1.0 / D)
        var = jnp.broadcast_to(var, (xv.shape[0], 128))
        if chain:
            last[key] = var
        size = _pow2_sqrt(jnp.maximum(var, TINY))
        g = _pow2_inv(size)
        u = jnp.concatenate([z[:, _tile(j)] * g for j in range(8)], axis=1)
        return u, lax.rsqrt(var + EPS) * size

    def ln1(base, n, r, chain=False):
        ua_, sa = ln(x[pl.ds(pl.multiple_of(base + r, n), n), :], chain, 'ln1')
        ub, sb = ln(x[pl.ds(pl.multiple_of(base + HM + r, n), n), :], chain, 'ln1')
        ss = _a_sums(ua_[:, :512], ua_[:, 512:], ub[:, :512], ub[:, 512:])
        for i, val in enumerate(ss):
            put(xs1, i, 0, slice(r, r + n), val)
        for r0, s in ((r, sa), (HM + r, sb)):
            s1[r0:r0 + n, :] = s
            sq[r0:r0 + n, :] = s * QSCALE
            sv[HALO + r0:HALO + r0 + n, :] = _pow2(s)
        return (sa + sb)[0:8]

    def ln2(half, r, chain):
        rows = slice(half * HM + r, half * HM + r + 16)
        u, s = ln(xt[rows, :], chain)
        (put_b if half else put_a)(xs2, r, u)
        p = s * s * stat[0:1, :] + stat[1:2, :]
        size = _pow2_sqrt(p)
        g = _pow2_inv(size)
        gh[rows, :] = g
        sg[rows, :] = s * g
        sh[rows, :] = size * size

    def qkv_dst(g, j, half):
        if g == 0:
            return q.at[j, pl.ds(half * HM, HM), :]
        return (k, v)[g - 1].at[j, pl.ds(HALO + half * HM, HM), :]

    def qkv_p1(g, c):
        sc = (sq if g == 0 else s1)[0:HM, :]
        sc = jnp.concatenate([sc, sc], axis=1)
        md = P(mm, xs1, wq, c=g * 2 + c)

        def out(j, half, val):
            for t in range(2):
                qkv_dst(g, c * 2 + j + t, half)[...] = val[:, _tile(t)]
        m3 = md(M3)
        m5 = md(M5)
        out(4, 0, (m3 + m5) * sc)
        m1 = md(M1)
        out(4, 1, m1 + m3)
        acc = m1 - m5
        m4 = md(M4)
        out(0, 1, m4)
        out(0, 0, (acc + m4 + md(M7)) * sc)

    def qkv_p2(g, c):
        sc = (sq if g == 0 else s1)[HM:TM, :]
        m2 = mm(xs1, wq, M2, g * 2 + c)
        acc = []
        for t in range(2):
            l, r = qkv_dst(g, c * 2 + t, 1), qkv_dst(g, c * 2 + t + 4, 1)
            l[...] = (l[...] + m2[:, _tile(t)]) * sc
            acc.append(r[...] - m2[:, _tile(t)])
        m6 = mm(xs1, wq, M6, g * 2 + c)
        for t in range(2):
            qkv_dst(g, c * 2 + t + 4, 1)[...] = (acc[t] + m6[:, _tile(t)]) * sc

    def window(ref, lead, r):
        return [ref[lead + (pl.ds(HALO + r - DIL * w, 8), slice(None))] for w in range(W)]

    def qk8(r, first, chain):
        qs = [q[j, r:r + 8, :] for j in range(8)]
        if chain:
            qs = [after('qk', t) for t in qs]
        ks = [window(k, (j,), r) for j in range(8)]
        ls = []
        for w in range(W):
            p = _tree(jnp.add, [qs[j] * ks[j][w] for j in range(8)])
            p = (p + pltpu.roll(p, 64, 1)) + (pltpu.roll(p, 32, 1) + pltpu.roll(p, 96, 1))
            if r - DIL * w < 0:
                p = jnp.where(jnp.logical_and(first, sub + (r - DIL * w) < 0), NEG, p)
            ls.append(p)
        last['qk'] = ls[0]
        m = _tree(jnp.maximum, ls)
        es = [jnp.exp2(l - m) for l in ls]
        sc = _tree(jnp.maximum, window(sv, (), r))
        so[r:r + 8, :] = sc
        den = _tree(jnp.add, es)
        inv = pltpu.reciprocal(den, approx=True)
        inv = inv * (2.0 - den * inv) * _pow2_inv(sc)
        for w in range(W):
            pr[w, r:r + 8, :] = es[w] * inv
        return inv

    def pv8(r):
        ps = [pr[w, r:r + 8, :] for w in range(W)]
        return jnp.concatenate(
            [_tree(jnp.add, [a * b for a, b in zip(ps, window(v, (j,), r))]) for j in range(8)], axis=1)

    def pv16(half, r):
        r0 = half * HM + r
        (put_b if half else put_a)(os_, r, jnp.concatenate([pv8(r0), pv8(r0 + 8)], axis=0))

    def v_first(first):
        for j in range(8):
            v0 = jnp.broadcast_to(v[j, HALO:HALO + 1, :], (HALO, 128))
            v[j, 0:HALO, :] = jnp.where(first, v0, v[j, 0:HALO, :])

    def halo_save():
        sv[0:HALO, :] = sv[TM:TM + HALO, :]
        for j in range(8):
            k[j, 0:HALO, :] = k[j, TM:TM + HALO, :]
            v[j, 0:HALO, :] = v[j, TM:TM + HALO, :]

    def acc_x(base, half, j, val):
        rows = pl.ds(pl.multiple_of(base + half * HM, HM), HM)
        sc = so[half * HM:(half + 1) * HM, :]
        for t in range(2):
            r = x[rows, _tile(j + t)] + val[:, _tile(t)] * sc
            xt[half * HM:(half + 1) * HM, _tile(j + t)] = r
            if half:
                x[rows, _tile(j + t)] = r

    def wo_p1(base, c):
        cols = _tile(c * 2, 2)
        m3 = mm(os_, wo, M3, c)
        part[2, :, cols] = m3
        m5 = mm(os_, wo, M5, c)
        part[0, :, cols] = m5
        acc_x(base, 0, 4 + c * 2, m3 + m5)

    def wo_p2(base, c):
        cols = _tile(c * 2, 2)
        m1 = mm(os_, wo, M1, c)
        part[2, :, cols] = part[2, :, cols] + m1
        acc = m1 - part[0, :, cols]
        m4 = mm(os_, wo, M4, c)
        part[1, :, cols] = m4
        acc_x(base, 0, c * 2, acc + m4 + mm(os_, wo, M7, c))

    def wo_p3(base, c):
        cols = _tile(c * 2, 2)
        m2 = mm(os_, wo, M2, c)
        acc_x(base, 1, c * 2, part[1, :, cols] + m2)
        acc = part[2, :, cols] - m2
        acc_x(base, 1, 4 + c * 2, acc + mm(os_, wo, M6, c))

    def w1_pre(c):
        pre[0, :, _tile(c * 2, 2)] = mm(xs2, w1, M3, c)
        pre[1, :, _tile(c * 2, 2)] = mm(xs2, w1, M5, c)

    def w1_chunk(c, kick):
        md = P(mm, xs2, w1, c=c)

        def act(z, half, side):
            rows = slice(half * HM, (half + 1) * HM)
            out = []
            for t in range(2):
                b = b1[0:1, _tile(side * 14 + c * 2 + t)]
                y = jnp.maximum(z[:, _tile(t)] * sg[rows, :] + gh[rows, :] * b, 0.0)
                out.append(y * y)
            return jnp.concatenate(out, axis=1)

        def out(i, val):
            put(hs, i, c * 2, slice(0, HM), val)
        if c < NPRE:
            m3, m5 = pre[0, :, _tile(c * 2, 2)], pre[1, :, _tile(c * 2, 2)]
        else:
            m3, m5 = md(M3), md(M5)
        h12 = act(m3 + m5, 0, 1)
        m4 = md(M4)
        acc1 = m4 - m5
        m2 = md(M2)
        h21 = act(m4 + m2, 1, 0)
        acc2 = m3 - m2
        m1 = md(M1)
        acc1, acc2 = acc1 + m1, acc2 + m1
        h22 = act(acc2 + md(M6), 1, 1)
        out(M2, h21 + h22)
        out(M4, h22)
        out(M7, h12 - h22)
        h11 = act(acc1 + md(M7), 0, 0)
        if c == 0 and kick:
            last['ln1'] = h11[0:16, 0:128]
        out(M1, h11 + h22)
        out(M3, h11)
        out(M5, h11 + h12)
        out(M6, h21 - h11)

    def fin(res, base, slot, half, c, side, val, sc):
        rows = pl.ds(pl.multiple_of(base + half * HM, HM), HM)
        for t in range(2):
            cols = _tile(side * 4 + c * 2 + t)
            r = res(rows, cols) + val[:, _tile(t)] * sc + b2[:, cols][0:1]
            x[rows, cols] = r
            ostage[slot, half, :, cols] = r.astype(bf16)

    def w2_p1(base, slot, c):
        done = P(fin, lambda rows, cols: xt[0:HM, cols], base, slot, 0, c, sc=sh[0:HM, :])
        m3 = mm(hs, w2, M3, c)
        m5 = mm(hs, w2, M5, c)
        done(1, m3 + m5)
        m1 = mm(hs, w2, M1, c)
        carry[1, :, _tile(2 * c, 2)] = m1 + m3
        acc = m1 - m5
        m4 = mm(hs, w2, M4, c)
        carry[0, :, _tile(2 * c, 2)] = m4
        done(0, acc + m4 + mm(hs, w2, M7, c))
        if c == 1:
            carry[2, :, 0:128] = sh[HM:TM, :]

    def w2_p2(base, slot, c):
        done = P(fin, lambda rows, cols: x[rows, cols], base, slot, 1, c, sc=carry[2, :, 0:128])
        m2 = mm(hs, w2, M2, c)
        done(0, carry[0, :, _tile(2 * c, 2)] + m2)
        acc = carry[1, :, _tile(2 * c, 2)] - m2
        done(1, acc + mm(hs, w2, M6, c))

    def put_sums(dst, rows, t, blocks):
        bits = []
        for i, s in enumerate(_b_sums(*blocks)):
            put(dst, i, t, rows, s)
            if i in (M4, M7):
                bits += [pltpu.bitcast(s[a:a + 8, 0:128], i32) for a in range(0, s.shape[0], 16)]
        return pltpu.bitcast(_tree(jnp.bitwise_or, bits), f32)

    def permuted(r, n, g):
        lane = lax.broadcasted_iota(i32, (n // 2, 128), 1)
        src = ((lane & 31) << 2) | (lane >> 5)
        ts = [pltpu.bitcast(wqkv_raw[r:r + n, _tile(g * 8 + j)], u32) for j in range(8)]
        ts = [pltpu.roll(t, 4 * j, 1) if j else t for j, t in enumerate(ts)]
        ts = _skew_select(ts, lane, 4)
        return [pltpu.bitcast(jnp.take_along_axis(t, (src + 4 * j) & 127, axis=1), bf16).astype(f32)
                for j, t in enumerate(ts)]

    def prep_qkv(g, n, r):
        top, bot = permuted(r, n, g), permuted(512 + r, n, g)
        return _tree(jnp.maximum, [
            put_sums(wq, slice(r, r + n), g * 4 + t, (top[t], top[t + 4], bot[t], bot[t + 4])) for t in range(4)])

    def prep_wo(t, d3, h1):
        blk = {}
        for side in range(2):
            for d4 in range(2):
                for h0 in range(2):
                    src = []
                    for hh in range(8):
                        r = hh * 128 + h1 * 64 + h0 * 32 + d4 * 16
                        val = wo_raw[r:r + 16, _tile(t + 4 * side)].astype(f32)[8 * d3:8 * d3 + 8]
                        src.append(pltpu.roll(val, hh, 0) if hh else val)
                    for dl, val in enumerate(_skew_select(src, sub, 1)):
                        blk[d4, side, h0, dl] = pltpu.roll(val, 8 - dl, 0) if dl else val
        out = []
        for dl in range(8):
            r = d3 * 256 + dl * 32 + h1 * 16
            out.append(put_sums(wo, slice(r, r + 16), t,
                                [jnp.concatenate([blk[d4, side, 0, dl], blk[d4, side, 1, dl]], axis=0)
                                 for d4 in range(2) for side in range(2)]))
        return _tree(jnp.maximum, out)

    def w1_blocks(t, r):
        return [w1_raw[rr:rr + 64, _tile(j)].astype(f32) for rr in (r, 512 + r) for j in (t, t + 14)]

    def prep_w1(t, r):
        return put_sums(w1, slice(r, r + 64), t, w1_blocks(t, r))

    def prep_w1_first():
        es = []
        for t in range(2):
            for r in range(0, 512, 64):
                blocks = w1_blocks(t, r)
                put_sums(w1, slice(r, r + 64), t, blocks)
                e = _tree(jnp.add, [y * y for y in blocks])
                es.append(_tree(jnp.add, [e[a:a + 8] for a in range(0, 64, 8)]))
        tot = jnp.sum(jnp.sum(_tree(jnp.add, es), axis=1, keepdims=True), axis=0, keepdims=True)
        stat[0:1, :] = jnp.broadcast_to(tot * (1.0 / 512), (1, 128))
        bb = b1[0:1, :]
        stat[1:2, :] = jnp.broadcast_to(jnp.sum(bb * bb, axis=1, keepdims=True) * (1.0 / F) + TINY, (1, 128))

    def prep_w2(t, r):
        return put_sums(w2, slice(r, r + 64), t,
                        [w2_raw[rr:rr + 64, _tile(j)].astype(f32) for rr in (r, HF + r) for j in (t, t + 4)])

    def cvt_x(r):
        val = xin[r:r + 64, :].astype(f32)
        x[r:r + 64, :] = val
        return _tree(jnp.add, [val[a:a + 8, 0:128] for a in range(0, 64, 8)])

    def dma(src, dst, block, i):
        return pltpu.make_async_copy(src.at[block], dst.at[block], isem.at[i])

    full = slice(None)
    cp_x0 = [[dma(x_hbm, xin, (pl.ds(half * HM + r, 128), full), 10 + 1024 // RQ + 2 * (r // 128) + half)
              for half in range(2)] for r in range(0, HM, 128)]
    cp_x1 = dma(x_hbm, xin, (pl.ds(TM, S - TM), full), 1)
    cp_k, cp_v = (dma(wqkv_hbm, wqkv_raw, (full, pl.ds(g * D, D)), 1 + g) for g in (1, 2))
    cp_wo = dma(wo_hbm, wo_raw, (full, full), 4)
    cp_w2 = dma(w2_hbm, w2_raw, (full, full), 5)
    cp_w1 = dma(w1_hbm, w1_raw, (full, full), 6)
    cp_q = [[dma(wqkv_hbm, wqkv_raw, (pl.ds(s * 512 + n * RQ, RQ), pl.ds(0, D)), 10 + 2 * n + s) for s in range(2)]
            for n in range(512 // RQ)]

    def step(t, peeled):
        base = (t % NT) * TM
        pbase = ((t + NT - 1) % NT) * TM
        nbase = ((t + 1) % NT) * TM
        slot = t % 2
        first = t % NT == 0
        clock[0] = 0
        last.clear()
        qk_items = [P(qk8, r, first, not peeled) for r in range(0, TM, 8)]
        ln1_items = [P(ln1, nbase, 16, r, True) for r in range(0, HM, 16)]

        def two(f, *a):
            for c in range(2):
                f(*a, c)
        if peeled:
            for cp in [*sum(cp_x0 + cp_q, []), cp_k, cp_v, cp_wo, cp_w1, cp_w2, cp_x1]:
                cp.start()
            sv[0:HALO, :] = jnp.zeros((HALO, 128), f32)
            k[:, 0:HALO, :] = jnp.zeros((8, HALO, 128), f32)
            v[:, 0:HALO, :] = jnp.zeros((8, HALO, 128), f32)
            b1[0:1, :] = b1_ref[...].astype(f32).reshape(1, F)
            b2[...] = jnp.broadcast_to(b2_ref[...].astype(f32).reshape(1, D), (8, D))
            ostage[slot, 1] = jnp.zeros((HM, D), bf16)
            for r, cps in zip(range(0, HM, 128), cp_x0):
                for cp in cps:
                    cp.wait()
                for rr in (r, r + 64, HM + r, HM + r + 64):
                    cvt_x(rr)
                ln1(base, 128, r)
            for n, cps in enumerate(cp_q):
                for cp in cps:
                    cp.wait()
                for r in range(n * RQ, (n + 1) * RQ, 128):
                    prep_qkv(0, 128, r)
            attn = plan(QKF, qk_items)
            qkv_p1(0, 0)
            qkv_p2(0, 0)
            cp_k.wait()
            job = plan(TK, [P(prep_qkv, 1, 64, r) for r in range(0, 512, 64)])
            qkv_p1(0, 1)
            qkv_p2(0, 1)
            finish(job)
            qkv_p1(1, 0)
            cp_v.wait()
            cp_wo.wait()
            job = plan(TV, [P(prep_qkv, 2, 64, r) for r in range(0, 512, 64)])
            job_wo = plan(TO, [P(prep_wo, tt, d3, h1) for tt in range(4) for d3 in range(2) for h1 in range(2)])
            qkv_p1(1, 1)
            two(qkv_p2, 1)
            finish(job)
        else:
            attn = plan(QK, qk_items)
            two(qkv_p1, 0)
            two(qkv_p1, 1)
            two(qkv_p2, 0)
            two(qkv_p2, 1)
        two(qkv_p1, 2)
        v_first(first)
        two(qkv_p2, 2)
        finish(attn)
        for half in range(2):
            for r in range(0, HM, 16):
                pv16(half, r)
        if peeled:
            finish(job_wo)
        else:
            w2_p2(pbase, slot, 0)
        two(wo_p1, base)
        halo_save()
        if peeled:
            cp_w1.wait()
            prep_w1_first()
            jobs = {}
            for c in range(1, 7):
                lo = clock[0] + TA[0] + (c - 1) * TA[1]
                jobs[c] = plan((lo, lo + TA[1]), [P(prep_w1, tt, r) for tt in (2 * c, 2 * c + 1) for r in range(0, 512, 64)])
        two(wo_p2, base)
        two(wo_p3, base)
        if not peeled:
            w2_p2(pbase, slot, 1)
        for half in range(2):
            for r in range(0, HM, 16):
                ln2(half, r, not peeled)
        for c in range(NPRE):
            if peeled and c:
                finish(jobs[c])
            w1_pre(c)
        for c in range(7):
            if peeled and c == CB:
                for cc in jobs:
                    finish(jobs[cc])
                cp_w2.wait()
                cp_x1.wait()
                job = plan((clock[0] + T2[0], clock[0] + T2[1]),
                           [P(prep_w2, tt, r) for tt in range(4) for r in range(0, HF, 64)])
            w1_chunk(c, not peeled)
            if c == 0 and not peeled:
                job_ln1 = plan((clock[0] + L1[0], clock[0] + L1[1]), ln1_items)
        if peeled:
            finish(job)
            for r in range(TM, 2 * TM, 64):
                cvt_x(r)
            late = (clock[0] + L1[0], clock[0] + L1[1])
            job_ln1 = plan(late, ln1_items)
            job = plan(late, [P(cvt_x, r) for r in range(2 * TM, S, 64)])
        else:
            finish(job_ln1)
        two(w2_p1, base, slot)
        if peeled:
            finish(job_ln1)
            finish(job)
        assert not queue

    def out_copies(t):
        return [pltpu.make_async_copy(
            ostage.at[t % 2, half],
            out_hbm.at[pl.ds(pl.multiple_of(((t + (NT - 1) * half) % NT) * TM + half * HM, HM), HM), :],
            osem.at[half]) for half in range(2)]

    step(0, True)

    def body(t, c):
        cps = out_copies(t - 1)
        for cp in cps:
            cp.start()
        step(t, False)
        for cp in cps:
            cp.wait()
        return c

    lax.fori_loop(1, 2 * NT, body, 0)
    cps = out_copies(2 * NT - 1)
    for cp in cps:
        cp.start()

    def last_copies(c):
        return [pltpu.make_async_copy(ostage.at[0, 1, :, _tile(4 * side + 2 * c, 2)],
                                      out_hbm.at[pl.ds(S - HM, HM), _tile(4 * side + 2 * c, 2)],
                                      osem.at[2 + 2 * c + side]) for side in range(2)]

    def last_rows(c, _):
        w2_p2(S - TM, 0, c)
        for cp in last_copies(c):
            cp.start()

    lax.fori_loop(0, 2, last_rows, None)
    for cp in cps + last_copies(0) + last_copies(1):
        cp.wait()


@jax.jit
def pallas_interleave_layers__sliding_local_dilated__dense_activation_squared_relu__prompt_kernel(A_x, A_wqkv, A_wo, B_x, B_w1, B_b1, B_w2, B_b2):
    del B_x
    hbm = pl.BlockSpec(memory_space=pl.ANY)
    vmem = pl.BlockSpec(memory_space=pltpu.VMEM)
    V = pltpu.VMEM
    out = pl.pallas_call(
        _kernel,
        in_specs=[hbm, hbm, hbm, hbm, vmem, hbm, vmem],
        out_specs=hbm,
        out_shape=jax.ShapeDtypeStruct((S, D), bf16),
        scratch_shapes=[
            V((2, 2, HM, D), bf16), V((S, D), bf16), V((S, D), f32),
            V((D, 3 * D), bf16), V((D, D), bf16), V((D, F), bf16), V((F, D), bf16),
            V((7, 12, 512, 128), bf16), V((7, 4, 512, 128), bf16),
            V((7, 14, 512, 128), bf16), V((7, 4, HF, 128), bf16),
            V((7, 4, HM, 128), bf16), V((7, 4, HM, 128), bf16), V((7, 4, HM, 128), bf16), V((7, 14, HM, 128), bf16),
            V((8, TM, 128), f32), V((8, TM + HALO, 128), f32), V((8, TM + HALO, 128), f32), V((W, TM, 128), f32),
            V((HM, D), f32), V((TM, D), f32),
            V((3, HM, 512), f32), V((2, HM, 256 * NPRE), f32), V((3, HM, 512), f32),
            V((TM, 128), f32), V((TM, 128), f32), V((TM + HALO, 128), f32), V((TM, 128), f32),
            V((TM, 128), f32), V((TM, 128), f32), V((TM, 128), f32),
            V((8, F), f32), V((8, D), f32), V((8, 128), f32),
            pltpu.SemaphoreType.DMA((14 + 1024 // RQ,)), pltpu.SemaphoreType.DMA((6,)),
        ],
        compiler_params=pltpu.CompilerParams(vmem_limit_bytes=127 * 1024 * 1024),
    )(A_x.reshape(S, D), A_wqkv, A_wo, B_w1, B_b1, B_w2, B_b2)
    return out.reshape(1, S, D)
```
